```python
import jax
import jax.numpy as jnp

def _softmax(x, axis=-1):
    return jax.nn.softmax(x, axis=axis)

def _gelu(x):
    return jax.nn.gelu(x, approximate=True)

def _silu(x):
    return jax.nn.silu(x)

def _sigmoid(x):
    return jax.nn.sigmoid(x)

def _layernorm(x, axis=-1, eps=1e-05):
    m = jnp.mean(x, axis=axis, keepdims=True)
    v = jnp.var(x, axis=axis, keepdims=True)
    return (x - m) / jnp.sqrt(v + eps)

def _scatter_add(tgt, idx, src, axis=0):
    return tgt.at[idx].add(src)

def _segment_sum(src, seg, n):
    return jax.ops.segment_sum(src, seg, n)

class _Rng:

    def __init__(self, key):
        self._k = key

    def _next(self):
        self._k, sub = jax.random.split(self._k)
        return sub

    def normal(self, shape):
        return jax.random.normal(self._next(), shape, dtype=jnp.bfloat16)

    def randint(self, lo, hi, shape):
        return jax.random.randint(self._next(), shape, lo, hi, dtype=jnp.int32)

    def uniform(self, shape, lo=0.0, hi=1.0):
        return jax.random.uniform(self._next(), shape, jnp.bfloat16, lo, hi)

    def permutation(self, n):
        return jax.random.permutation(self._next(), n)
kernel_name = 'sequential_preLN__memory_aug_infini_attn__moe_arch_mod__prompt'

def setup_inputs():
    _rng = _Rng(jax.random.key(int.from_bytes(__import__("os").urandom(4), "little")))
    _w = lambda a: (lambda t: t.astype(jnp.bfloat16) if jnp.issubdtype(t.dtype, jnp.floating) else t)(jnp.asarray(a))

    def _A_setup():
        B, S, D, H = (1, 2048, 576, 32)
        N = 4
        L = max(1, S // N)
        sc = D ** (-0.5)
        return {'x': _w((lambda *s: _rng.normal(s) * 0.05)(B, N * L, D)), 'wq': _w((lambda *s: _rng.normal(s) * 0.05)(D, D) * sc), 'wk': _w((lambda *s: _rng.normal(s) * 0.05)(D, D) * sc), 'wv': _w((lambda *s: _rng.normal(s) * 0.05)(D, D) * sc), 'wo': _w((lambda *s: _rng.normal(s) * 0.05)(D, D) * sc), 'beta': _w((lambda *s: _rng.normal(s) * 0.05)(H))}
    _A_in = _A_setup()

    def _B_setup():
        B, S, D, F, C = (1, 2048, 576, 4608, 1)
        return {'x': _w((lambda *s: _rng.normal(s) * 0.05)(B, S, D)), 'w_r': _w((lambda *s: _rng.normal(s) * 0.05)(D)), 'w_gate': _w((lambda *s: _rng.normal(s) * 0.05)(D, F)), 'w_up': _w((lambda *s: _rng.normal(s) * 0.05)(D, F)), 'w_down': _w((lambda *s: _rng.normal(s) * 0.05)(F, D))}
    _B_in = _B_setup()
    return {'A_x': _A_in['x'], 'A_wq': _A_in['wq'], 'A_wk': _A_in['wk'], 'A_wv': _A_in['wv'], 'A_wo': _A_in['wo'], 'A_beta': _A_in['beta'], 'B_x': _B_in['x'], 'B_w_r': _B_in['w_r'], 'B_w_gate': _B_in['w_gate'], 'B_w_up': _B_in['w_up'], 'B_w_down': _B_in['w_down']}

def reference(A_x, A_wq, A_wk, A_wv, A_wo, A_beta, B_x, B_w_r, B_w_gate, B_w_up, B_w_down):

    def _A_ref(x, wq, wk, wv, wo, beta):
        B, S, D = x.shape
        H = 32
        Dh = D // H
        N = 4
        L = S // N
        q = (lambda x, *d: x.transpose(*d))((x @ wq).reshape(B, S, H, Dh), 0, 2, 1, 3).reshape(B, H, N, L, Dh)
        k = (lambda x, *d: x.transpose(*d))((x @ wk).reshape(B, S, H, Dh), 0, 2, 1, 3).reshape(B, H, N, L, Dh)
        v = (lambda x, *d: x.transpose(*d))((x @ wv).reshape(B, S, H, Dh), 0, 2, 1, 3).reshape(B, H, N, L, Dh)
        phi = lambda t: jnp.where(t > 0, t + 1.0, jnp.exp(t))
        scale = Dh ** (-0.5)
        ar = jnp.arange(L)
        mask = (lambda x, dt: x.astype(dt))(ar[:, None] < ar[None, :], x.dtype) * -1000000000.0
        g = _sigmoid(beta).reshape(1, H, 1, 1)
        M = jnp.einsum('bhd,bhe->bhde', q[:, :, 0, 0, :] * 0.0, q[:, :, 0, 0, :] * 0.0)
        z = q[:, :, 0, 0, :] * 0.0
        outs = []
        for s in range(N):
            qs, ks, vs = (q[:, :, s].copy(), k[:, :, s].copy(), v[:, :, s].copy())
            logits = jnp.einsum('bhqd,bhkd->bhqk', qs, ks) * scale + mask
            p = _softmax(logits, axis=-1)
            a_dot = jnp.einsum('bhqk,bhkd->bhqd', p, vs)
            pq = phi(qs)
            num = jnp.einsum('bhld,bhde->bhle', pq, M)
            den = jnp.einsum('bhld,bhd->bhl', pq, z)[..., None] + 1e-06
            a_mem = num / den
            o = g * a_mem + (1.0 - g) * a_dot
            outs.append(o)
            pk = phi(ks)
            M = M + jnp.einsum('bhld,bhle->bhde', pk, vs)
            z = z + jnp.einsum('bhld->bhd', pk)
        o = (lambda x, *d: x.transpose(*d))(jnp.stack(outs, 2).reshape(B, H, S, Dh), 0, 2, 1, 3).reshape(B, S, D)
        return o @ wo

    def _B_ref(x, w_r, w_gate, w_up, w_down):
        B, S, D = x.shape
        C = 1
        r = x @ w_r
        idx = jnp.argsort(-r, axis=-1)[:, :C]
        idx_e = jnp.repeat(idx.reshape(B, C, 1), D, axis=2)
        x_sel = jnp.take_along_axis(x, idx_e, axis=1)
        g = _silu(x_sel @ w_gate)
        u = x_sel @ w_up
        y = g * u @ w_down
        r_sel = _sigmoid(jnp.take_along_axis(r, idx, axis=1))
        y = y * r_sel.reshape(B, C, 1)
        b_off = (jnp.arange(B) * S).reshape(B, 1)
        flat_idx = (idx + b_off).reshape(B * C)
        zero = (x * 0.0).reshape(B * S, D)
        upd = _scatter_add(zero, flat_idx, y.reshape(B * C, D), axis=0)
        return x + upd.reshape(B, S, D)
    x = A_x
    h = x + _A_ref(_layernorm(x, axis=-1), A_wq, A_wk, A_wv, A_wo, A_beta)
    h2 = h + _B_ref(_layernorm(h, axis=-1), B_w_r, B_w_gate, B_w_up, B_w_down)
    return h2
```

```python
import jax
import jax.numpy as jnp
from jax import lax
import jax.experimental.pallas as pl
import jax.experimental.pallas.tpu as pltpu

u32 = jnp.uint32
f32 = jnp.float32
bf16 = jnp.bfloat16
i32 = jnp.int32

S = 2048
D = 576
DP = 640
F = 4608
NSEG = 4
L = 512
H = 32
DH = 18
NG = 5
OFF = (0, 128, 384, 768)
LOG2E = 1.4426950408889634
QSCALE = float(DH ** (-0.5)) * LOG2E
EPS = 1e-05
BOUND = 30.0
VBOUND = 1e20
NT = (((1,), (1,)), ((), ()))
UN_FAST = 8
UN_SLOW = 2


def _unpack(x):
    return pltpu.bitcast(x, bf16)


def _pack(x):
    return pltpu.bitcast(x, u32)


def _iota(shape, dim):
    return lax.broadcasted_iota(i32, shape, dim)


def _perm_rows(w):
    c = w.shape[1]
    parts = []
    for g in range(NG):
        if g < NG - 1:
            parts += [w[63 * g:63 * g + 63], jnp.zeros((1, c), u32)]
        else:
            parts += [w[252:288], jnp.zeros((28, c), u32)]
    return jnp.concatenate(parts, axis=0)


def _pad_lanes(x):
    return jnp.concatenate([x, jnp.zeros((x.shape[0], DP - D), x.dtype)], axis=1)


def _layernorm(xf):
    m = jnp.sum(xf, axis=1, keepdims=True) * (1.0 / D)
    xc = xf - m
    v = jnp.sum(xc * xc, axis=1, keepdims=True) * (1.0 / D)
    return xc * lax.rsqrt(v + EPS)


def _phi(t):
    return jnp.where(t > 0, t + 1.0, jnp.exp2(t * LOG2E))


def _sigmoid(t):
    return 1.0 / (1.0 + jnp.exp(-t))


def _kernel(x_hbm, wq_hbm, wk_hbm, wv_hbm, wo_hbm, beta_ref, wr_ref, wg_hbm, wu_hbm, wd_hbm,
            out_hbm,
            x_v, wq_v, wk_v, wv_v, wo_v, wg_v, wu_v, wd_v,
            wqvt, wkt, wop, xn, kp, phk, qt, phq, vt, ot, pb0, pb1, sb0, sb1, mb0, mb1,
            mt, mlhs, h_v, hn_v, out_v, msk, omg, grow, best, sems):

    def cp(src, dst, i):
        return pltpu.make_async_copy(src, dst, sems.at[i])

    x_cp = [cp(x_hbm.at[pl.ds(L * s, L)], x_v.at[pl.ds(L * s, L)], s) for s in range(NSEG)]
    wk_cp, wq_cp, wv_cp, wo_cp = (cp(wk_hbm, wk_v, 4), cp(wq_hbm, wq_v, 5),
                                  cp(wv_hbm, wv_v, 6), cp(wo_hbm, wo_v, 7))
    wg_cp, wu_cp, wd_cp = cp(wg_hbm, wg_v, 8), cp(wu_hbm, wu_v, 9), cp(wd_hbm, wd_v, 10)
    o_cp = [cp(out_v.at[pl.ds(L * s, L)], out_hbm.at[pl.ds(L * s, L)], 11 + s) for s in range(NSEG)]

    x_cp[0].start()
    wk_cp.start()
    wq_cp.start()
    wv_cp.start()
    wo_cp.start()
    for s in range(1, NSEG):
        x_cp[s].start()
    wg_cp.start()
    wu_cp.start()
    wd_cp.start()

    r64 = _iota((64, 128), 0)
    for j in range(7):
        msk[j] = jnp.where((r64 >= 9 * j) & (r64 < 9 * j + 9), u32(0xFFFFFFFF), u32(0))
    g_lane = _sigmoid(beta_ref[...].astype(f32))
    g_lane = jnp.concatenate([g_lane, jnp.zeros((1, 128 - H), f32)], axis=1)
    lane128 = _iota((128, 128), 1)
    row128 = _iota((128, 128), 0)
    head_in_group = lax.shift_right_logical(row128 * 57, 10)
    for g in range(NG):
        hid = jnp.where(head_in_group < 7, head_in_group + 7 * g, 999)
        sel = jnp.where(lane128 == hid, jnp.broadcast_to(g_lane, (128, 128)), 0.0)
        grow[g] = jnp.broadcast_to(jnp.sum(sel, axis=1, keepdims=True), (128, 128))
    r32 = _iota((32, 128), 0)
    for h in range(H):
        j = h % 7
        off = 18 * j - 16 * ((9 * j) // 8)
        gh = jnp.broadcast_to(g_lane[:, h:h + 1], (32, 128))
        omg[h] = jnp.where((r32 >= off) & (r32 < off + 18), 1.0 - gh, 0.0)
    head_col = lax.shift_right_logical(lane128 * 57, 10)
    bd_mask = (head_in_group == head_col) & (head_in_group < 7)

    def prep_t(w_ref):
        wt = _pack(w_ref[...].T)
        return _pad_lanes(_perm_rows(wt))

    wk_cp.wait()
    wkt[...] = prep_t(wk_v)
    wq_cp.wait()
    wqvt[0:320, :] = prep_t(wq_v)
    wv_cp.wait()
    wqvt[320:640, :] = prep_t(wv_v)
    wo_cp.wait()
    wop[...] = _pad_lanes(_perm_rows(_pack(wo_v[...])))

    best[0] = jnp.full((8, 128), -jnp.inf, f32)
    best[1] = jnp.zeros((8, 128), f32)
    wr = wr_ref[...].astype(f32)

    diag = _iota((128, 128), 0) <= _iota((128, 128), 1)

    def qk_logits(h, i):
        g, j = h // 7, h % 7
        n = 128 * (i + 1)
        qw = qt[g, :, 128 * i:128 * (i + 1)] & msk[j]
        s = jnp.dot(_unpack(kp[g, 0:n // 2, :]), _unpack(qw), preferred_element_type=f32)
        sl = jnp.where(diag, s[n - 128:], -1e30)
        return sl if i == 0 else jnp.concatenate([s[:n - 128], sl], axis=0)

    def pv(h, i, pb):
        g, j = h // 7, h % 7
        n = 128 * (i + 1)
        a8 = pl.multiple_of(((9 * j) // 8) * 8, 8)
        vw = vt[g, pl.ds(a8, 16), 0:n]
        mk = msk[j, pl.ds(a8, 16), :]
        mk = jnp.concatenate([mk] * (i + 1), axis=1)
        vw = (vw & mk) | (jnp.full((16, n), 0x3F803F80, u32) & ~mk)
        o = jnp.dot(_unpack(vw), pb, preferred_element_type=f32)
        og = omg[h]
        mk0 = _unpack(mk[:, 0:128]).astype(f32)
        del mk0
        r32_ = _iota((32, 128), 0)
        off = 18 * j - 2 * a8
        is_head = (r32_ >= off) & (r32_ < off + 18)
        lsum = jnp.sum(jnp.where(is_head, 0.0, o), axis=0, keepdims=True)
        r = pl.reciprocal(lsum, approx=True) * 14.0
        w16 = pl.multiple_of(a8 * 2, 16)
        ot[g, pl.ds(w16, 32), 128 * i:128 * (i + 1)] += o * (r * og)

    pbs = (pb0, pb1)
    sbs = (sb0, sb1)
    mbs = (mb0, mb1)
    IORD = (3, 2, 1, 0)

    def fast_qk(h, i, pbuf):
        n = 128 * (i + 1)
        p = jnp.exp2(qk_logits(h, i)).astype(bf16)
        pbuf[OFF[i] // 2:(OFF[i] + n) // 2, :] = _pack(p)

    def fast_pv(h, i, pbuf):
        n = 128 * (i + 1)
        pv(h, i, _unpack(pbuf[OFF[i] // 2:(OFF[i] + n) // 2, :]))

    def slow_qk(h, i, sbuf, mbuf):
        n = 128 * (i + 1)
        s = qk_logits(h, i)
        sbuf[OFF[i]:OFF[i] + n, :] = s
        mbuf[8 * i:8 * i + 8, :] = jnp.broadcast_to(jnp.max(s, axis=0, keepdims=True), (8, 128))

    def slow_pv(h, i, sbuf, mbuf):
        n = 128 * (i + 1)
        s = sbuf[OFF[i]:OFF[i] + n, :]
        p = jnp.exp2(s - mbuf[8 * i:8 * i + 1, :]).astype(bf16)
        pv(h, i, p)

    def attention_fast():
        for i in IORD:
            fast_qk(0, i, pbs[0])

        def body(it, c):
            for u in range(UN_FAST):
                h = it * UN_FAST + u
                hn_ = jnp.minimum(h + 1, H - 1)
                for i in IORD:
                    fast_qk(hn_, i, pbs[1 - u % 2])
                for i in IORD:
                    fast_pv(h, i, pbs[u % 2])
            return c
        lax.fori_loop(0, H // UN_FAST, body, 0)

    def attention_slow():
        for i in IORD:
            slow_qk(0, i, sbs[0], mbs[0])

        def body(it, c):
            for u in range(UN_SLOW):
                h = it * UN_SLOW + u
                hn_ = jnp.minimum(h + 1, H - 1)
                for i in IORD:
                    slow_qk(hn_, i, sbs[1 - u % 2], mbs[1 - u % 2])
                for i in IORD:
                    slow_pv(h, i, sbs[u % 2], mbs[u % 2])
            return c
        lax.fori_loop(0, H // UN_SLOW, body, 0)

    def segment(s, c):
        r0 = pl.multiple_of(s * L, L)
        for t in range(NSEG):
            @pl.when(s == t)
            def _():
                x_cp[t].wait()

        xf = x_v[pl.ds(r0, L), :].astype(f32)
        xnb = _pad_lanes(_layernorm(xf).astype(bf16))
        xn[...] = _pack(xnb)
        xnv = _unpack(xn[...])

        kf = lax.dot_general(xnv, _unpack(wkt[...]), NT, preferred_element_type=f32)
        kb = _pack(kf.astype(bf16))
        pk = _pack(_phi(kf).astype(bf16))
        for g in range(NG):
            kp[g] = kb[:, 128 * g:128 * (g + 1)]
            phk[g] = pk[:, 128 * g:128 * (g + 1)]
        mk_ = jnp.max(jnp.max(jnp.abs(kf), axis=0, keepdims=True), axis=1, keepdims=True)

        qv = lax.dot_general(_unpack(wqvt[...]), xnv, NT, preferred_element_type=f32)
        qf = qv[0:DP]
        vf = qv[DP:2 * DP]
        qs = qf * QSCALE
        qb = _pack(qs.astype(bf16))
        pq = _pack(_phi(qf).astype(bf16))
        vb = _pack(vf.astype(bf16))
        for g in range(NG):
            qt[g] = qb[64 * g:64 * (g + 1)]
            phq[g] = pq[64 * g:64 * (g + 1)]
            vt[g] = vb[64 * g:64 * (g + 1)]
        mq_ = jnp.max(jnp.max(jnp.abs(qs), axis=0, keepdims=True), axis=1, keepdims=True)
        mv_ = jnp.max(jnp.max(jnp.abs(vf), axis=0, keepdims=True), axis=1, keepdims=True)
        bound = mq_ * mk_ * (DH * 1.02)
        ok = jnp.where((bound <= BOUND) & (mv_ <= VBOUND), 1, 0).astype(i32)
        safe = jnp.max(ok) > 0

        @pl.when(s == 0)
        def _():
            ot[...] = jnp.zeros((NG, 128, L), f32)

        @pl.when(s > 0)
        def _():
            for g in range(NG):
                nd = jnp.dot(_unpack(mlhs[g]), _unpack(phq[g]), preferred_element_type=f32)
                num = nd[0:128]
                den = nd[128:256] + 1e-06
                gr = grow[g]
                ot[g] = num * (pl.reciprocal(den, approx=True) * jnp.concatenate([gr] * 4, axis=1))

        @pl.when(safe)
        def _():
            attention_fast()

        @pl.when(jnp.logical_not(safe))
        def _():
            attention_slow()

        @pl.when(s < NSEG - 1)
        def _():
            r64_ = _iota((64, L), 0)
            ones = jnp.full((64, L), 0x3F803F80, u32)
            for g in range(NG):
                lhs = jnp.where(r64_ == 63, ones, vt[g])
                upd = jnp.dot(_unpack(lhs), _unpack(phk[g]), preferred_element_type=f32)
                prev = jnp.where(s == 0, 0.0, mt[g])
                cur = prev + upd
                mt[g] = cur
                m_bd = jnp.where(bd_mask, cur, 0.0)
                z_bd = jnp.where(bd_mask, jnp.broadcast_to(cur[126:127, :], (128, 128)), 0.0)
                mlhs[g] = _pack(jnp.concatenate([m_bd, z_bd], axis=0).astype(bf16))

        ob = jnp.concatenate([ot[g] for g in range(NG)], axis=0).astype(bf16)
        on = ob.T
        ao = jnp.dot(on, _unpack(wop[...]), preferred_element_type=f32)[:, 0:D]
        hb = (x_v[pl.ds(r0, L), :].astype(f32) + ao).astype(bf16)
        hf = hb.astype(f32)
        hnb = _layernorm(hf).astype(bf16)
        hnf = hnb.astype(f32)
        h_v[pl.ds(r0, L), :] = hb
        hn_v[pl.ds(r0, L), :] = hnb
        out_v[pl.ds(r0, L), :] = (hf + hnf).astype(bf16)
        rr = jnp.sum(hnf * wr, axis=1, keepdims=True).astype(bf16).astype(f32)
        rr = jnp.broadcast_to(rr, (L, 128))
        bv = best[0]
        bi = best[1]
        sub = _iota((8, 128), 0).astype(f32)
        base = (s * L).astype(f32)
        for t in range(L // 8):
            rt = rr[8 * t:8 * t + 8]
            upd_ = rt > bv
            bv = jnp.where(upd_, rt, bv)
            bi = jnp.where(upd_, sub + (base + float(8 * t)), bi)
        best[0] = bv
        best[1] = bi
        for t in range(NSEG):
            @pl.when(s == t)
            def _():
                o_cp[t].start()
        return c

    mt[...] = jnp.zeros((NG, 128, 128), f32)
    lax.fori_loop(0, NSEG, segment, 0)

    bv = best[0]
    bi = best[1]
    vmax = jnp.max(bv, axis=0, keepdims=True)
    cand = jnp.where(bv == vmax, bi, float(S))
    imin = jnp.min(cand, axis=0, keepdims=True)
    idx = jnp.minimum(jnp.max(imin).astype(i32), S - 1)
    idx16 = pl.multiple_of((idx // 16) * 16, 16)
    sel = (_iota((16, 1), 0) + idx16) == idx
    hn16 = hn_v[pl.ds(idx16, 16), :]
    h16 = h_v[pl.ds(idx16, 16), :]
    xs = jnp.where(sel, hn16, jnp.zeros_like(hn16))
    wg_cp.wait()
    wu_cp.wait()
    gt = jnp.dot(xs, wg_v[...], preferred_element_type=f32)
    up = jnp.dot(xs, wu_v[...], preferred_element_type=f32)
    act = (gt * _sigmoid(gt) * up).astype(bf16)
    wd_cp.wait()
    y = jnp.dot(act, wd_v[...], preferred_element_type=f32)
    rsel = _sigmoid(vmax[:, 0:1])
    y = (y * rsel).astype(bf16).astype(f32)
    fin = (h16.astype(f32) + (hn16.astype(f32) + jnp.where(sel, y, 0.0))).astype(bf16)
    for s in range(NSEG):
        o_cp[s].wait()
    out_v[pl.ds(idx16, 16), :] = fin
    pc = cp(out_v.at[pl.ds(idx16, 16)], out_hbm.at[pl.ds(idx16, 16)], 15)
    pc.start()
    pc.wait()


@jax.jit
def pallas_sequential_preLN__memory_aug_infini_attn__moe_arch_mod__prompt_kernel(
    A_x: jax.Array,
    A_wq: jax.Array,
    A_wk: jax.Array,
    A_wv: jax.Array,
    A_wo: jax.Array,
    A_beta: jax.Array,
    B_x: jax.Array,
    B_w_r: jax.Array,
    B_w_gate: jax.Array,
    B_w_up: jax.Array,
    B_w_down: jax.Array,
):
    del B_x
    x = A_x.reshape(S, D)
    beta = A_beta.reshape(1, H)
    wr = B_w_r.reshape(1, D)
    anyspec = pl.BlockSpec(memory_space=pl.ANY)
    vm = pl.BlockSpec(memory_space=pltpu.VMEM)
    V = pltpu.VMEM
    scratch = [
        V((S, D), bf16),
        V((D, D), bf16), V((D, D), bf16), V((D, D), bf16), V((D, D), bf16),
        V((D, F), bf16), V((D, F), bf16), V((F, D), bf16),
        V((2 * DP // 2, DP), u32),
        V((DP // 2, DP), u32),
        V((DP // 2, DP), u32),
        V((L // 2, DP), u32),
        V((NG, L // 2, 128), u32),
        V((NG, L // 2, 128), u32),
        V((NG, 64, L), u32),
        V((NG, 64, L), u32),
        V((NG, 64, L), u32),
        V((NG, 128, L), f32),
        V((640, 128), u32), V((640, 128), u32),
        V((1280, 128), f32), V((1280, 128), f32),
        V((32, 128), f32), V((32, 128), f32),
        V((NG, 128, 128), f32),
        V((NG, 128, 128), u32),
        V((S, D), bf16), V((S, D), bf16), V((S, D), bf16),
        V((7, 64, 128), u32),
        V((H, 32, 128), f32),
        V((NG, 128, 128), f32),
        V((2, 8, 128), f32),
        pltpu.SemaphoreType.DMA((16,)),
    ]
    out = pl.pallas_call(
        _kernel,
        out_shape=jax.ShapeDtypeStruct((S, D), bf16),
        in_specs=[anyspec, anyspec, anyspec, anyspec, anyspec, vm, vm, anyspec, anyspec, anyspec],
        out_specs=anyspec,
        scratch_shapes=scratch,
        compiler_params=pltpu.CompilerParams(vmem_limit_bytes=100 * 1024 * 1024),
    )(x, A_wq, A_wk, A_wv, A_wo, beta, wr, B_w_gate, B_w_up, B_w_down)
    return out.reshape(1, S, D)
```

```python
import jax
import jax.numpy as jnp
from jax import lax
import jax.experimental.pallas as pl
import jax.experimental.pallas.tpu as pltpu

u32 = jnp.uint32
f32 = jnp.float32
bf16 = jnp.bfloat16
i32 = jnp.int32

S = 2048
D = 576
DP = 640
DC = 592
F = 4608
NSEG = 4
L = 512
NTILE = S // 128
H = 32
DH = 18
NG = 5
OFF = (0, 128, 384, 768)
LOG2E = 1.4426950408889634
QSCALE = float(DH ** (-0.5)) * LOG2E
EPS = 1e-05
BOUND = 30.0
VBOUND = 1e20
NT = (((1,), (1,)), ((), ()))
UN_FAST = 8
UN_SLOW = 2


def _unpack(x):
    return pltpu.bitcast(x, bf16)


def _pack(x):
    return pltpu.bitcast(x, u32)


def _iota(shape, dim):
    return lax.broadcasted_iota(i32, shape, dim)


def _perm_rows(w, tail):
    c = w.shape[1]
    parts = []
    for g in range(NG):
        if g < NG - 1:
            parts += [w[63 * g:63 * g + 63], jnp.zeros((1, c), u32)]
        else:
            parts += [w[252:288], jnp.zeros((tail - 36, c), u32)]
    return jnp.concatenate(parts, axis=0)


def _pad_lanes(x):
    return jnp.concatenate([x, jnp.zeros((x.shape[0], DP - D), x.dtype)], axis=1)


def _layernorm_t(xf):
    m = jnp.sum(xf, axis=0, keepdims=True) * (1.0 / D)
    xc = xf - m
    v = jnp.sum(xc * xc, axis=0, keepdims=True) * (1.0 / D)
    return xc * lax.rsqrt(v + EPS)


def _phi(t):
    return jnp.where(t > 0, t + 1.0, jnp.exp2(t * LOG2E))


def _sigmoid(t):
    return 1.0 / (1.0 + jnp.exp(-t))


def _absmax(x):
    return jnp.max(jnp.max(jnp.abs(x), axis=0, keepdims=True), axis=1, keepdims=True)


def _kernel(x_hbm, wq_hbm, wk_hbm, wv_hbm, wo_hbm, beta_ref, wr_ref, wg_hbm, wu_hbm, wd_hbm,
            out_hbm,
            x_v, wq_v, wk_v, wv_v, wo_v, wg_v, wu_v, wd_v,
            wall, wot, xn, kp, phk, qt, phq, vt, ot, pb0, pb1, sb0, sb1, mb0, mb1,
            mt, mlhs, h_v, hn_v, out_v, msk, omg, grow, wcol, best, sems):

    def cp(src, dst, i):
        return pltpu.make_async_copy(src, dst, sems.at[i])

    x_cp = [cp(x_hbm.at[:, pl.ds(128 * t, 128)], x_v.at[t], t // 4) for t in range(NTILE)]
    wq_cp, wk_cp, wv_cp, wo_cp = (cp(wq_hbm, wq_v, 4), cp(wk_hbm, wk_v, 5),
                                  cp(wv_hbm, wv_v, 6), cp(wo_hbm, wo_v, 7))
    wg_cp, wu_cp, wd_cp = cp(wg_hbm, wg_v, 8), cp(wu_hbm, wu_v, 9), cp(wd_hbm, wd_v, 10)
    o_cp = [cp(out_v.at[t], out_hbm.at[:, pl.ds(128 * t, 128)], 11 + t // 4) for t in range(NTILE)]

    wq_cp.start()
    for t in range(4):
        x_cp[t].start()
    wk_cp.start()
    wv_cp.start()
    wo_cp.start()
    for t in range(4, NTILE):
        x_cp[t].start()
    wg_cp.start()
    wu_cp.start()
    wd_cp.start()

    r64 = _iota((64, 128), 0)
    for j in range(7):
        msk[j] = jnp.where((r64 >= 9 * j) & (r64 < 9 * j + 9), u32(0xFFFFFFFF), u32(0))
    g_lane = _sigmoid(beta_ref[...].astype(f32))
    g_lane = jnp.concatenate([g_lane, jnp.zeros((1, 128 - H), f32)], axis=1)
    lane128 = _iota((128, 128), 1)
    row128 = _iota((128, 128), 0)
    head_in_group = lax.shift_right_logical(row128 * 57, 10)
    for g in range(NG):
        hid = jnp.where(head_in_group < 7, head_in_group + 7 * g, 999)
        sel = jnp.where(lane128 == hid, jnp.broadcast_to(g_lane, (128, 128)), 0.0)
        grow[g] = jnp.broadcast_to(jnp.sum(sel, axis=1, keepdims=True), (128, 128))
    r32 = _iota((32, 128), 0)
    for h in range(H):
        j = h % 7
        off = 18 * j - 16 * ((9 * j) // 8)
        gh = jnp.broadcast_to(g_lane[:, h:h + 1], (32, 128))
        omg[h] = jnp.where((r32 >= off) & (r32 < off + 18), 1.0 - gh, 0.0)
    head_col = lax.shift_right_logical(lane128 * 57, 10)
    bd_mask = (head_in_group == head_col) & (head_in_group < 7)
    wr = _pad_lanes(wr_ref[...].astype(f32))
    wcol[...] = jnp.broadcast_to(wr, (128, DP)).T[0:D]
    xn[288:320, :] = jnp.zeros((32, L), u32)
    best[0] = jnp.full((8, 128), -jnp.inf, f32)
    best[1] = jnp.zeros((8, 128), f32)
    mt[...] = jnp.zeros((NG, 128, 128), f32)

    def prep_t(w_ref):
        wt = _pack(w_ref[...].T)
        return _pad_lanes(_perm_rows(wt, 40))

    wq_cp.wait()
    wall[0:296, :] = prep_t(wq_v)
    wk_cp.wait()
    wall[296:592, :] = prep_t(wk_v)
    wv_cp.wait()
    wall[592:888, :] = prep_t(wv_v)
    wo_cp.wait()
    wot[...] = _pack(_unpack(_perm_rows(_pack(wo_v[...]), 64)).T)

    diag = _iota((128, 128), 0) <= _iota((128, 128), 1)

    def qk_logits(h, i):
        g, j = h // 7, h % 7
        n = 128 * (i + 1)
        qw = qt[g, :, 128 * i:128 * (i + 1)] & msk[j]
        s = jnp.dot(_unpack(kp[g, 0:n // 2, :]), _unpack(qw), preferred_element_type=f32)
        sl = jnp.where(diag, s[n - 128:], -1e30)
        return sl if i == 0 else jnp.concatenate([s[:n - 128], sl], axis=0)

    def pv(h, i, pb):
        g, j = h // 7, h % 7
        n = 128 * (i + 1)
        a8 = pl.multiple_of(((9 * j) // 8) * 8, 8)
        vw = vt[g, pl.ds(a8, 16), 0:n]
        mk = msk[j, pl.ds(a8, 16), :]
        mk = jnp.concatenate([mk] * (i + 1), axis=1)
        vw = (vw & mk) | (jnp.full((16, n), 0x3F803F80, u32) & ~mk)
        o = jnp.dot(_unpack(vw), pb, preferred_element_type=f32)
        og = omg[h]
        r32_ = _iota((32, 128), 0)
        off = 18 * j - 2 * a8
        is_head = (r32_ >= off) & (r32_ < off + 18)
        lsum = jnp.sum(jnp.where(is_head, 0.0, o), axis=0, keepdims=True)
        r = pl.reciprocal(lsum, approx=True) * 14.0
        w16 = pl.multiple_of(a8 * 2, 16)
        ot[g, pl.ds(w16, 32), 128 * i:128 * (i + 1)] += o * (r * og)

    pbs = (pb0, pb1)
    sbs = (sb0, sb1)
    mbs = (mb0, mb1)
    IORD = (3, 2, 1, 0)

    def fast_qk(h, i, pbuf):
        n = 128 * (i + 1)
        p = jnp.exp2(qk_logits(h, i)).astype(bf16)
        pbuf[OFF[i] // 2:(OFF[i] + n) // 2, :] = _pack(p)

    def fast_pv(h, i, pbuf):
        n = 128 * (i + 1)
        pv(h, i, _unpack(pbuf[OFF[i] // 2:(OFF[i] + n) // 2, :]))

    def slow_qk(h, i, sbuf, mbuf):
        n = 128 * (i + 1)
        s = qk_logits(h, i)
        sbuf[OFF[i]:OFF[i] + n, :] = s
        mbuf[8 * i:8 * i + 8, :] = jnp.broadcast_to(jnp.max(s, axis=0, keepdims=True), (8, 128))

    def slow_pv(h, i, sbuf, mbuf):
        n = 128 * (i + 1)
        s = sbuf[OFF[i]:OFF[i] + n, :]
        p = jnp.exp2(s - mbuf[8 * i:8 * i + 1, :]).astype(bf16)
        pv(h, i, p)

    def attention_fast():
        for i in IORD:
            fast_qk(0, i, pbs[0])

        def body(it, c):
            for u in range(UN_FAST):
                h = it * UN_FAST + u
                hn_ = jnp.minimum(h + 1, H - 1)
                for i in IORD:
                    fast_qk(hn_, i, pbs[1 - u % 2])
                for i in IORD:
                    fast_pv(h, i, pbs[u % 2])
            return c
        lax.fori_loop(0, H // UN_FAST, body, 0)

    def attention_slow():
        for i in IORD:
            slow_qk(0, i, sbs[0], mbs[0])

        def body(it, c):
            for u in range(UN_SLOW):
                h = it * UN_SLOW + u
                hn_ = jnp.minimum(h + 1, H - 1)
                for i in IORD:
                    slow_qk(hn_, i, sbs[1 - u % 2], mbs[1 - u % 2])
                for i in IORD:
                    slow_pv(h, i, sbs[u % 2], mbs[u % 2])
            return c
        lax.fori_loop(0, H // UN_SLOW, body, 0)

    def segment(s, c):
        for t in range(NSEG):
            @pl.when(s == t)
            def _():
                for u in range(4):
                    x_cp[4 * t + u].wait()

        for t in range(4):
            xf = x_v[4 * s + t].astype(f32)
            xn[0:288, 128 * t:128 * (t + 1)] = _pack(_layernorm_t(xf).astype(bf16))

        qkv = jnp.dot(_unpack(wall[...]), _unpack(xn[...]), preferred_element_type=f32)
        mx = []
        for w in range(3):
            m_ = None
            for g in range(NG):
                nr = 128 if g < NG - 1 else 80
                a = qkv[DC * w + 128 * g:DC * w + 128 * g + nr]
                if w == 0:
                    phq[g, 0:nr // 2] = _pack(_phi(a).astype(bf16))
                    a = a * QSCALE
                    qt[g, 0:nr // 2] = _pack(a.astype(bf16))
                elif w == 1:
                    phk[g, 0:nr // 2] = _pack(_phi(a).astype(bf16))
                    ab = a.astype(bf16)
                    if nr < 128:
                        ab = jnp.concatenate([ab, jnp.zeros((128 - nr, L), bf16)], axis=0)
                    kp[g] = _pack(ab.T)
                else:
                    vt[g, 0:nr // 2] = _pack(a.astype(bf16))
                am = jnp.max(jnp.abs(a).reshape(nr // 8, 8, L), axis=0)
                m_ = am if m_ is None else jnp.maximum(m_, am)
            mx.append(_absmax(m_))
        bound = mx[0] * mx[1] * (DH * 1.02)
        ok = jnp.where((bound <= BOUND) & (mx[2] <= VBOUND), 1, 0).astype(i32)
        safe = jnp.max(ok) > 0

        @pl.when(s == 0)
        def _():
            ot[...] = jnp.zeros((NG, 128, L), f32)
            for ref in (qt, phq, phk, vt):
                ref[NG - 1, 40:64] = jnp.zeros((24, L), u32)

        @pl.when(s > 0)
        def _():
            for g in range(NG):
                nd = jnp.dot(_unpack(mlhs[g]), _unpack(phq[g]), preferred_element_type=f32)
                num = nd[0:128]
                den = nd[128:256] + 1e-06
                gr = grow[g]
                ot[g] = num * (pl.reciprocal(den, approx=True) * jnp.concatenate([gr] * 4, axis=1))

        @pl.when(safe)
        def _():
            attention_fast()

        @pl.when(jnp.logical_not(safe))
        def _():
            attention_slow()

        @pl.when(s < NSEG - 1)
        def _():
            r64_ = _iota((64, L), 0)
            ones = jnp.full((64, L), 0x3F803F80, u32)
            for g in range(NG):
                lhs = jnp.where(r64_ == 63, ones, vt[g])
                upd = lax.dot_general(_unpack(lhs), _unpack(phk[g]), NT,
                                      preferred_element_type=f32)
                cur = mt[g] + upd
                mt[g] = cur
                m_bd = jnp.where(bd_mask, cur, 0.0)
                z_bd = jnp.where(bd_mask, jnp.broadcast_to(cur[126:127, :], (128, 128)), 0.0)
                mlhs[g] = _pack(jnp.concatenate([m_bd, z_bd], axis=0).astype(bf16))

        ob = jnp.concatenate([ot[g] for g in range(NG)], axis=0).astype(bf16)
        ao = jnp.dot(_unpack(wot[...]), ob, preferred_element_type=f32)
        bv = best[0]
        bi = best[1]
        lane = _iota((8, 128), 1).astype(f32)
        for t in range(4):
            hb = (x_v[4 * s + t].astype(f32) + ao[:, 128 * t:128 * (t + 1)]).astype(bf16)
            hf = hb.astype(f32)
            hnb = _layernorm_t(hf).astype(bf16)
            hnf = hnb.astype(f32)
            h_v[4 * s + t] = hb
            hn_v[4 * s + t] = hnb
            out_v[4 * s + t] = (hf + hnf).astype(bf16)
            rr = jnp.sum(hnf * wcol[...], axis=0, keepdims=True).astype(bf16).astype(f32)
            rt = jnp.broadcast_to(rr, (8, 128))
            upd_ = rt > bv
            bv = jnp.where(upd_, rt, bv)
            bi = jnp.where(upd_, lane + (s * L + 128 * t).astype(f32), bi)
        best[0] = bv
        best[1] = bi
        for t in range(NSEG):
            @pl.when(s == t)
            def _():
                for u in range(4):
                    o_cp[4 * t + u].start()
        return c

    lax.fori_loop(0, NSEG, segment, 0)

    bv = best[0]
    bi = best[1]
    vmax = jnp.max(bv, axis=1, keepdims=True)
    cand = jnp.where(bv == vmax, bi, float(S))
    imin = jnp.min(cand, axis=1, keepdims=True)
    idx = jnp.minimum(jnp.max(imin).astype(i32), S - 1)
    tile = idx // 128
    col = idx - tile * 128
    col16 = pl.multiple_of((col // 16) * 16, 16)
    hn_t = hn_v[tile]
    lane_sel = _iota((D, 128), 1) == col
    xs_t = jnp.where(lane_sel, hn_t, jnp.zeros_like(hn_t))
    xs_t = jnp.concatenate([xs_t, jnp.zeros((DP - D, 128), bf16)], axis=0)
    pb0[0:64, :] = jnp.zeros((64, 128), u32)
    xall = xs_t.T
    xn[0:64, 0:L] = _pack(xall[:, 0:L])
    pb0[0:64, :] = _pack(xall[:, L:DP])
    c8 = pl.multiple_of(col16 // 2, 8)
    xs = _unpack(jnp.concatenate([xn[pl.ds(c8, 8), 0:L], pb0[pl.ds(c8, 8), 0:64]], axis=1))
    wg_cp.wait()
    wu_cp.wait()
    gt = jnp.dot(xs, wg_v[...], preferred_element_type=f32)
    up = jnp.dot(xs, wu_v[...], preferred_element_type=f32)
    act = (gt * _sigmoid(gt) * up).astype(bf16)
    wd_cp.wait()
    y = lax.dot_general(act, wd_v[...], NT, preferred_element_type=f32)
    rsel = _sigmoid(vmax[0:1, 0:1])
    yb = (y * rsel).astype(bf16)
    y128 = jnp.concatenate([_pad_lanes(yb), jnp.zeros((112, DP), bf16)], axis=0)
    yt = y128.T[0:D].astype(f32)
    ycol = jnp.sum(jnp.where(_iota((D, 128), 1) == (col - col16), yt, 0.0), axis=1, keepdims=True)
    fin = (h_v[tile].astype(f32)
           + (hn_t.astype(f32) + jnp.where(lane_sel, ycol, 0.0))).astype(bf16)
    for t in range(NTILE):
        o_cp[t].wait()
    out_v[tile] = fin
    pc = cp(out_v.at[tile], out_hbm.at[:, pl.ds(pl.multiple_of(tile * 128, 128), 128)], 15)
    pc.start()
    pc.wait()


@jax.jit
def pallas_sequential_preLN__memory_aug_infini_attn__moe_arch_mod__prompt_kernel(
    A_x: jax.Array,
    A_wq: jax.Array,
    A_wk: jax.Array,
    A_wv: jax.Array,
    A_wo: jax.Array,
    A_beta: jax.Array,
    B_x: jax.Array,
    B_w_r: jax.Array,
    B_w_gate: jax.Array,
    B_w_up: jax.Array,
    B_w_down: jax.Array,
):
    del B_x
    xt = A_x.reshape(S, D).T
    wdt = B_w_down.T
    beta = A_beta.reshape(1, H)
    wr = B_w_r.reshape(1, D)
    hbm = pl.BlockSpec(memory_space=pltpu.HBM)
    vm = pl.BlockSpec(memory_space=pltpu.VMEM)
    V = pltpu.VMEM
    scratch = [
        V((NTILE, D, 128), bf16),
        V((D, D), bf16), V((D, D), bf16), V((D, D), bf16), V((D, D), bf16),
        V((D, F), bf16), V((D, F), bf16), V((D, F), bf16),
        V((3 * DC // 2, DP), u32),
        V((D // 2, DP), u32),
        V((DP // 2, L), u32),
        V((NG, L // 2, 128), u32),
        V((NG, 64, L), u32),
        V((NG, 64, L), u32),
        V((NG, 64, L), u32),
        V((NG, 64, L), u32),
        V((NG, 128, L), f32),
        V((640, 128), u32), V((640, 128), u32),
        V((1280, 128), f32), V((1280, 128), f32),
        V((32, 128), f32), V((32, 128), f32),
        V((NG, 128, 128), f32),
        V((NG, 128, 128), u32),
        V((NTILE, D, 128), bf16), V((NTILE, D, 128), bf16), V((NTILE, D, 128), bf16),
        V((7, 64, 128), u32),
        V((H, 32, 128), f32),
        V((NG, 128, 128), f32),
        V((D, 128), f32),
        V((2, 8, 128), f32),
        pltpu.SemaphoreType.DMA((16,)),
    ]
    out_t = pl.pallas_call(
        _kernel,
        out_shape=jax.ShapeDtypeStruct((D, S), bf16),
        in_specs=[hbm, hbm, hbm, hbm, hbm, vm, vm, hbm, hbm, hbm],
        out_specs=hbm,
        scratch_shapes=scratch,
        compiler_params=pltpu.CompilerParams(vmem_limit_bytes=100 * 1024 * 1024),
    )(xt, A_wq, A_wk, A_wv, A_wo, beta, wr, B_w_gate, B_w_up, wdt)
    return out_t.T.reshape(1, S, D)
```

```python
import jax
import jax.numpy as jnp
from jax import lax
import jax.experimental.pallas as pl
import jax.experimental.pallas.tpu as pltpu

u32 = jnp.uint32
f32 = jnp.float32
bf16 = jnp.bfloat16
i32 = jnp.int32

S = 2048
D = 576
DP = 640
DC = 592
F = 4608
NSEG = 4
L = 512
NTILE = S // 128
H = 32
DH = 18
NG = 5
OFF = (0, 128, 384, 768)
LOG2E = 1.4426950408889634
QSCALE = float(DH ** (-0.5)) * LOG2E
EPS = 1e-05
BOUND = 30.0
VBOUND = 1e20
NT = (((1,), (1,)), ((), ()))
UN_FAST = 8
UN_SLOW = 2
POST_AT = 0
GCH = 5
PCH = 64


def _unpack(x):
    return pltpu.bitcast(x, bf16)


def _pack(x):
    return pltpu.bitcast(x, u32)


def _iota(shape, dim):
    return lax.broadcasted_iota(i32, shape, dim)


def _perm_rows(w, tail):
    c = w.shape[1]
    parts = []
    for g in range(NG):
        if g < NG - 1:
            parts += [w[63 * g:63 * g + 63], jnp.zeros((1, c), u32)]
        else:
            parts += [w[252:288], jnp.zeros((tail - 36, c), u32)]
    return jnp.concatenate(parts, axis=0)


def _pad_lanes(x):
    return jnp.concatenate([x, jnp.zeros((x.shape[0], DP - D), x.dtype)], axis=1)


def _layernorm_t(xf):
    m = jnp.sum(xf, axis=0, keepdims=True) * (1.0 / D)
    xc = xf - m
    v = jnp.sum(xc * xc, axis=0, keepdims=True) * (1.0 / D)
    return xc * lax.rsqrt(v + EPS)


def _phi(t):
    return jnp.where(t > 0, t + 1.0, jnp.exp2(t * LOG2E))


def _sigmoid(t):
    return 1.0 / (1.0 + jnp.exp(-t))


def _absmax(x):
    return jnp.max(jnp.max(jnp.abs(x), axis=0, keepdims=True), axis=1, keepdims=True)


def _kernel(x_hbm, wq_hbm, wk_hbm, wv_hbm, wo_hbm, beta_ref, wr_ref, wg_hbm, wu_hbm, wd_hbm,
            out_hbm,
            x_v, wq_v, wk_v, wv_v, wo_v, wg_v, wu_v, wd_v,
            wall, wot, xn, kp, phk, qt, phq, vt, ot, pb0, pb1, sb0, sb1, mb0, mb1,
            mt, mlhs, hbuf, st, mxs, h_v, hn_v, out_v, msk, omg, grow, wcol, best, sems):

    def cp(src, dst, i):
        return pltpu.make_async_copy(src, dst, sems.at[i])

    x_cp = [cp(x_hbm.at[:, pl.ds(128 * t, 128)], x_v.at[t], t // 4) for t in range(NTILE)]
    wq_cp, wk_cp, wv_cp, wo_cp = (cp(wq_hbm, wq_v, 4), cp(wk_hbm, wk_v, 5),
                                  cp(wv_hbm, wv_v, 6), cp(wo_hbm, wo_v, 7))
    wg_cp, wu_cp, wd_cp = cp(wg_hbm, wg_v, 8), cp(wu_hbm, wu_v, 9), cp(wd_hbm, wd_v, 10)
    o_cp = [cp(out_v.at[t], out_hbm.at[:, pl.ds(128 * t, 128)], 11 + t // 4) for t in range(NTILE)]

    wq_cp.start()
    for t in range(4):
        x_cp[t].start()
    wk_cp.start()
    wv_cp.start()
    wo_cp.start()
    for t in range(4, NTILE):
        x_cp[t].start()
    wg_cp.start()
    wu_cp.start()
    wd_cp.start()

    r64 = _iota((64, 128), 0)
    for j in range(7):
        msk[j] = jnp.where((r64 >= 9 * j) & (r64 < 9 * j + 9), u32(0xFFFFFFFF), u32(0))
    g_lane = _sigmoid(beta_ref[...].astype(f32))
    g_lane = jnp.concatenate([g_lane, jnp.zeros((1, 128 - H), f32)], axis=1)
    lane128 = _iota((128, 128), 1)
    row128 = _iota((128, 128), 0)
    head_in_group = lax.shift_right_logical(row128 * 57, 10)
    for g in range(NG):
        hid = jnp.where(head_in_group < 7, head_in_group + 7 * g, 999)
        sel = jnp.where(lane128 == hid, jnp.broadcast_to(g_lane, (128, 128)), 0.0)
        grow[g] = jnp.broadcast_to(jnp.sum(sel, axis=1, keepdims=True), (128, 128))
    r32 = _iota((32, 128), 0)
    for h in range(H):
        j = h % 7
        off = 18 * j - 16 * ((9 * j) // 8)
        gh = jnp.broadcast_to(g_lane[:, h:h + 1], (32, 128))
        omg[h] = jnp.where((r32 >= off) & (r32 < off + 18), 1.0 - gh, 0.0)
    head_col = lax.shift_right_logical(lane128 * 57, 10)
    bd_mask = (head_in_group == head_col) & (head_in_group < 7)
    wr = _pad_lanes(wr_ref[...].astype(f32))
    wcol[...] = jnp.broadcast_to(wr, (128, DP)).T[0:D]
    xn[288:320, :] = jnp.zeros((32, L), u32)
    best[0] = jnp.full((8, 128), -jnp.inf, f32)
    best[1] = jnp.zeros((8, 128), f32)
    mt[...] = jnp.zeros((NG, 128, 128), f32)
    hbuf[...] = jnp.zeros((4, D, 128), bf16)
    st[...] = jnp.zeros((4, 8, 128), f32)
    for ref in (qt, phq, phk, vt):
        ref[NG - 1, 40:64] = jnp.zeros((24, L), u32)

    def prep_t(w_ref):
        wt = _pack(w_ref[...].T)
        return _pad_lanes(_perm_rows(wt, 40))

    wq_cp.wait()
    wall[0:296, :] = prep_t(wq_v)
    wk_cp.wait()
    wall[296:592, :] = prep_t(wk_v)
    wv_cp.wait()
    wall[592:888, :] = prep_t(wv_v)
    wo_cp.wait()
    wot[...] = _pack(_unpack(_perm_rows(_pack(wo_v[...]), 64)).T)

    diag = _iota((128, 128), 0) <= _iota((128, 128), 1)

    def qk_logits(h, i):
        g, j = h // 7, h % 7
        n = 128 * (i + 1)
        qw = qt[g, :, 128 * i:128 * (i + 1)] & msk[j]
        s = jnp.dot(_unpack(kp[g, 0:n // 2, :]), _unpack(qw), preferred_element_type=f32)
        sl = jnp.where(diag, s[n - 128:], -1e30)
        return sl if i == 0 else jnp.concatenate([s[:n - 128], sl], axis=0)

    def pv(h, i, pb):
        g, j = h // 7, h % 7
        n = 128 * (i + 1)
        a8 = pl.multiple_of(((9 * j) // 8) * 8, 8)
        vw = vt[g, pl.ds(a8, 16), 0:n]
        mk = msk[j, pl.ds(a8, 16), :]
        mk = jnp.concatenate([mk] * (i + 1), axis=1)
        vw = (vw & mk) | (jnp.full((16, n), 0x3F803F80, u32) & ~mk)
        o = jnp.dot(_unpack(vw), pb, preferred_element_type=f32)
        og = omg[h]
        r32_ = _iota((32, 128), 0)
        off = 18 * j - 2 * a8
        is_head = (r32_ >= off) & (r32_ < off + 18)
        lsum = jnp.sum(jnp.where(is_head, 0.0, o), axis=0, keepdims=True)
        r = pl.reciprocal(lsum, approx=True) * 14.0
        w16 = pl.multiple_of(a8 * 2, 16)
        ot[g, pl.ds(w16, 32), 128 * i:128 * (i + 1)] += o * (r * og)

    pbs = (pb0, pb1)
    sbs = (sb0, sb1)
    mbs = (mb0, mb1)
    IORD = (3, 2, 1, 0)

    def fast_qk(h, i, pbuf):
        n = 128 * (i + 1)
        p = jnp.exp2(qk_logits(h, i)).astype(bf16)
        pbuf[OFF[i] // 2:(OFF[i] + n) // 2, :] = _pack(p)

    def fast_pv(h, i, pbuf):
        n = 128 * (i + 1)
        pv(h, i, _unpack(pbuf[OFF[i] // 2:(OFF[i] + n) // 2, :]))

    def slow_qk(h, i, sbuf, mbuf):
        n = 128 * (i + 1)
        s = qk_logits(h, i)
        sbuf[OFF[i]:OFF[i] + n, :] = s
        mbuf[8 * i:8 * i + 8, :] = jnp.broadcast_to(jnp.max(s, axis=0, keepdims=True), (8, 128))

    def slow_pv(h, i, sbuf, mbuf):
        n = 128 * (i + 1)
        s = sbuf[OFF[i]:OFF[i] + n, :]
        p = jnp.exp2(s - mbuf[8 * i:8 * i + 1, :]).astype(bf16)
        pv(h, i, p)

    def attention_fast():
        def heads(h0, last):
            for u in range(UN_FAST):
                h = h0 + u
                if not (last and u == UN_FAST - 1):
                    for i in IORD:
                        fast_qk(h + 1, i, pbs[1 - u % 2])
                for i in IORD:
                    fast_pv(h, i, pbs[u % 2])

        for i in IORD:
            fast_qk(0, i, pbs[0])

        def body(it, c):
            heads(it * UN_FAST, False)
            return c
        lax.fori_loop(0, H // UN_FAST - 1, body, 0)
        heads(H - UN_FAST, True)

    def attention_slow():
        for i in IORD:
            slow_qk(0, i, sbs[0], mbs[0])

        def body(it, c):
            for u in range(UN_SLOW):
                h = it * UN_SLOW + u
                hn_ = jnp.minimum(h + 1, H - 1)
                for i in IORD:
                    slow_qk(hn_, i, sbs[1 - u % 2], mbs[1 - u % 2])
                for i in IORD:
                    slow_pv(h, i, sbs[u % 2], mbs[u % 2])
            return c
        lax.fori_loop(0, H // UN_SLOW, body, 0)

    def wait_x(seg):
        for t in range(NSEG):
            @pl.when(seg == t)
            def _():
                for u in range(4):
                    x_cp[4 * t + u].wait()

    def layer_norm_tile(seg, t):
        xf = x_v[4 * seg + t].astype(f32)
        xn[0:288, 128 * t:128 * (t + 1)] = _pack(_layernorm_t(xf).astype(bf16))

    def post_tile(seg, t, valid):
        bv = best[0]
        bi = best[1]
        lane = _iota((8, 128), 1).astype(f32)
        m = st[t, 0:1, :]
        rs = st[t, 1:2, :]
        rr = None
        for ch in range(D // PCH):
            rsl = slice(PCH * ch, PCH * (ch + 1))
            hf = hbuf[t, rsl].astype(f32)
            hnb = ((hf - m) * rs).astype(bf16)
            hnf = hnb.astype(f32)
            hn_v[4 * seg + t, rsl] = hnb
            out_v[4 * seg + t, rsl] = (hf + hnf).astype(bf16)
            r_ = jnp.sum((hnf * wcol[rsl]).reshape(PCH // 8, 8, 128), axis=0)
            rr = r_ if rr is None else rr + r_
        rr = jnp.sum(rr, axis=0, keepdims=True).astype(bf16).astype(f32)
        rt = jnp.broadcast_to(rr, (8, 128))
        upd_ = rt > bv
        if valid is not None:
            upd_ = jnp.logical_and(upd_, valid)
        best[0] = jnp.where(upd_, rt, bv)
        best[1] = jnp.where(upd_, lane + jnp.asarray(seg * L + 128 * t, i32).astype(f32), bi)

    def start_out(seg):
        for t in range(NSEG):
            @pl.when(seg == t)
            def _():
                for u in range(4):
                    o_cp[4 * t + u].start()

    def segment(s, c):
        sp = jnp.maximum(s - 1, 0)
        mx = [None, None, None]
        for t in range(4):
            cs = slice(128 * t, 128 * (t + 1))
            xt_ = _unpack(xn[:, cs])
            for w in range(3):
                m_ = None
                res = None
                for g in range(NG):
                    nr = 128 if g < NG - 1 else 80
                    if g % GCH == 0:
                        r0_ = DC * w + 128 * g
                        r1_ = min(r0_ + 128 * GCH, DC * (w + 1))
                        res = jnp.dot(_unpack(wall[r0_ // 2:r1_ // 2, :]), xt_,
                                      preferred_element_type=f32)
                    a = res[128 * (g % GCH):128 * (g % GCH) + nr]
                    if w == 0:
                        phq[g, 0:nr // 2, cs] = _pack(_phi(a).astype(bf16))
                        a = a * QSCALE
                        qt[g, 0:nr // 2, cs] = _pack(a.astype(bf16))
                    elif w == 1:
                        phk[g, 0:nr // 2, cs] = _pack(_phi(a).astype(bf16))
                        ab = a.astype(bf16)
                        if nr < 128:
                            ab = jnp.concatenate([ab, jnp.zeros((128 - nr, 128), bf16)], axis=0)
                        kp[g, 64 * t:64 * (t + 1), :] = _pack(ab.T)
                    else:
                        vt[g, 0:nr // 2, cs] = _pack(a.astype(bf16))
                    am = jnp.max(jnp.abs(a).reshape(nr // 8, 8, 128), axis=0)
                    m_ = am if m_ is None else jnp.maximum(m_, am)
                mx[w] = m_ if mx[w] is None else jnp.maximum(mx[w], m_)
                if w == POST_AT:
                    post_tile(sp, t, s > 0)
        for w in range(3):
            mxs[w] = mx[w]

        @pl.when(s > 0)
        def _():
            start_out(s - 1)

        @pl.when(s == 0)
        def _():
            ot[...] = jnp.zeros((NG, 128, L), f32)

        @pl.when(s > 0)
        def _():
            for g in range(NG):
                nd = jnp.dot(_unpack(mlhs[g]), _unpack(phq[g]), preferred_element_type=f32)
                num = nd[0:128]
                den = nd[128:256] + 1e-06
                gr = grow[g]
                ot[g] = num * (pl.reciprocal(den, approx=True) * jnp.concatenate([gr] * 4, axis=1))

        mxv = [_absmax(mxs[w]) for w in range(3)]
        bound = mxv[0] * mxv[1] * (DH * 1.02)
        ok = jnp.where((bound <= BOUND) & (mxv[2] <= VBOUND), 1, 0).astype(i32)
        safe = jnp.max(ok) > 0

        @pl.when(safe)
        def _():
            attention_fast()

        @pl.when(jnp.logical_not(safe))
        def _():
            attention_slow()

        @pl.when(s < NSEG - 1)
        def _():
            r64_ = _iota((64, L), 0)
            ones = jnp.full((64, L), 0x3F803F80, u32)
            for g in range(NG):
                lhs = jnp.where(r64_ == 63, ones, vt[g])
                upd = lax.dot_general(_unpack(lhs), _unpack(phk[g]), NT,
                                      preferred_element_type=f32)
                cur = mt[g] + upd
                mt[g] = cur
                m_bd = jnp.where(bd_mask, cur, 0.0)
                z_bd = jnp.where(bd_mask, jnp.broadcast_to(cur[126:127, :], (128, 128)), 0.0)
                mlhs[g] = _pack(jnp.concatenate([m_bd, z_bd], axis=0).astype(bf16))
            wait_x(s + 1)

        sn = jnp.minimum(s + 1, NSEG - 1)
        for t in range(4):
            cs = slice(128 * t, 128 * (t + 1))
            ob = jnp.concatenate([ot[g, :, cs] for g in range(NG)], axis=0).astype(bf16)
            ao = jnp.dot(_unpack(wot[...]), ob, preferred_element_type=f32)
            piv = s1 = s2 = None
            for ch in range(D // PCH):
                rsl = slice(PCH * ch, PCH * (ch + 1))
                hb = (x_v[4 * s + t, rsl].astype(f32) + ao[rsl]).astype(bf16)
                hbuf[t, rsl] = hb
                h_v[4 * s + t, rsl] = hb
                hf = hb.astype(f32)
                if piv is None:
                    piv = hf[0:1, :]
                dd = hf - piv
                a1 = jnp.sum(dd.reshape(PCH // 8, 8, 128), axis=0)
                a2 = jnp.sum((dd * dd).reshape(PCH // 8, 8, 128), axis=0)
                s1 = a1 if s1 is None else s1 + a1
                s2 = a2 if s2 is None else s2 + a2
            e1 = jnp.sum(s1, axis=0, keepdims=True) * (1.0 / D)
            e2 = jnp.sum(s2, axis=0, keepdims=True) * (1.0 / D)
            var = jnp.maximum(e2 - e1 * e1, 0.0)
            st[t, 0:1, :] = piv + e1
            st[t, 1:2, :] = lax.rsqrt(var + EPS)
            layer_norm_tile(sn, t)
        return c

    for u in range(4):
        x_cp[u].wait()
    for t in range(4):
        layer_norm_tile(0, t)
    lax.fori_loop(0, NSEG, segment, 0)
    for t in range(4):
        post_tile(NSEG - 1, t, None)
    for u in range(4):
        o_cp[4 * (NSEG - 1) + u].start()

    bv = best[0]
    bi = best[1]
    vmax = jnp.max(bv, axis=1, keepdims=True)
    cand = jnp.where(bv == vmax, bi, float(S))
    imin = jnp.min(cand, axis=1, keepdims=True)
    idx = jnp.minimum(jnp.max(imin).astype(i32), S - 1)
    tile = idx // 128
    col = idx - tile * 128
    col16 = pl.multiple_of((col // 16) * 16, 16)
    hn_t = hn_v[tile]
    lane_sel = _iota((D, 128), 1) == col
    xs_t = jnp.where(lane_sel, hn_t, jnp.zeros_like(hn_t))
    xs_t = jnp.concatenate([xs_t, jnp.zeros((DP - D, 128), bf16)], axis=0)
    pb0[0:64, :] = jnp.zeros((64, 128), u32)
    xall = xs_t.T
    xn[0:64, 0:L] = _pack(xall[:, 0:L])
    pb0[0:64, :] = _pack(xall[:, L:DP])
    c8 = pl.multiple_of(col16 // 2, 8)
    xs = _unpack(jnp.concatenate([xn[pl.ds(c8, 8), 0:L], pb0[pl.ds(c8, 8), 0:64]], axis=1))
    wg_cp.wait()
    wu_cp.wait()
    gt = jnp.dot(xs, wg_v[...], preferred_element_type=f32)
    up = jnp.dot(xs, wu_v[...], preferred_element_type=f32)
    act = (gt * _sigmoid(gt) * up).astype(bf16)
    wd_cp.wait()
    y = lax.dot_general(act, wd_v[...], NT, preferred_element_type=f32)
    rsel = _sigmoid(vmax[0:1, 0:1])
    yb = (y * rsel).astype(bf16)
    y128 = jnp.concatenate([_pad_lanes(yb), jnp.zeros((112, DP), bf16)], axis=0)
    yt = y128.T[0:D].astype(f32)
    ycol = jnp.sum(jnp.where(_iota((D, 128), 1) == (col - col16), yt, 0.0), axis=1, keepdims=True)
    fin = (h_v[tile].astype(f32)
           + (hn_t.astype(f32) + jnp.where(lane_sel, ycol, 0.0))).astype(bf16)
    for t in range(NTILE):
        o_cp[t].wait()
    out_v[tile] = fin
    pc = cp(out_v.at[tile], out_hbm.at[:, pl.ds(pl.multiple_of(tile * 128, 128), 128)], 15)
    pc.start()
    pc.wait()


@jax.jit
def pallas_sequential_preLN__memory_aug_infini_attn__moe_arch_mod__prompt_kernel(
    A_x: jax.Array,
    A_wq: jax.Array,
    A_wk: jax.Array,
    A_wv: jax.Array,
    A_wo: jax.Array,
    A_beta: jax.Array,
    B_x: jax.Array,
    B_w_r: jax.Array,
    B_w_gate: jax.Array,
    B_w_up: jax.Array,
    B_w_down: jax.Array,
):
    del B_x
    xt = A_x.reshape(S, D).T
    wdt = B_w_down.T
    beta = A_beta.reshape(1, H)
    wr = B_w_r.reshape(1, D)
    hbm = pl.BlockSpec(memory_space=pltpu.HBM)
    vm = pl.BlockSpec(memory_space=pltpu.VMEM)
    V = pltpu.VMEM
    scratch = [
        V((NTILE, D, 128), bf16),
        V((D, D), bf16), V((D, D), bf16), V((D, D), bf16), V((D, D), bf16),
        V((D, F), bf16), V((D, F), bf16), V((D, F), bf16),
        V((3 * DC // 2, DP), u32),
        V((D // 2, DP), u32),
        V((DP // 2, L), u32),
        V((NG, L // 2, 128), u32),
        V((NG, 64, L), u32),
        V((NG, 64, L), u32),
        V((NG, 64, L), u32),
        V((NG, 64, L), u32),
        V((NG, 128, L), f32),
        V((640, 128), u32), V((640, 128), u32),
        V((1280, 128), f32), V((1280, 128), f32),
        V((32, 128), f32), V((32, 128), f32),
        V((NG, 128, 128), f32),
        V((NG, 128, 128), u32),
        V((4, D, 128), bf16),
        V((4, 8, 128), f32),
        V((3, 8, 128), f32),
        V((NTILE, D, 128), bf16), V((NTILE, D, 128), bf16), V((NTILE, D, 128), bf16),
        V((7, 64, 128), u32),
        V((H, 32, 128), f32),
        V((NG, 128, 128), f32),
        V((D, 128), f32),
        V((2, 8, 128), f32),
        pltpu.SemaphoreType.DMA((16,)),
    ]
    out_t = pl.pallas_call(
        _kernel,
        out_shape=jax.ShapeDtypeStruct((D, S), bf16),
        in_specs=[hbm, hbm, hbm, hbm, hbm, vm, vm, hbm, hbm, hbm],
        out_specs=hbm,
        scratch_shapes=scratch,
        compiler_params=pltpu.CompilerParams(vmem_limit_bytes=100 * 1024 * 1024),
    )(xt, A_wq, A_wk, A_wv, A_wo, beta, wr, B_w_gate, B_w_up, wdt)
    return out_t.T.reshape(1, S, D)
```

```python
import jax
import jax.numpy as jnp
from jax import lax
import jax.experimental.pallas as pl
import jax.experimental.pallas.tpu as pltpu

u32 = jnp.uint32
f32 = jnp.float32
bf16 = jnp.bfloat16
i32 = jnp.int32

S = 2048
D = 576
DP = 640
DC = 592
F = 4608
NSEG = 4
L = 512
NTILE = S // 128
H = 32
DH = 18
NG = 5
OFF = (0, 128, 384, 768)
LOG2E = 1.4426950408889634
QSCALE = float(DH ** (-0.5)) * LOG2E
EPS = 1e-05
BOUND = 30.0
VBOUND = 1e20
NT = (((1,), (1,)), ((), ()))
UN_FAST = 8
UN_SLOW = 2
POST_AT = 0
GCH = 1
DEP = True
PSTART = 0
PPS = 1
PCH = 64


def _unpack(x):
    return pltpu.bitcast(x, bf16)


def _pack(x):
    return pltpu.bitcast(x, u32)


def _iota(shape, dim):
    return lax.broadcasted_iota(i32, shape, dim)


def _perm_rows(w, tail):
    c = w.shape[1]
    parts = []
    for g in range(NG):
        if g < NG - 1:
            parts += [w[63 * g:63 * g + 63], jnp.zeros((1, c), u32)]
        else:
            parts += [w[252:288], jnp.zeros((tail - 36, c), u32)]
    return jnp.concatenate(parts, axis=0)


def _pad_lanes(x):
    return jnp.concatenate([x, jnp.zeros((x.shape[0], DP - D), x.dtype)], axis=1)


def _layernorm_t(xf):
    m = jnp.sum(xf, axis=0, keepdims=True) * (1.0 / D)
    xc = xf - m
    v = jnp.sum(xc * xc, axis=0, keepdims=True) * (1.0 / D)
    return xc * lax.rsqrt(v + EPS)


def _phi(t):
    return jnp.where(t > 0, t + 1.0, jnp.exp2(t * LOG2E))


def _sigmoid(t):
    return 1.0 / (1.0 + jnp.exp(-t))


def _absmax(x):
    return jnp.max(jnp.max(jnp.abs(x), axis=0, keepdims=True), axis=1, keepdims=True)


def _kernel(x_hbm, wq_hbm, wk_hbm, wv_hbm, wo_hbm, beta_ref, wr_ref, wg_hbm, wu_hbm, wd_hbm,
            out_hbm,
            x_v, wq_v, wk_v, wv_v, wo_v, wg_v, wu_v, wd_v,
            wall, wot, xn, kp, phk, qt, phq, vt, ot, pb0, pb1, sb0, sb1, mb0, mb1,
            mt, mlhs, hbuf, st, mxs, racc, h_v, hn_v, out_v, msk, omg, grow, wcol, best, sems):

    def cp(src, dst, i):
        return pltpu.make_async_copy(src, dst, sems.at[i])

    x_cp = [cp(x_hbm.at[:, pl.ds(128 * t, 128)], x_v.at[t], t // 4) for t in range(NTILE)]
    wq_cp, wk_cp, wv_cp, wo_cp = (cp(wq_hbm, wq_v, 4), cp(wk_hbm, wk_v, 5),
                                  cp(wv_hbm, wv_v, 6), cp(wo_hbm, wo_v, 7))
    wg_cp, wu_cp, wd_cp = cp(wg_hbm, wg_v, 8), cp(wu_hbm, wu_v, 9), cp(wd_hbm, wd_v, 10)
    o_cp = [cp(out_v.at[t], out_hbm.at[:, pl.ds(128 * t, 128)], 11 + t // 4) for t in range(NTILE)]

    wq_cp.start()
    for t in range(4):
        x_cp[t].start()
    wk_cp.start()
    wv_cp.start()
    wo_cp.start()
    for t in range(4, NTILE):
        x_cp[t].start()
    wg_cp.start()
    wu_cp.start()
    wd_cp.start()

    r64 = _iota((64, 128), 0)
    for j in range(7):
        msk[j] = jnp.where((r64 >= 9 * j) & (r64 < 9 * j + 9), u32(0xFFFFFFFF), u32(0))
    g_lane = _sigmoid(beta_ref[...].astype(f32))
    g_lane = jnp.concatenate([g_lane, jnp.zeros((1, 128 - H), f32)], axis=1)
    lane128 = _iota((128, 128), 1)
    row128 = _iota((128, 128), 0)
    head_in_group = lax.shift_right_logical(row128 * 57, 10)
    for g in range(NG):
        hid = jnp.where(head_in_group < 7, head_in_group + 7 * g, 999)
        sel = jnp.where(lane128 == hid, jnp.broadcast_to(g_lane, (128, 128)), 0.0)
        grow[g] = jnp.broadcast_to(jnp.sum(sel, axis=1, keepdims=True), (128, 128))
    r32 = _iota((32, 128), 0)
    for h in range(H):
        j = h % 7
        off = 18 * j - 16 * ((9 * j) // 8)
        gh = jnp.broadcast_to(g_lane[:, h:h + 1], (32, 128))
        omg[h] = jnp.where((r32 >= off) & (r32 < off + 18), 1.0 - gh, 0.0)
    head_col = lax.shift_right_logical(lane128 * 57, 10)
    bd_mask = (head_in_group == head_col) & (head_in_group < 7)
    wr = _pad_lanes(wr_ref[...].astype(f32))
    wcol[...] = jnp.broadcast_to(wr, (128, DP)).T[0:D]
    xn[288:320, :] = jnp.zeros((32, L), u32)
    best[0] = jnp.full((8, 128), -jnp.inf, f32)
    best[1] = jnp.zeros((8, 128), f32)
    mt[...] = jnp.zeros((NG, 128, 128), f32)
    hbuf[...] = jnp.zeros((4, D, 128), bf16)
    st[...] = jnp.zeros((4, 8, 128), f32)
    for ref in (qt, phq, phk, vt):
        ref[NG - 1, 40:64] = jnp.zeros((24, L), u32)

    def prep_t(w_ref):
        wt = _pack(w_ref[...].T)
        return _pad_lanes(_perm_rows(wt, 40))

    wq_cp.wait()
    wall[0:296, :] = prep_t(wq_v)
    wk_cp.wait()
    wall[296:592, :] = prep_t(wk_v)
    wv_cp.wait()
    wall[592:888, :] = prep_t(wv_v)
    wo_cp.wait()
    wot[...] = _pack(_unpack(_perm_rows(_pack(wo_v[...]), 64)).T)

    diag = _iota((128, 128), 0) <= _iota((128, 128), 1)

    def qk_logits(h, i):
        g, j = h // 7, h % 7
        n = 128 * (i + 1)
        qw = qt[g, :, 128 * i:128 * (i + 1)] & msk[j]
        s = jnp.dot(_unpack(kp[g, 0:n // 2, :]), _unpack(qw), preferred_element_type=f32)
        sl = jnp.where(diag, s[n - 128:], -1e30)
        return sl if i == 0 else jnp.concatenate([s[:n - 128], sl], axis=0)

    def pv(h, i, pb):
        g, j = h // 7, h % 7
        n = 128 * (i + 1)
        a8 = pl.multiple_of(((9 * j) // 8) * 8, 8)
        vw = vt[g, pl.ds(a8, 16), 0:n]
        mk = msk[j, pl.ds(a8, 16), :]
        mk = jnp.concatenate([mk] * (i + 1), axis=1)
        vw = (vw & mk) | (jnp.full((16, n), 0x3F803F80, u32) & ~mk)
        o = jnp.dot(_unpack(vw), pb, preferred_element_type=f32)
        og = omg[h]
        r32_ = _iota((32, 128), 0)
        off = 18 * j - 2 * a8
        is_head = (r32_ >= off) & (r32_ < off + 18)
        lsum = jnp.sum(jnp.where(is_head, 0.0, o), axis=0, keepdims=True)
        r = pl.reciprocal(lsum, approx=True) * 14.0
        w16 = pl.multiple_of(a8 * 2, 16)
        ot[g, pl.ds(w16, 32), 128 * i:128 * (i + 1)] += o * (r * og)

    pbs = (pb0, pb1)
    sbs = (sb0, sb1)
    mbs = (mb0, mb1)
    IORD = (3, 2, 1, 0)

    def fast_qk(h, i, pbuf):
        n = 128 * (i + 1)
        p = jnp.exp2(qk_logits(h, i)).astype(bf16)
        pbuf[OFF[i] // 2:(OFF[i] + n) // 2, :] = _pack(p)

    def fast_pv(h, i, pbuf):
        n = 128 * (i + 1)
        pv(h, i, _unpack(pbuf[OFF[i] // 2:(OFF[i] + n) // 2, :]))

    def slow_qk(h, i, sbuf, mbuf):
        n = 128 * (i + 1)
        s = qk_logits(h, i)
        sbuf[OFF[i]:OFF[i] + n, :] = s
        mbuf[8 * i:8 * i + 8, :] = jnp.broadcast_to(jnp.max(s, axis=0, keepdims=True), (8, 128))

    def slow_pv(h, i, sbuf, mbuf):
        n = 128 * (i + 1)
        s = sbuf[OFF[i]:OFF[i] + n, :]
        p = jnp.exp2(s - mbuf[8 * i:8 * i + 1, :]).astype(bf16)
        pv(h, i, p)

    def attention_fast():
        def heads(h0, last):
            for u in range(UN_FAST):
                h = h0 + u
                if not (last and u == UN_FAST - 1):
                    for i in IORD:
                        fast_qk(h + 1, i, pbs[1 - u % 2])
                for i in IORD:
                    fast_pv(h, i, pbs[u % 2])

        for i in IORD:
            fast_qk(0, i, pbs[0])

        def body(it, c):
            heads(it * UN_FAST, False)
            return c
        lax.fori_loop(0, H // UN_FAST - 1, body, 0)
        heads(H - UN_FAST, True)

    def attention_slow():
        for i in IORD:
            slow_qk(0, i, sbs[0], mbs[0])

        def body(it, c):
            for u in range(UN_SLOW):
                h = it * UN_SLOW + u
                hn_ = jnp.minimum(h + 1, H - 1)
                for i in IORD:
                    slow_qk(hn_, i, sbs[1 - u % 2], mbs[1 - u % 2])
                for i in IORD:
                    slow_pv(h, i, sbs[u % 2], mbs[u % 2])
            return c
        lax.fori_loop(0, H // UN_SLOW, body, 0)

    def wait_x(seg):
        for t in range(NSEG):
            @pl.when(seg == t)
            def _():
                for u in range(4):
                    x_cp[4 * t + u].wait()

    def layer_norm_tile(seg, t):
        xf = x_v[4 * seg + t].astype(f32)
        xn[0:288, 128 * t:128 * (t + 1)] = _pack(_layernorm_t(xf).astype(bf16))

    NPC = D // PCH

    def post_piece(seg, t, ch, valid):
        m = st[t, 0:1, :]
        rs = st[t, 1:2, :]
        rsl = slice(PCH * ch, PCH * (ch + 1))
        hf = hbuf[t, rsl].astype(f32)
        hnb = ((hf - m) * rs).astype(bf16)
        hnf = hnb.astype(f32)
        hn_v[4 * seg + t, rsl] = hnb
        ob_ = (hf + hnf).astype(bf16)
        out_v[4 * seg + t, rsl] = ob_
        r_ = jnp.sum((hnf * wcol[rsl]).reshape(PCH // 8, 8, 128), axis=0)
        if ch > 0:
            r_ = r_ + racc[...]
        if ch < NPC - 1:
            racc[...] = r_
        else:
            bv = best[0]
            bi = best[1]
            lane = _iota((8, 128), 1).astype(f32)
            rr = jnp.sum(r_, axis=0, keepdims=True).astype(bf16).astype(f32)
            rt = jnp.broadcast_to(rr, (8, 128))
            upd_ = rt > bv
            if valid is not None:
                upd_ = jnp.logical_and(upd_, valid)
            best[0] = jnp.where(upd_, rt, bv)
            best[1] = jnp.where(upd_, lane + jnp.asarray(seg * L + 128 * t, i32).astype(f32), bi)
        return _pack(ob_[0:16]) | pltpu.bitcast(r_, u32)

    def start_out(seg):
        for t in range(NSEG):
            @pl.when(seg == t)
            def _():
                for u in range(4):
                    o_cp[4 * t + u].start()

    def segment(s, c):
        sp = jnp.maximum(s - 1, 0)
        mx = [None, None, None]
        pieces = [(t, ch) for t in range(4) for ch in range(NPC)]
        zero = jnp.full((8, 128), lax.shift_right_logical(s, 8), i32).astype(u32)
        tok = None
        slot = 0
        for t in range(4):
            cs = slice(128 * t, 128 * (t + 1))
            xt_ = _unpack(xn[:, cs])
            for w in range(3):
                m_ = None
                res = None
                for g in range(NG):
                    nr = 128 if g < NG - 1 else 80
                    if g % GCH == 0:
                        r0_ = DC * w + 128 * g
                        r1_ = min(r0_ + 128 * GCH, DC * (w + 1))
                        lhs = wall[r0_ // 2:r1_ // 2, :]
                        if tok is not None and DEP:
                            head = lhs[0:8, 0:128] | (tok & zero)
                            lhs = jnp.concatenate([
                                jnp.concatenate([head, lhs[0:8, 128:]], axis=1), lhs[8:]], axis=0)
                            tok = None
                        res = jnp.dot(_unpack(lhs), xt_, preferred_element_type=f32)
                        slot += 1
                        if slot > PSTART and pieces:
                            for _ in range(PPS):
                                if pieces:
                                    t_, ch_ = pieces.pop(0)
                                    tk = post_piece(sp, t_, ch_, s > 0)
                                    tok = tk if tok is None else tok | tk
                    a = res[128 * (g % GCH):128 * (g % GCH) + nr]
                    if w == 0:
                        phq[g, 0:nr // 2, cs] = _pack(_phi(a).astype(bf16))
                        a = a * QSCALE
                        qt[g, 0:nr // 2, cs] = _pack(a.astype(bf16))
                    elif w == 1:
                        phk[g, 0:nr // 2, cs] = _pack(_phi(a).astype(bf16))
                        ab = a.astype(bf16)
                        if nr < 128:
                            ab = jnp.concatenate([ab, jnp.zeros((128 - nr, 128), bf16)], axis=0)
                        kp[g, 64 * t:64 * (t + 1), :] = _pack(ab.T)
                    else:
                        vt[g, 0:nr // 2, cs] = _pack(a.astype(bf16))
                    am = jnp.max(jnp.abs(a).reshape(nr // 8, 8, 128), axis=0)
                    m_ = am if m_ is None else jnp.maximum(m_, am)
                mx[w] = m_ if mx[w] is None else jnp.maximum(mx[w], m_)
        assert not pieces
        for w in range(3):
            mxs[w] = mx[w]

        @pl.when(s > 0)
        def _():
            start_out(s - 1)

        @pl.when(s == 0)
        def _():
            ot[...] = jnp.zeros((NG, 128, L), f32)

        @pl.when(s > 0)
        def _():
            for g in range(NG):
                nd = jnp.dot(_unpack(mlhs[g]), _unpack(phq[g]), preferred_element_type=f32)
                num = nd[0:128]
                den = nd[128:256] + 1e-06
                gr = grow[g]
                ot[g] = num * (pl.reciprocal(den, approx=True) * jnp.concatenate([gr] * 4, axis=1))

        mxv = [_absmax(mxs[w]) for w in range(3)]
        bound = mxv[0] * mxv[1] * (DH * 1.02)
        ok = jnp.where((bound <= BOUND) & (mxv[2] <= VBOUND), 1, 0).astype(i32)
        safe = jnp.max(ok) > 0

        @pl.when(safe)
        def _():
            attention_fast()

        @pl.when(jnp.logical_not(safe))
        def _():
            attention_slow()

        @pl.when(s < NSEG - 1)
        def _():
            r64_ = _iota((64, L), 0)
            ones = jnp.full((64, L), 0x3F803F80, u32)
            for g in range(NG):
                lhs = jnp.where(r64_ == 63, ones, vt[g])
                upd = lax.dot_general(_unpack(lhs), _unpack(phk[g]), NT,
                                      preferred_element_type=f32)
                cur = mt[g] + upd
                mt[g] = cur
                m_bd = jnp.where(bd_mask, cur, 0.0)
                z_bd = jnp.where(bd_mask, jnp.broadcast_to(cur[126:127, :], (128, 128)), 0.0)
                mlhs[g] = _pack(jnp.concatenate([m_bd, z_bd], axis=0).astype(bf16))
            wait_x(s + 1)

        sn = jnp.minimum(s + 1, NSEG - 1)
        for t in range(4):
            cs = slice(128 * t, 128 * (t + 1))
            ob = jnp.concatenate([ot[g, :, cs] for g in range(NG)], axis=0).astype(bf16)
            ao = jnp.dot(_unpack(wot[...]), ob, preferred_element_type=f32)
            piv = s1 = s2 = None
            for ch in range(D // PCH):
                rsl = slice(PCH * ch, PCH * (ch + 1))
                hb = (x_v[4 * s + t, rsl].astype(f32) + ao[rsl]).astype(bf16)
                hbuf[t, rsl] = hb
                h_v[4 * s + t, rsl] = hb
                hf = hb.astype(f32)
                if piv is None:
                    piv = hf[0:1, :]
                dd = hf - piv
                a1 = jnp.sum(dd.reshape(PCH // 8, 8, 128), axis=0)
                a2 = jnp.sum((dd * dd).reshape(PCH // 8, 8, 128), axis=0)
                s1 = a1 if s1 is None else s1 + a1
                s2 = a2 if s2 is None else s2 + a2
            e1 = jnp.sum(s1, axis=0, keepdims=True) * (1.0 / D)
            e2 = jnp.sum(s2, axis=0, keepdims=True) * (1.0 / D)
            var = jnp.maximum(e2 - e1 * e1, 0.0)
            st[t, 0:1, :] = piv + e1
            st[t, 1:2, :] = lax.rsqrt(var + EPS)
            layer_norm_tile(sn, t)
        return c

    for u in range(4):
        x_cp[u].wait()
    for t in range(4):
        layer_norm_tile(0, t)
    lax.fori_loop(0, NSEG, segment, 0)
    for t in range(4):
        for ch in range(NPC):
            post_piece(NSEG - 1, t, ch, None)
    for u in range(4):
        o_cp[4 * (NSEG - 1) + u].start()

    bv = best[0]
    bi = best[1]
    vmax = jnp.max(bv, axis=1, keepdims=True)
    cand = jnp.where(bv == vmax, bi, float(S))
    imin = jnp.min(cand, axis=1, keepdims=True)
    idx = jnp.minimum(jnp.max(imin).astype(i32), S - 1)
    tile = idx // 128
    col = idx - tile * 128
    col16 = pl.multiple_of((col // 16) * 16, 16)
    hn_t = hn_v[tile]
    lane_sel = _iota((D, 128), 1) == col
    xs_t = jnp.where(lane_sel, hn_t, jnp.zeros_like(hn_t))
    xs_t = jnp.concatenate([xs_t, jnp.zeros((DP - D, 128), bf16)], axis=0)
    pb0[0:64, :] = jnp.zeros((64, 128), u32)
    xall = xs_t.T
    xn[0:64, 0:L] = _pack(xall[:, 0:L])
    pb0[0:64, :] = _pack(xall[:, L:DP])
    c8 = pl.multiple_of(col16 // 2, 8)
    xs = _unpack(jnp.concatenate([xn[pl.ds(c8, 8), 0:L], pb0[pl.ds(c8, 8), 0:64]], axis=1))
    wg_cp.wait()
    wu_cp.wait()
    gt = jnp.dot(xs, wg_v[...], preferred_element_type=f32)
    up = jnp.dot(xs, wu_v[...], preferred_element_type=f32)
    act = (gt * _sigmoid(gt) * up).astype(bf16)
    wd_cp.wait()
    y = lax.dot_general(act, wd_v[...], NT, preferred_element_type=f32)
    rsel = _sigmoid(vmax[0:1, 0:1])
    yb = (y * rsel).astype(bf16)
    y128 = jnp.concatenate([_pad_lanes(yb), jnp.zeros((112, DP), bf16)], axis=0)
    yt = y128.T[0:D].astype(f32)
    ycol = jnp.sum(jnp.where(_iota((D, 128), 1) == (col - col16), yt, 0.0), axis=1, keepdims=True)
    fin = (h_v[tile].astype(f32)
           + (hn_t.astype(f32) + jnp.where(lane_sel, ycol, 0.0))).astype(bf16)
    for t in range(NTILE):
        o_cp[t].wait()
    out_v[tile] = fin
    pc = cp(out_v.at[tile], out_hbm.at[:, pl.ds(pl.multiple_of(tile * 128, 128), 128)], 15)
    pc.start()
    pc.wait()


@jax.jit
def pallas_sequential_preLN__memory_aug_infini_attn__moe_arch_mod__prompt_kernel(
    A_x: jax.Array,
    A_wq: jax.Array,
    A_wk: jax.Array,
    A_wv: jax.Array,
    A_wo: jax.Array,
    A_beta: jax.Array,
    B_x: jax.Array,
    B_w_r: jax.Array,
    B_w_gate: jax.Array,
    B_w_up: jax.Array,
    B_w_down: jax.Array,
):
    del B_x
    xt = A_x.reshape(S, D).T
    wdt = B_w_down.T
    beta = A_beta.reshape(1, H)
    wr = B_w_r.reshape(1, D)
    hbm = pl.BlockSpec(memory_space=pltpu.HBM)
    vm = pl.BlockSpec(memory_space=pltpu.VMEM)
    V = pltpu.VMEM
    scratch = [
        V((NTILE, D, 128), bf16),
        V((D, D), bf16), V((D, D), bf16), V((D, D), bf16), V((D, D), bf16),
        V((D, F), bf16), V((D, F), bf16), V((D, F), bf16),
        V((3 * DC // 2, DP), u32),
        V((D // 2, DP), u32),
        V((DP // 2, L), u32),
        V((NG, L // 2, 128), u32),
        V((NG, 64, L), u32),
        V((NG, 64, L), u32),
        V((NG, 64, L), u32),
        V((NG, 64, L), u32),
        V((NG, 128, L), f32),
        V((640, 128), u32), V((640, 128), u32),
        V((1280, 128), f32), V((1280, 128), f32),
        V((32, 128), f32), V((32, 128), f32),
        V((NG, 128, 128), f32),
        V((NG, 128, 128), u32),
        V((4, D, 128), bf16),
        V((4, 8, 128), f32),
        V((3, 8, 128), f32),
        V((8, 128), f32),
        V((NTILE, D, 128), bf16), V((NTILE, D, 128), bf16), V((NTILE, D, 128), bf16),
        V((7, 64, 128), u32),
        V((H, 32, 128), f32),
        V((NG, 128, 128), f32),
        V((D, 128), f32),
        V((2, 8, 128), f32),
        pltpu.SemaphoreType.DMA((16,)),
    ]
    out_t = pl.pallas_call(
        _kernel,
        out_shape=jax.ShapeDtypeStruct((D, S), bf16),
        in_specs=[hbm, hbm, hbm, hbm, hbm, vm, vm, hbm, hbm, hbm],
        out_specs=hbm,
        scratch_shapes=scratch,
        compiler_params=pltpu.CompilerParams(vmem_limit_bytes=100 * 1024 * 1024),
    )(xt, A_wq, A_wk, A_wv, A_wo, beta, wr, B_w_gate, B_w_up, wdt)
    return out_t.T.reshape(1, S, D)
```

```python
import jax
import jax.numpy as jnp
from jax import lax
import jax.experimental.pallas as pl
import jax.experimental.pallas.tpu as pltpu

u32 = jnp.uint32
f32 = jnp.float32
bf16 = jnp.bfloat16
i32 = jnp.int32

S = 2048
D = 576
DP = 640
DC = 592
F = 4608
NSEG = 4
L = 512
NTILE = S // 128
H = 32
DH = 18
NG = 5
OFF = (0, 128, 384, 768)
LOG2E = 1.4426950408889634
QSCALE = float(DH ** (-0.5)) * LOG2E
EPS = 1e-05
BOUND = 30.0
VBOUND = 1e20
NT = (((1,), (1,)), ((), ()))
UN_FAST = 8
UN_SLOW = 2
POST_AT = 0
GCH = 1
DEP = True
PSTART = 0
PPS = 1
PCH = 64


def _unpack(x):
    return pltpu.bitcast(x, bf16)


def _pack(x):
    return pltpu.bitcast(x, u32)


def _iota(shape, dim):
    return lax.broadcasted_iota(i32, shape, dim)


def _perm_rows(w, tail):
    c = w.shape[1]
    parts = []
    for g in range(NG):
        if g < NG - 1:
            parts += [w[63 * g:63 * g + 63], jnp.zeros((1, c), u32)]
        else:
            parts += [w[252:288], jnp.zeros((tail - 36, c), u32)]
    return jnp.concatenate(parts, axis=0)


def _pad_lanes(x):
    return jnp.concatenate([x, jnp.zeros((x.shape[0], DP - D), x.dtype)], axis=1)


def _layernorm_t(xf):
    m = jnp.sum(xf, axis=0, keepdims=True) * (1.0 / D)
    xc = xf - m
    v = jnp.sum(xc * xc, axis=0, keepdims=True) * (1.0 / D)
    return xc * lax.rsqrt(v + EPS)


def _phi(t):
    return jnp.where(t > 0, t + 1.0, jnp.exp2(t * LOG2E))


def _sigmoid(t):
    return 1.0 / (1.0 + jnp.exp(-t))


def _absmax(x):
    return jnp.max(jnp.max(jnp.abs(x), axis=0, keepdims=True), axis=1, keepdims=True)


def _kernel(x_hbm, wq_hbm, wk_hbm, wv_hbm, wo_hbm, beta_ref, wr_ref, wg_hbm, wu_hbm, wd_hbm,
            out_hbm,
            x_v, wq_v, wk_v, wv_v, wo_v, wg_v, wu_v, wd_v,
            wall, wot, xn, kp, phk, qt, phq, vt, ot, pb0, pb1, sb0, sb1, mb0, mb1,
            mt, mlhs, hbuf, st, mxs, racc, h_v, hn_v, out_v, msk, omg, grow, wcol, best, sems):

    def cp(src, dst, i):
        return pltpu.make_async_copy(src, dst, sems.at[i])

    x_cp = [cp(x_hbm.at[:, pl.ds(128 * t, 128)], x_v.at[t], t // 4) for t in range(NTILE)]
    wq_cp, wk_cp, wv_cp, wo_cp = (cp(wq_hbm, wq_v, 4), cp(wk_hbm, wk_v, 5),
                                  cp(wv_hbm, wv_v, 6), cp(wo_hbm, wo_v, 7))
    wg_cp, wu_cp, wd_cp = cp(wg_hbm, wg_v, 8), cp(wu_hbm, wu_v, 9), cp(wd_hbm, wd_v, 10)
    o_cp = [cp(out_v.at[t], out_hbm.at[:, pl.ds(128 * t, 128)], 11 + t // 4) for t in range(NTILE)]

    wq_cp.start()
    for t in range(4):
        x_cp[t].start()
    wk_cp.start()
    wv_cp.start()
    wo_cp.start()
    for t in range(4, NTILE):
        x_cp[t].start()

    r64 = _iota((64, 128), 0)
    for j in range(7):
        msk[j] = jnp.where((r64 >= 9 * j) & (r64 < 9 * j + 9), u32(0xFFFFFFFF), u32(0))
    g_lane = _sigmoid(beta_ref[...].astype(f32))
    g_lane = jnp.concatenate([g_lane, jnp.zeros((1, 128 - H), f32)], axis=1)
    lane128 = _iota((128, 128), 1)
    row128 = _iota((128, 128), 0)
    head_in_group = lax.shift_right_logical(row128 * 57, 10)
    for g in range(NG):
        hid = jnp.where(head_in_group < 7, head_in_group + 7 * g, 999)
        sel = jnp.where(lane128 == hid, jnp.broadcast_to(g_lane, (128, 128)), 0.0)
        grow[g] = jnp.broadcast_to(jnp.sum(sel, axis=1, keepdims=True), (128, 128))
    r32 = _iota((32, 128), 0)
    for h in range(H):
        j = h % 7
        off = 18 * j - 16 * ((9 * j) // 8)
        gh = jnp.broadcast_to(g_lane[:, h:h + 1], (32, 128))
        omg[h] = jnp.where((r32 >= off) & (r32 < off + 18), 1.0 - gh, 0.0)
    head_col = lax.shift_right_logical(lane128 * 57, 10)
    bd_mask = (head_in_group == head_col) & (head_in_group < 7)
    wr = _pad_lanes(wr_ref[...].astype(f32))
    wcol[...] = jnp.broadcast_to(wr, (128, DP)).T[0:D]
    xn[288:320, :] = jnp.zeros((32, L), u32)
    best[0] = jnp.full((8, 128), -jnp.inf, f32)
    best[1] = jnp.zeros((8, 128), f32)
    mt[...] = jnp.zeros((NG, 128, 128), f32)
    hbuf[...] = jnp.zeros((4, D, 128), bf16)
    st[...] = jnp.zeros((4, 8, 128), f32)
    for ref in (qt, phq, phk, vt):
        ref[NG - 1, 40:64] = jnp.zeros((24, L), u32)

    def prep_t(w_ref):
        wt = _pack(w_ref[...].T)
        return _pad_lanes(_perm_rows(wt, 40))

    wq_cp.wait()
    wall[0:296, :] = prep_t(wq_v)
    wk_cp.wait()
    wall[296:592, :] = prep_t(wk_v)
    wv_cp.wait()
    wall[592:888, :] = prep_t(wv_v)
    wo_cp.wait()
    wg_cp.start()
    wu_cp.start()
    wd_cp.start()
    wot[...] = _pack(_unpack(_perm_rows(_pack(wo_v[...]), 64)).T)

    diag = _iota((128, 128), 0) <= _iota((128, 128), 1)

    def qk_logits(h, i):
        g, j = h // 7, h % 7
        n = 128 * (i + 1)
        qw = qt[g, :, 128 * i:128 * (i + 1)] & msk[j]
        s = jnp.dot(_unpack(kp[g, 0:n // 2, :]), _unpack(qw), preferred_element_type=f32)
        sl = jnp.where(diag, s[n - 128:], -1e30)
        return sl if i == 0 else jnp.concatenate([s[:n - 128], sl], axis=0)

    def pv(h, i, pb):
        g, j = h // 7, h % 7
        n = 128 * (i + 1)
        a8 = pl.multiple_of(((9 * j) // 8) * 8, 8)
        vw = vt[g, pl.ds(a8, 16), 0:n]
        mk = msk[j, pl.ds(a8, 16), :]
        mk = jnp.concatenate([mk] * (i + 1), axis=1)
        vw = (vw & mk) | (jnp.full((16, n), 0x3F803F80, u32) & ~mk)
        o = jnp.dot(_unpack(vw), pb, preferred_element_type=f32)
        og = omg[h]
        r32_ = _iota((32, 128), 0)
        off = 18 * j - 2 * a8
        is_head = (r32_ >= off) & (r32_ < off + 18)
        lsum = jnp.sum(jnp.where(is_head, 0.0, o), axis=0, keepdims=True)
        r = pl.reciprocal(lsum, approx=True) * 14.0
        w16 = pl.multiple_of(a8 * 2, 16)
        ot[g, pl.ds(w16, 32), 128 * i:128 * (i + 1)] += o * (r * og)

    pbs = (pb0, pb1)
    sbs = (sb0, sb1)
    mbs = (mb0, mb1)
    IORD = (3, 2, 1, 0)

    def fast_qk(h, i, pbuf):
        g, j = h // 7, h % 7
        a = (9 * j) // 8
        n = 128 * (i + 1)
        qw = qt[g, 8 * a:8 * a + 16, 128 * i:128 * (i + 1)] & msk[j, 8 * a:8 * a + 16, :]
        parts = [jnp.zeros((8 * a, 128), u32)] if a > 0 else []
        parts.append(qw)
        if 48 - 8 * a > 0:
            parts.append(jnp.zeros((48 - 8 * a, 128), u32))
        qm = _unpack(jnp.concatenate(parts, axis=0))
        s = jnp.dot(_unpack(kp[g, 0:n // 2, :]), qm, preferred_element_type=f32)
        sl = jnp.where(diag, s[n - 128:], -1e30)
        s = sl if i == 0 else jnp.concatenate([s[:n - 128], sl], axis=0)
        pbuf[OFF[i] // 2:(OFF[i] + n) // 2, :] = _pack(jnp.exp2(s).astype(bf16))

    def fast_pv(h, i, pbuf):
        g, j = h // 7, h % 7
        a = (9 * j) // 8
        n = 128 * (i + 1)
        pb = _unpack(pbuf[OFF[i] // 2:(OFF[i] + n) // 2, :])
        mk = msk[j, 8 * a:8 * a + 16, :]
        mk = jnp.concatenate([mk] * (i + 1), axis=1)
        vw = (vt[g, 8 * a:8 * a + 16, 0:n] & mk) | (jnp.full((16, n), 0x3F803F80, u32) & ~mk)
        o = jnp.dot(_unpack(vw), pb, preferred_element_type=f32)
        off = 18 * j - 16 * a
        l8 = o[24:32] if off <= 6 else o[0:8]
        r = pl.reciprocal(l8, approx=True)
        for t in range(4):
            if 8 * t + 8 <= off or 8 * t >= off + 18:
                continue
            rs_ = slice(16 * a + 8 * t, 16 * a + 8 * t + 8)
            cs = slice(128 * i, 128 * (i + 1))
            ot[g, rs_, cs] += o[8 * t:8 * t + 8] * (r * omg[h, 8 * t:8 * t + 8, :])

    def slow_qk(h, i, sbuf, mbuf):
        n = 128 * (i + 1)
        s = qk_logits(h, i)
        sbuf[OFF[i]:OFF[i] + n, :] = s
        mbuf[8 * i:8 * i + 8, :] = jnp.broadcast_to(jnp.max(s, axis=0, keepdims=True), (8, 128))

    def slow_pv(h, i, sbuf, mbuf):
        n = 128 * (i + 1)
        s = sbuf[OFF[i]:OFF[i] + n, :]
        p = jnp.exp2(s - mbuf[8 * i:8 * i + 1, :]).astype(bf16)
        pv(h, i, p)

    def attention_fast():
        for i in IORD:
            fast_qk(0, i, pbs[0])
        for h in range(H):
            if h + 1 < H:
                for i in IORD:
                    fast_qk(h + 1, i, pbs[(h + 1) % 2])
            for i in IORD:
                fast_pv(h, i, pbs[h % 2])

    def attention_slow():
        for i in IORD:
            slow_qk(0, i, sbs[0], mbs[0])

        def body(it, c):
            for u in range(UN_SLOW):
                h = it * UN_SLOW + u
                hn_ = jnp.minimum(h + 1, H - 1)
                for i in IORD:
                    slow_qk(hn_, i, sbs[1 - u % 2], mbs[1 - u % 2])
                for i in IORD:
                    slow_pv(h, i, sbs[u % 2], mbs[u % 2])
            return c
        lax.fori_loop(0, H // UN_SLOW, body, 0)

    def wait_x(seg):
        for t in range(NSEG):
            @pl.when(seg == t)
            def _():
                for u in range(4):
                    x_cp[4 * t + u].wait()

    def layer_norm_tile(seg, t):
        xf = x_v[4 * seg + t].astype(f32)
        xn[0:288, 128 * t:128 * (t + 1)] = _pack(_layernorm_t(xf).astype(bf16))

    NPC = D // PCH

    def post_piece(seg, t, ch, valid):
        m = st[t, 0:1, :]
        rs = st[t, 1:2, :]
        rsl = slice(PCH * ch, PCH * (ch + 1))
        hf = hbuf[t, rsl].astype(f32)
        hnb = ((hf - m) * rs).astype(bf16)
        hnf = hnb.astype(f32)
        hn_v[4 * seg + t, rsl] = hnb
        ob_ = (hf + hnf).astype(bf16)
        out_v[4 * seg + t, rsl] = ob_
        r_ = jnp.sum((hnf * wcol[rsl]).reshape(PCH // 8, 8, 128), axis=0)
        if ch > 0:
            r_ = r_ + racc[...]
        if ch < NPC - 1:
            racc[...] = r_
        else:
            bv = best[0]
            bi = best[1]
            lane = _iota((8, 128), 1).astype(f32)
            rr = jnp.sum(r_, axis=0, keepdims=True).astype(bf16).astype(f32)
            rt = jnp.broadcast_to(rr, (8, 128))
            upd_ = rt > bv
            if valid is not None:
                upd_ = jnp.logical_and(upd_, valid)
            best[0] = jnp.where(upd_, rt, bv)
            best[1] = jnp.where(upd_, lane + jnp.asarray(seg * L + 128 * t, i32).astype(f32), bi)
        return _pack(ob_[0:16]) | pltpu.bitcast(r_, u32)

    def start_out(seg):
        for t in range(NSEG):
            @pl.when(seg == t)
            def _():
                for u in range(4):
                    o_cp[4 * t + u].start()

    def segment(s, c):
        sp = jnp.maximum(s - 1, 0)
        mx = [None, None, None]
        pieces = [(t, ch) for t in range(4) for ch in range(NPC)]
        zero = jnp.full((8, 128), lax.shift_right_logical(s, 8), i32).astype(u32)
        tok = None
        slot = 0
        for t in range(4):
            cs = slice(128 * t, 128 * (t + 1))
            xt_ = _unpack(xn[:, cs])
            for w in range(3):
                m_ = None
                res = None
                for g in range(NG):
                    nr = 128 if g < NG - 1 else 80
                    if g % GCH == 0:
                        r0_ = DC * w + 128 * g
                        r1_ = min(r0_ + 128 * GCH, DC * (w + 1))
                        lhs = wall[r0_ // 2:r1_ // 2, :]
                        if tok is not None and DEP:
                            head = lhs[0:8, 0:128] | (tok & zero)
                            lhs = jnp.concatenate([
                                jnp.concatenate([head, lhs[0:8, 128:]], axis=1), lhs[8:]], axis=0)
                            tok = None
                        res = jnp.dot(_unpack(lhs), xt_, preferred_element_type=f32)
                        slot += 1
                        if slot > PSTART and pieces:
                            for _ in range(PPS):
                                if pieces:
                                    t_, ch_ = pieces.pop(0)
                                    tk = post_piece(sp, t_, ch_, s > 0)
                                    tok = tk if tok is None else tok | tk
                    a = res[128 * (g % GCH):128 * (g % GCH) + nr]
                    if w == 0:
                        phq[g, 0:nr // 2, cs] = _pack(_phi(a).astype(bf16))
                        a = a * QSCALE
                        qt[g, 0:nr // 2, cs] = _pack(a.astype(bf16))
                    elif w == 1:
                        phk[g, 0:nr // 2, cs] = _pack(_phi(a).astype(bf16))
                        ab = a.astype(bf16)
                        if nr < 128:
                            ab = jnp.concatenate([ab, jnp.zeros((128 - nr, 128), bf16)], axis=0)
                        kp[g, 64 * t:64 * (t + 1), :] = _pack(ab.T)
                    else:
                        vt[g, 0:nr // 2, cs] = _pack(a.astype(bf16))
                    am = jnp.max(jnp.abs(a).reshape(nr // 8, 8, 128), axis=0)
                    m_ = am if m_ is None else jnp.maximum(m_, am)
                mx[w] = m_ if mx[w] is None else jnp.maximum(mx[w], m_)
        assert not pieces
        for w in range(3):
            mxs[w] = mx[w]

        @pl.when(s > 0)
        def _():
            start_out(s - 1)

        @pl.when(s == 0)
        def _():
            ot[...] = jnp.zeros((NG, 128, L), f32)

        @pl.when(s > 0)
        def _():
            for g in range(NG):
                nd = jnp.dot(_unpack(mlhs[g]), _unpack(phq[g]), preferred_element_type=f32)
                num = nd[0:128]
                den = nd[128:256] + 1e-06
                gr = grow[g]
                ot[g] = num * (pl.reciprocal(den, approx=True) * jnp.concatenate([gr] * 4, axis=1))

        mxv = [_absmax(mxs[w]) for w in range(3)]
        bound = mxv[0] * mxv[1] * (DH * 1.02)
        ok = jnp.where((bound <= BOUND) & (mxv[2] <= VBOUND), 1, 0).astype(i32)
        safe = jnp.max(ok) > 0

        @pl.when(safe)
        def _():
            attention_fast()

        @pl.when(jnp.logical_not(safe))
        def _():
            attention_slow()

        @pl.when(s < NSEG - 1)
        def _():
            r64_ = _iota((64, L), 0)
            ones = jnp.full((64, L), 0x3F803F80, u32)
            for g in range(NG):
                lhs = jnp.where(r64_ == 63, ones, vt[g])
                upd = lax.dot_general(_unpack(lhs), _unpack(phk[g]), NT,
                                      preferred_element_type=f32)
                cur = mt[g] + upd
                mt[g] = cur
                m_bd = jnp.where(bd_mask, cur, 0.0)
                z_bd = jnp.where(bd_mask, jnp.broadcast_to(cur[126:127, :], (128, 128)), 0.0)
                mlhs[g] = _pack(jnp.concatenate([m_bd, z_bd], axis=0).astype(bf16))
            wait_x(s + 1)

        sn = jnp.minimum(s + 1, NSEG - 1)
        for t in range(4):
            cs = slice(128 * t, 128 * (t + 1))
            ob = jnp.concatenate([ot[g, :, cs] for g in range(NG)], axis=0).astype(bf16)
            ao = jnp.dot(_unpack(wot[...]), ob, preferred_element_type=f32)
            piv = s1 = s2 = None
            for ch in range(D // PCH):
                rsl = slice(PCH * ch, PCH * (ch + 1))
                hb = (x_v[4 * s + t, rsl].astype(f32) + ao[rsl]).astype(bf16)
                hbuf[t, rsl] = hb
                h_v[4 * s + t, rsl] = hb
                hf = hb.astype(f32)
                if piv is None:
                    piv = hf[0:1, :]
                dd = hf - piv
                a1 = jnp.sum(dd.reshape(PCH // 8, 8, 128), axis=0)
                a2 = jnp.sum((dd * dd).reshape(PCH // 8, 8, 128), axis=0)
                s1 = a1 if s1 is None else s1 + a1
                s2 = a2 if s2 is None else s2 + a2
            e1 = jnp.sum(s1, axis=0, keepdims=True) * (1.0 / D)
            e2 = jnp.sum(s2, axis=0, keepdims=True) * (1.0 / D)
            var = jnp.maximum(e2 - e1 * e1, 0.0)
            st[t, 0:1, :] = piv + e1
            st[t, 1:2, :] = lax.rsqrt(var + EPS)
            layer_norm_tile(sn, t)
        return c

    for u in range(4):
        x_cp[u].wait()
    for t in range(4):
        layer_norm_tile(0, t)
    lax.fori_loop(0, NSEG, segment, 0)
    for t in range(4):
        for ch in range(NPC):
            post_piece(NSEG - 1, t, ch, None)
    for u in range(4):
        o_cp[4 * (NSEG - 1) + u].start()

    bv = best[0]
    bi = best[1]
    vmax = jnp.max(bv, axis=1, keepdims=True)
    cand = jnp.where(bv == vmax, bi, float(S))
    imin = jnp.min(cand, axis=1, keepdims=True)
    idx = jnp.minimum(jnp.max(imin).astype(i32), S - 1)
    tile = idx // 128
    col = idx - tile * 128
    col16 = pl.multiple_of((col // 16) * 16, 16)
    hn_t = hn_v[tile]
    lane_sel = _iota((D, 128), 1) == col
    xs_t = jnp.where(lane_sel, hn_t, jnp.zeros_like(hn_t))
    xs_t = jnp.concatenate([xs_t, jnp.zeros((DP - D, 128), bf16)], axis=0)
    pb0[0:64, :] = jnp.zeros((64, 128), u32)
    xall = xs_t.T
    xn[0:64, 0:L] = _pack(xall[:, 0:L])
    pb0[0:64, :] = _pack(xall[:, L:DP])
    c8 = pl.multiple_of(col16 // 2, 8)
    xs = _unpack(jnp.concatenate([xn[pl.ds(c8, 8), 0:L], pb0[pl.ds(c8, 8), 0:64]], axis=1))
    wg_cp.wait()
    wu_cp.wait()
    gt = jnp.dot(xs, wg_v[...], preferred_element_type=f32)
    up = jnp.dot(xs, wu_v[...], preferred_element_type=f32)
    act = (gt * _sigmoid(gt) * up).astype(bf16)
    wd_cp.wait()
    y = lax.dot_general(act, wd_v[...], NT, preferred_element_type=f32)
    rsel = _sigmoid(vmax[0:1, 0:1])
    yb = (y * rsel).astype(bf16)
    y128 = jnp.concatenate([_pad_lanes(yb), jnp.zeros((112, DP), bf16)], axis=0)
    yt = y128.T[0:D].astype(f32)
    ycol = jnp.sum(jnp.where(_iota((D, 128), 1) == (col - col16), yt, 0.0), axis=1, keepdims=True)
    fin = (h_v[tile].astype(f32)
           + (hn_t.astype(f32) + jnp.where(lane_sel, ycol, 0.0))).astype(bf16)
    for t in range(NTILE):
        o_cp[t].wait()
    out_v[tile] = fin
    pc = cp(out_v.at[tile], out_hbm.at[:, pl.ds(pl.multiple_of(tile * 128, 128), 128)], 15)
    pc.start()
    pc.wait()


@jax.jit
def pallas_sequential_preLN__memory_aug_infini_attn__moe_arch_mod__prompt_kernel(
    A_x: jax.Array,
    A_wq: jax.Array,
    A_wk: jax.Array,
    A_wv: jax.Array,
    A_wo: jax.Array,
    A_beta: jax.Array,
    B_x: jax.Array,
    B_w_r: jax.Array,
    B_w_gate: jax.Array,
    B_w_up: jax.Array,
    B_w_down: jax.Array,
):
    del B_x
    xt = A_x.reshape(S, D).T
    wdt = B_w_down.T
    beta = A_beta.reshape(1, H)
    wr = B_w_r.reshape(1, D)
    hbm = pl.BlockSpec(memory_space=pltpu.HBM)
    vm = pl.BlockSpec(memory_space=pltpu.VMEM)
    V = pltpu.VMEM
    scratch = [
        V((NTILE, D, 128), bf16),
        V((D, D), bf16), V((D, D), bf16), V((D, D), bf16), V((D, D), bf16),
        V((D, F), bf16), V((D, F), bf16), V((D, F), bf16),
        V((3 * DC // 2, DP), u32),
        V((D // 2, DP), u32),
        V((DP // 2, L), u32),
        V((NG, L // 2, 128), u32),
        V((NG, 64, L), u32),
        V((NG, 64, L), u32),
        V((NG, 64, L), u32),
        V((NG, 64, L), u32),
        V((NG, 128, L), f32),
        V((640, 128), u32), V((640, 128), u32),
        V((1280, 128), f32), V((1280, 128), f32),
        V((32, 128), f32), V((32, 128), f32),
        V((NG, 128, 128), f32),
        V((NG, 128, 128), u32),
        V((4, D, 128), bf16),
        V((4, 8, 128), f32),
        V((3, 8, 128), f32),
        V((8, 128), f32),
        V((NTILE, D, 128), bf16), V((NTILE, D, 128), bf16), V((NTILE, D, 128), bf16),
        V((7, 64, 128), u32),
        V((H, 32, 128), f32),
        V((NG, 128, 128), f32),
        V((D, 128), f32),
        V((2, 8, 128), f32),
        pltpu.SemaphoreType.DMA((16,)),
    ]
    out_t = pl.pallas_call(
        _kernel,
        out_shape=jax.ShapeDtypeStruct((D, S), bf16),
        in_specs=[hbm, hbm, hbm, hbm, hbm, vm, vm, hbm, hbm, hbm],
        out_specs=hbm,
        scratch_shapes=scratch,
        compiler_params=pltpu.CompilerParams(vmem_limit_bytes=100 * 1024 * 1024),
    )(xt, A_wq, A_wk, A_wv, A_wo, beta, wr, B_w_gate, B_w_up, wdt)
    return out_t.T.reshape(1, S, D)
```

```python
import jax
import jax.numpy as jnp
from jax import lax
import jax.experimental.pallas as pl
import jax.experimental.pallas.tpu as pltpu

u32 = jnp.uint32
f32 = jnp.float32
bf16 = jnp.bfloat16
i32 = jnp.int32

S = 2048
D = 576
DP = 640
DC = 592
F = 4608
NSEG = 4
L = 512
NTILE = S // 128
H = 32
DH = 18
NG = 5
OFF = (0, 128, 384, 768)
LOG2E = 1.4426950408889634
QSCALE = float(DH ** (-0.5)) * LOG2E
EPS = 1e-05
BOUND = 30.0
VBOUND = 1e20
NT = (((1,), (1,)), ((), ()))
UN_FAST = 8
UN_SLOW = 2
POST_AT = 0
GCH = 1
DEP = True
PSTART = 0
PPS = 1
PCH = 64


def _unpack(x):
    return pltpu.bitcast(x, bf16)


def _pack(x):
    return pltpu.bitcast(x, u32)


def _iota(shape, dim):
    return lax.broadcasted_iota(i32, shape, dim)


def _perm_rows(w, tail):
    c = w.shape[1]
    parts = []
    for g in range(NG):
        if g < NG - 1:
            parts += [w[63 * g:63 * g + 63], jnp.zeros((1, c), u32)]
        else:
            parts += [w[252:288], jnp.zeros((tail - 36, c), u32)]
    return jnp.concatenate(parts, axis=0)


def _pad_lanes(x):
    return jnp.concatenate([x, jnp.zeros((x.shape[0], DP - D), x.dtype)], axis=1)


def _layernorm_t(xf):
    m = jnp.sum(xf, axis=0, keepdims=True) * (1.0 / D)
    xc = xf - m
    v = jnp.sum(xc * xc, axis=0, keepdims=True) * (1.0 / D)
    return xc * lax.rsqrt(v + EPS)


def _phi(t):
    return jnp.where(t > 0, t + 1.0, jnp.exp2(t * LOG2E))


def _sigmoid(t):
    return 1.0 / (1.0 + jnp.exp(-t))


def _absmax(x):
    return jnp.max(jnp.max(jnp.abs(x), axis=0, keepdims=True), axis=1, keepdims=True)


def _kernel(x_hbm, wq_hbm, wk_hbm, wv_hbm, wo_hbm, beta_hbm, wr_hbm, wg_hbm, wu_hbm, wd_hbm,
            out_hbm,
            x_v, wq_v, wk_v, wv_v, wo_v, wg_v, wu_v, wd_v,
            wall, wot, xn, kp, phk, qt, phq, vt, ot, pb0, pb1, sb0, sb1, mb0, mb1,
            mt, mlhs, hbuf, st, mxs, racc, h_v, hn_v, out_v, msk, omg, grow, wcol, best, beta_ref, wr_ref, sems):

    def cp(src, dst, i):
        return pltpu.make_async_copy(src, dst, sems.at[i])

    x_cp = [cp(x_hbm.at[:, pl.ds(128 * t, 128)], x_v.at[t], t // 4) for t in range(NTILE)]
    wq_cp, wk_cp, wv_cp, wo_cp = (cp(wq_hbm, wq_v, 4), cp(wk_hbm, wk_v, 5),
                                  cp(wv_hbm, wv_v, 6), cp(wo_hbm, wo_v, 7))
    wg_cp, wu_cp, wd_cp = cp(wg_hbm, wg_v, 8), cp(wu_hbm, wu_v, 9), cp(wd_hbm, wd_v, 10)
    o_cp = [cp(out_v.at[t], out_hbm.at[:, pl.ds(128 * t, 128)], 11 + t // 4) for t in range(NTILE)]

    beta_cp = cp(beta_hbm, beta_ref, 16)
    wr_cp = cp(wr_hbm, wr_ref, 17)
    beta_cp.start()
    wr_cp.start()
    for t in range(4):
        x_cp[t].start()
    wq_cp.start()

    r64 = _iota((64, 128), 0)
    for j in range(7):
        msk[j] = jnp.where((r64 >= 9 * j) & (r64 < 9 * j + 9), u32(0xFFFFFFFF), u32(0))
    beta_cp.wait()
    wr_cp.wait()
    g_lane = _sigmoid(beta_ref[...].astype(f32))
    g_lane = jnp.concatenate([g_lane, jnp.zeros((1, 128 - H), f32)], axis=1)
    lane128 = _iota((128, 128), 1)
    row128 = _iota((128, 128), 0)
    head_in_group = lax.shift_right_logical(row128 * 57, 10)
    for g in range(NG):
        hid = jnp.where(head_in_group < 7, head_in_group + 7 * g, 999)
        sel = jnp.where(lane128 == hid, jnp.broadcast_to(g_lane, (128, 128)), 0.0)
        grow[g] = jnp.broadcast_to(jnp.sum(sel, axis=1, keepdims=True), (128, 128))
    r32 = _iota((32, 128), 0)
    for h in range(H):
        j = h % 7
        off = 18 * j - 16 * ((9 * j) // 8)
        gh = jnp.broadcast_to(g_lane[:, h:h + 1], (32, 128))
        omg[h] = jnp.where((r32 >= off) & (r32 < off + 18), 1.0 - gh, 0.0)
    head_col = lax.shift_right_logical(lane128 * 57, 10)
    bd_mask = (head_in_group == head_col) & (head_in_group < 7)
    wr = _pad_lanes(wr_ref[...].astype(f32).reshape(1, D))
    wcol[...] = jnp.broadcast_to(wr, (128, DP)).T[0:D]
    xn[288:320, :] = jnp.zeros((32, L), u32)
    best[0] = jnp.full((8, 128), -jnp.inf, f32)
    best[1] = jnp.zeros((8, 128), f32)
    mt[...] = jnp.zeros((NG, 128, 128), f32)
    hbuf[...] = jnp.zeros((4, D, 128), bf16)
    st[...] = jnp.zeros((4, 8, 128), f32)
    for ref in (qt, phq, phk, vt):
        ref[NG - 1, 40:64] = jnp.zeros((24, L), u32)

    def prep_t(w_ref):
        wt = _pack(w_ref[...].T)
        return _pad_lanes(_perm_rows(wt, 40))

    def layer_norm_tile(seg, t):
        xf = x_v[4 * seg + t].astype(f32)
        xn[0:288, 128 * t:128 * (t + 1)] = _pack(_layernorm_t(xf).astype(bf16))

    wk_cp.start()
    for u in range(4):
        x_cp[u].wait()
    wv_cp.start()
    for t in range(4):
        layer_norm_tile(0, t)
    wq_cp.wait()
    wo_cp.start()
    wall[0:296, :] = prep_t(wq_v)
    wk_cp.wait()
    for t in range(4, NTILE):
        x_cp[t].start()
    wall[296:592, :] = prep_t(wk_v)
    wv_cp.wait()
    wall[592:888, :] = prep_t(wv_v)
    wo_cp.wait()
    wg_cp.start()
    wu_cp.start()
    wd_cp.start()
    wot[...] = _pack(_unpack(_perm_rows(_pack(wo_v[...]), 64)).T)

    diag = _iota((128, 128), 0) <= _iota((128, 128), 1)

    def qk_logits(h, i):
        g, j = h // 7, h % 7
        n = 128 * (i + 1)
        qw = qt[g, :, 128 * i:128 * (i + 1)] & msk[j]
        s = jnp.dot(_unpack(kp[g, 0:n // 2, :]), _unpack(qw), preferred_element_type=f32)
        sl = jnp.where(diag, s[n - 128:], -1e30)
        return sl if i == 0 else jnp.concatenate([s[:n - 128], sl], axis=0)

    def pv(h, i, pb):
        g, j = h // 7, h % 7
        n = 128 * (i + 1)
        a8 = pl.multiple_of(((9 * j) // 8) * 8, 8)
        vw = vt[g, pl.ds(a8, 16), 0:n]
        mk = msk[j, pl.ds(a8, 16), :]
        mk = jnp.concatenate([mk] * (i + 1), axis=1)
        vw = (vw & mk) | (jnp.full((16, n), 0x3F803F80, u32) & ~mk)
        o = jnp.dot(_unpack(vw), pb, preferred_element_type=f32)
        og = omg[h]
        r32_ = _iota((32, 128), 0)
        off = 18 * j - 2 * a8
        is_head = (r32_ >= off) & (r32_ < off + 18)
        lsum = jnp.sum(jnp.where(is_head, 0.0, o), axis=0, keepdims=True)
        r = pl.reciprocal(lsum, approx=True) * 14.0
        w16 = pl.multiple_of(a8 * 2, 16)
        ot[g, pl.ds(w16, 32), 128 * i:128 * (i + 1)] += o * (r * og)

    pbs = (pb0, pb1)
    sbs = (sb0, sb1)
    mbs = (mb0, mb1)
    IORD = (3, 2, 1, 0)

    def fast_qk(h, i, pbuf):
        g, j = h // 7, h % 7
        a = (9 * j) // 8
        n = 128 * (i + 1)
        qw = qt[g, 8 * a:8 * a + 16, 128 * i:128 * (i + 1)] & msk[j, 8 * a:8 * a + 16, :]
        parts = [jnp.zeros((8 * a, 128), u32)] if a > 0 else []
        parts.append(qw)
        if 48 - 8 * a > 0:
            parts.append(jnp.zeros((48 - 8 * a, 128), u32))
        qm = _unpack(jnp.concatenate(parts, axis=0))
        s = jnp.dot(_unpack(kp[g, 0:n // 2, :]), qm, preferred_element_type=f32)
        sl = jnp.where(diag, s[n - 128:], -1e30)
        s = sl if i == 0 else jnp.concatenate([s[:n - 128], sl], axis=0)
        pbuf[OFF[i] // 2:(OFF[i] + n) // 2, :] = _pack(jnp.exp2(s).astype(bf16))

    def fast_pv(h, i, pbuf):
        g, j = h // 7, h % 7
        a = (9 * j) // 8
        n = 128 * (i + 1)
        pb = _unpack(pbuf[OFF[i] // 2:(OFF[i] + n) // 2, :])
        mk = msk[j, 8 * a:8 * a + 16, :]
        mk = jnp.concatenate([mk] * (i + 1), axis=1)
        vw = (vt[g, 8 * a:8 * a + 16, 0:n] & mk) | (jnp.full((16, n), 0x3F803F80, u32) & ~mk)
        o = jnp.dot(_unpack(vw), pb, preferred_element_type=f32)
        off = 18 * j - 16 * a
        l8 = o[24:32] if off <= 6 else o[0:8]
        r = pl.reciprocal(l8, approx=True)
        for t in range(4):
            if 8 * t + 8 <= off or 8 * t >= off + 18:
                continue
            rs_ = slice(16 * a + 8 * t, 16 * a + 8 * t + 8)
            cs = slice(128 * i, 128 * (i + 1))
            ot[g, rs_, cs] += o[8 * t:8 * t + 8] * (r * omg[h, 8 * t:8 * t + 8, :])

    def slow_qk(h, i, sbuf, mbuf):
        n = 128 * (i + 1)
        s = qk_logits(h, i)
        sbuf[OFF[i]:OFF[i] + n, :] = s
        mbuf[8 * i:8 * i + 8, :] = jnp.broadcast_to(jnp.max(s, axis=0, keepdims=True), (8, 128))

    def slow_pv(h, i, sbuf, mbuf):
        n = 128 * (i + 1)
        s = sbuf[OFF[i]:OFF[i] + n, :]
        p = jnp.exp2(s - mbuf[8 * i:8 * i + 1, :]).astype(bf16)
        pv(h, i, p)

    def attention_fast():
        for i in IORD:
            fast_qk(0, i, pbs[0])
        for h in range(H):
            if h + 1 < H:
                for i in IORD:
                    fast_qk(h + 1, i, pbs[(h + 1) % 2])
            for i in IORD:
                fast_pv(h, i, pbs[h % 2])

    def attention_slow():
        for i in IORD:
            slow_qk(0, i, sbs[0], mbs[0])

        def body(it, c):
            for u in range(UN_SLOW):
                h = it * UN_SLOW + u
                hn_ = jnp.minimum(h + 1, H - 1)
                for i in IORD:
                    slow_qk(hn_, i, sbs[1 - u % 2], mbs[1 - u % 2])
                for i in IORD:
                    slow_pv(h, i, sbs[u % 2], mbs[u % 2])
            return c
        lax.fori_loop(0, H // UN_SLOW, body, 0)

    def wait_x(seg):
        for t in range(NSEG):
            @pl.when(seg == t)
            def _():
                for u in range(4):
                    x_cp[4 * t + u].wait()

    NPC = D // PCH

    def post_piece(seg, t, ch, valid):
        m = st[t, 0:1, :]
        rs = st[t, 1:2, :]
        rsl = slice(PCH * ch, PCH * (ch + 1))
        hf = hbuf[t, rsl].astype(f32)
        hnb = ((hf - m) * rs).astype(bf16)
        hnf = hnb.astype(f32)
        hn_v[4 * seg + t, rsl] = hnb
        ob_ = (hf + hnf).astype(bf16)
        out_v[4 * seg + t, rsl] = ob_
        r_ = jnp.sum((hnf * wcol[rsl]).reshape(PCH // 8, 8, 128), axis=0)
        if ch > 0:
            r_ = r_ + racc[...]
        if ch < NPC - 1:
            racc[...] = r_
        else:
            bv = best[0]
            bi = best[1]
            lane = _iota((8, 128), 1).astype(f32)
            rr = jnp.sum(r_, axis=0, keepdims=True).astype(bf16).astype(f32)
            rt = jnp.broadcast_to(rr, (8, 128))
            upd_ = rt > bv
            if valid is not None:
                upd_ = jnp.logical_and(upd_, valid)
            best[0] = jnp.where(upd_, rt, bv)
            best[1] = jnp.where(upd_, lane + jnp.asarray(seg * L + 128 * t, i32).astype(f32), bi)
        return _pack(ob_[0:16]) | pltpu.bitcast(r_, u32)

    def start_out(seg):
        for t in range(NSEG):
            @pl.when(seg == t)
            def _():
                for u in range(4):
                    o_cp[4 * t + u].start()

    def segment(s, c):
        sp = jnp.maximum(s - 1, 0)
        mx = [None, None, None]
        pieces = [(t, ch) for t in range(4) for ch in range(NPC)]
        zero = jnp.full((8, 128), lax.shift_right_logical(s, 8), i32).astype(u32)
        tok = None
        slot = 0
        for t in range(4):
            cs = slice(128 * t, 128 * (t + 1))
            xt_ = _unpack(xn[:, cs])
            for w in range(3):
                m_ = None
                res = None
                for g in range(NG):
                    nr = 128 if g < NG - 1 else 80
                    if g % GCH == 0:
                        r0_ = DC * w + 128 * g
                        r1_ = min(r0_ + 128 * GCH, DC * (w + 1))
                        lhs = wall[r0_ // 2:r1_ // 2, :]
                        if tok is not None and DEP:
                            head = lhs[0:8, 0:128] | (tok & zero)
                            lhs = jnp.concatenate([
                                jnp.concatenate([head, lhs[0:8, 128:]], axis=1), lhs[8:]], axis=0)
                            tok = None
                        res = jnp.dot(_unpack(lhs), xt_, preferred_element_type=f32)
                        slot += 1
                        if slot > PSTART and pieces:
                            for _ in range(PPS):
                                if pieces:
                                    t_, ch_ = pieces.pop(0)
                                    tk = post_piece(sp, t_, ch_, s > 0)
                                    tok = tk if tok is None else tok | tk
                    a = res[128 * (g % GCH):128 * (g % GCH) + nr]
                    if w == 0:
                        phq[g, 0:nr // 2, cs] = _pack(_phi(a).astype(bf16))
                        a = a * QSCALE
                        qt[g, 0:nr // 2, cs] = _pack(a.astype(bf16))
                    elif w == 1:
                        phk[g, 0:nr // 2, cs] = _pack(_phi(a).astype(bf16))
                        ab = a.astype(bf16)
                        if nr < 128:
                            ab = jnp.concatenate([ab, jnp.zeros((128 - nr, 128), bf16)], axis=0)
                        kp[g, 64 * t:64 * (t + 1), :] = _pack(ab.T)
                    else:
                        vt[g, 0:nr // 2, cs] = _pack(a.astype(bf16))
                    am = jnp.max(jnp.abs(a).reshape(nr // 8, 8, 128), axis=0)
                    m_ = am if m_ is None else jnp.maximum(m_, am)
                mx[w] = m_ if mx[w] is None else jnp.maximum(mx[w], m_)
        assert not pieces
        for w in range(3):
            mxs[w] = mx[w]

        @pl.when(s > 0)
        def _():
            start_out(s - 1)

        @pl.when(s == 0)
        def _():
            ot[...] = jnp.zeros((NG, 128, L), f32)

        @pl.when(s > 0)
        def _():
            for g in range(NG):
                nd = jnp.dot(_unpack(mlhs[g]), _unpack(phq[g]), preferred_element_type=f32)
                num = nd[0:128]
                den = nd[128:256] + 1e-06
                gr = grow[g]
                ot[g] = num * (pl.reciprocal(den, approx=True) * jnp.concatenate([gr] * 4, axis=1))

        mxv = [_absmax(mxs[w]) for w in range(3)]
        bound = mxv[0] * mxv[1] * (DH * 1.02)
        ok = jnp.where((bound <= BOUND) & (mxv[2] <= VBOUND), 1, 0).astype(i32)
        safe = jnp.max(ok) > 0

        @pl.when(safe)
        def _():
            attention_fast()

        @pl.when(jnp.logical_not(safe))
        def _():
            attention_slow()

        @pl.when(s < NSEG - 1)
        def _():
            r64_ = _iota((64, L), 0)
            ones = jnp.full((64, L), 0x3F803F80, u32)
            for g in range(NG):
                lhs = jnp.where(r64_ == 63, ones, vt[g])
                upd = lax.dot_general(_unpack(lhs), _unpack(phk[g]), NT,
                                      preferred_element_type=f32)
                cur = mt[g] + upd
                mt[g] = cur
                m_bd = jnp.where(bd_mask, cur, 0.0)
                z_bd = jnp.where(bd_mask, jnp.broadcast_to(cur[126:127, :], (128, 128)), 0.0)
                mlhs[g] = _pack(jnp.concatenate([m_bd, z_bd], axis=0).astype(bf16))
            wait_x(s + 1)

        sn = jnp.minimum(s + 1, NSEG - 1)
        for t in range(4):
            cs = slice(128 * t, 128 * (t + 1))
            ob = jnp.concatenate([ot[g, :, cs] for g in range(NG)], axis=0).astype(bf16)
            ao = jnp.dot(_unpack(wot[...]), ob, preferred_element_type=f32)
            piv = s1 = s2 = None
            for ch in range(D // PCH):
                rsl = slice(PCH * ch, PCH * (ch + 1))
                hb = (x_v[4 * s + t, rsl].astype(f32) + ao[rsl]).astype(bf16)
                hbuf[t, rsl] = hb
                h_v[4 * s + t, rsl] = hb
                hf = hb.astype(f32)
                if piv is None:
                    piv = hf[0:1, :]
                dd = hf - piv
                a1 = jnp.sum(dd.reshape(PCH // 8, 8, 128), axis=0)
                a2 = jnp.sum((dd * dd).reshape(PCH // 8, 8, 128), axis=0)
                s1 = a1 if s1 is None else s1 + a1
                s2 = a2 if s2 is None else s2 + a2
            e1 = jnp.sum(s1, axis=0, keepdims=True) * (1.0 / D)
            e2 = jnp.sum(s2, axis=0, keepdims=True) * (1.0 / D)
            var = jnp.maximum(e2 - e1 * e1, 0.0)
            st[t, 0:1, :] = piv + e1
            st[t, 1:2, :] = lax.rsqrt(var + EPS)
            layer_norm_tile(sn, t)
        return c

    lax.fori_loop(0, NSEG, segment, 0)
    for t in range(4):
        for ch in range(NPC):
            post_piece(NSEG - 1, t, ch, None)
    for u in range(4):
        o_cp[4 * (NSEG - 1) + u].start()

    bv = best[0]
    bi = best[1]
    vmax = jnp.max(bv, axis=1, keepdims=True)
    cand = jnp.where(bv == vmax, bi, float(S))
    imin = jnp.min(cand, axis=1, keepdims=True)
    idx = jnp.minimum(jnp.max(imin).astype(i32), S - 1)
    tile = idx // 128
    col = idx - tile * 128
    col16 = pl.multiple_of((col // 16) * 16, 16)
    hn_t = hn_v[tile]
    lane_sel = _iota((D, 128), 1) == col
    xs_t = jnp.where(lane_sel, hn_t, jnp.zeros_like(hn_t))
    xs_t = jnp.concatenate([xs_t, jnp.zeros((DP - D, 128), bf16)], axis=0)
    pb0[0:64, :] = jnp.zeros((64, 128), u32)
    xall = xs_t.T
    xn[0:64, 0:L] = _pack(xall[:, 0:L])
    pb0[0:64, :] = _pack(xall[:, L:DP])
    c8 = pl.multiple_of(col16 // 2, 8)
    xs = _unpack(jnp.concatenate([xn[pl.ds(c8, 8), 0:L], pb0[pl.ds(c8, 8), 0:64]], axis=1))
    wg_cp.wait()
    wu_cp.wait()
    gt = jnp.dot(xs, wg_v[...], preferred_element_type=f32)
    up = jnp.dot(xs, wu_v[...], preferred_element_type=f32)
    act = (gt * _sigmoid(gt) * up).astype(bf16)
    wd_cp.wait()
    y = lax.dot_general(act, wd_v[...], NT, preferred_element_type=f32)
    rsel = _sigmoid(vmax[0:1, 0:1])
    yb = (y * rsel).astype(bf16)
    y128 = jnp.concatenate([_pad_lanes(yb), jnp.zeros((112, DP), bf16)], axis=0)
    yt = y128.T[0:D].astype(f32)
    ycol = jnp.sum(jnp.where(_iota((D, 128), 1) == (col - col16), yt, 0.0), axis=1, keepdims=True)
    fin = (h_v[tile].astype(f32)
           + (hn_t.astype(f32) + jnp.where(lane_sel, ycol, 0.0))).astype(bf16)
    for t in range(NTILE):
        o_cp[t].wait()
    out_v[tile] = fin
    pc = cp(out_v.at[tile], out_hbm.at[:, pl.ds(pl.multiple_of(tile * 128, 128), 128)], 15)
    pc.start()
    pc.wait()


@jax.jit
def pallas_sequential_preLN__memory_aug_infini_attn__moe_arch_mod__prompt_kernel(
    A_x: jax.Array,
    A_wq: jax.Array,
    A_wk: jax.Array,
    A_wv: jax.Array,
    A_wo: jax.Array,
    A_beta: jax.Array,
    B_x: jax.Array,
    B_w_r: jax.Array,
    B_w_gate: jax.Array,
    B_w_up: jax.Array,
    B_w_down: jax.Array,
):
    del B_x
    xt = A_x.reshape(S, D).T
    wdt = B_w_down.T
    beta = A_beta.reshape(1, H)
    wr = B_w_r
    hbm = pl.BlockSpec(memory_space=pltpu.HBM)
    vm = pl.BlockSpec(memory_space=pltpu.VMEM)
    V = pltpu.VMEM
    scratch = [
        V((NTILE, D, 128), bf16),
        V((D, D), bf16), V((D, D), bf16), V((D, D), bf16), V((D, D), bf16),
        V((D, F), bf16), V((D, F), bf16), V((D, F), bf16),
        V((3 * DC // 2, DP), u32),
        V((D // 2, DP), u32),
        V((DP // 2, L), u32),
        V((NG, L // 2, 128), u32),
        V((NG, 64, L), u32),
        V((NG, 64, L), u32),
        V((NG, 64, L), u32),
        V((NG, 64, L), u32),
        V((NG, 128, L), f32),
        V((640, 128), u32), V((640, 128), u32),
        V((1280, 128), f32), V((1280, 128), f32),
        V((32, 128), f32), V((32, 128), f32),
        V((NG, 128, 128), f32),
        V((NG, 128, 128), u32),
        V((4, D, 128), bf16),
        V((4, 8, 128), f32),
        V((3, 8, 128), f32),
        V((8, 128), f32),
        V((NTILE, D, 128), bf16), V((NTILE, D, 128), bf16), V((NTILE, D, 128), bf16),
        V((7, 64, 128), u32),
        V((H, 32, 128), f32),
        V((NG, 128, 128), f32),
        V((D, 128), f32),
        V((2, 8, 128), f32),
        V((1, H), bf16), V((D,), bf16),
        pltpu.SemaphoreType.DMA((18,)),
    ]
    out_t = pl.pallas_call(
        _kernel,
        out_shape=jax.ShapeDtypeStruct((D, S), bf16),
        in_specs=[hbm] * 10,
        out_specs=hbm,
        scratch_shapes=scratch,
        compiler_params=pltpu.CompilerParams(vmem_limit_bytes=100 * 1024 * 1024),
    )(xt, A_wq, A_wk, A_wv, A_wo, beta, wr, B_w_gate, B_w_up, wdt)
    return out_t.T.reshape(1, S, D)
```

```python
import jax
import jax.numpy as jnp
from jax import lax
import jax.experimental.pallas as pl
import jax.experimental.pallas.tpu as pltpu

u32 = jnp.uint32
f32 = jnp.float32
bf16 = jnp.bfloat16
i32 = jnp.int32

S = 2048
D = 576
DP = 640
DC = 592
F = 4608
NSEG = 4
L = 512
NTILE = S // 128
H = 32
DH = 18
NG = 5
OFF = (0, 128, 384, 768)
LOG2E = 1.4426950408889634
QSCALE = float(DH ** (-0.5)) * LOG2E
EPS = 1e-05
BOUND = 30.0
VBOUND = 1e20
NT = (((1,), (1,)), ((), ()))
UN_FAST = 8
UN_SLOW = 2
POST_AT = 0
GCH = 1
DEP = True
PSTART = 0
PPS = 1
PSP = 1.0
PCH = 64


def _unpack(x):
    return pltpu.bitcast(x, bf16)


def _pack(x):
    return pltpu.bitcast(x, u32)


def _iota(shape, dim):
    return lax.broadcasted_iota(i32, shape, dim)


def _perm_rows(w, tail):
    c = w.shape[1]
    parts = []
    for g in range(NG):
        if g < NG - 1:
            parts += [w[63 * g:63 * g + 63], jnp.zeros((1, c), u32)]
        else:
            parts += [w[252:288], jnp.zeros((tail - 36, c), u32)]
    return jnp.concatenate(parts, axis=0)


def _pad_lanes(x):
    return jnp.concatenate([x, jnp.zeros((x.shape[0], DP - D), x.dtype)], axis=1)


def _layernorm_t(xf):
    m = jnp.sum(xf, axis=0, keepdims=True) * (1.0 / D)
    xc = xf - m
    v = jnp.sum(xc * xc, axis=0, keepdims=True) * (1.0 / D)
    return xc * lax.rsqrt(v + EPS)


def _phi(t):
    return jnp.where(t > 0, t + 1.0, jnp.exp2(t * LOG2E))


def _sigmoid(t):
    return 1.0 / (1.0 + jnp.exp(-t))


def _absmax(x):
    return jnp.max(jnp.max(jnp.abs(x), axis=0, keepdims=True), axis=1, keepdims=True)


def _kernel(x_hbm, wq_hbm, wk_hbm, wv_hbm, wo_hbm, beta_hbm, wr_hbm, wg_hbm, wu_hbm, wd_hbm,
            out_hbm,
            x_v, wq_v, wk_v, wv_v, wo_v, wg_v, wu_v, wd_v,
            wall, wot, wtmp, wtmp2, xn, kp, phk, qt, phq, vt, ot, pb0, pb1, sb0, sb1, mb0, mb1,
            mt, mlhs, hbuf, st, mxs, racc, h_v, hn_v, out_v, msk, omg, grow, wcol, best, beta_ref, wr_ref, sems):

    def cp(src, dst, i):
        return pltpu.make_async_copy(src, dst, sems.at[i])

    x_cp = [cp(x_hbm.at[:, pl.ds(128 * t, 128)], x_v.at[t], t // 4) for t in range(NTILE)]
    wq_cp, wk_cp, wv_cp, wo_cp = (cp(wq_hbm, wq_v, 4), cp(wk_hbm, wk_v, 5),
                                  cp(wv_hbm, wv_v, 6), cp(wo_hbm, wo_v, 7))
    wg_cp, wu_cp, wd_cp = cp(wg_hbm, wg_v, 8), cp(wu_hbm, wu_v, 9), cp(wd_hbm, wd_v, 10)
    o_cp = [cp(out_v.at[t], out_hbm.at[:, pl.ds(128 * t, 128)], 11 + t // 4) for t in range(NTILE)]

    beta_cp = cp(beta_hbm, beta_ref, 16)
    wr_cp = cp(wr_hbm, wr_ref, 17)
    beta_cp.start()
    wr_cp.start()
    for t in range(4):
        x_cp[t].start()
    wq_cp.start()

    lane128 = _iota((128, 128), 1)
    row128 = _iota((128, 128), 0)
    head_in_group = lax.shift_right_logical(row128 * 57, 10)
    head_col = lax.shift_right_logical(lane128 * 57, 10)
    bd_mask = (head_in_group == head_col) & (head_in_group < 7)

    def tok_of(v):
        return pltpu.bitcast(v[0:8, 0:128], u32)

    def p_masks():
        r64 = _iota((64, 128), 0)
        for j in range(7):
            msk[j] = jnp.where((r64 >= 9 * j) & (r64 < 9 * j + 9), u32(0xFFFFFFFF), u32(0))
        best[0] = jnp.full((8, 128), -jnp.inf, f32)
        best[1] = jnp.zeros((8, 128), f32)
        st[...] = jnp.zeros((4, 8, 128), f32)
        return None

    def p_zero_mt():
        mt[...] = jnp.zeros((NG, 128, 128), f32)
        return None

    def p_zero_h(t):
        def f():
            hbuf[t] = jnp.zeros((D, 128), bf16)
            return None
        return f

    def p_gate(part):
        def f():
            g_lane = _sigmoid(beta_ref[...].astype(f32))
            g_lane = jnp.concatenate([g_lane, jnp.zeros((1, 128 - H), f32)], axis=1)
            if part < NG:
                g = part
                hid = jnp.where(head_in_group < 7, head_in_group + 7 * g, 999)
                sel = jnp.where(lane128 == hid, jnp.broadcast_to(g_lane, (128, 128)), 0.0)
                v = jnp.broadcast_to(jnp.sum(sel, axis=1, keepdims=True), (128, 128))
                grow[g] = v
                return tok_of(v)
            r32 = _iota((32, 128), 0)
            tk = None
            for h in range(8 * (part - NG), 8 * (part - NG) + 8):
                j = h % 7
                off = 18 * j - 16 * ((9 * j) // 8)
                gh = jnp.broadcast_to(g_lane[:, h:h + 1], (32, 128))
                v = jnp.where((r32 >= off) & (r32 < off + 18), 1.0 - gh, 0.0)
                omg[h] = v
                tk = tok_of(v) if tk is None else tk | tok_of(v)
            return tk
        return f

    def p_wcol():
        wr = _pad_lanes(wr_ref[...].astype(f32).reshape(1, D))
        v = jnp.broadcast_to(wr, (128, DP)).T[0:D]
        wcol[...] = v
        return tok_of(v)

    def p_tr(w_ref, c):
        def f():
            wd_ = min(128, D - 128 * c)
            v = _pack(w_ref[:, 128 * c:128 * c + wd_].T)
            wtmp[64 * c:64 * c + wd_ // 2, :] = v
            return v[0:8, 0:128]
        return f

    def p_perm(w):
        def f():
            v = _pad_lanes(_perm_rows(wtmp[...], 40))
            wall[296 * w:296 * (w + 1), :] = v
            return v[0:8, 0:128] | v[288:296, 0:128]
        return f

    def p_wo_perm():
        v = _perm_rows(_pack(wo_v[...]), 64)
        wtmp2[...] = v
        return v[0:8, 0:128]

    def p_wo_tr(c):
        def f():
            wd_ = min(128, D - 128 * c)
            v = _pack(_unpack(wtmp2[:, 128 * c:128 * c + wd_]).T)
            wot[64 * c:64 * c + wd_ // 2, :] = v
            return v[0:8, 0:128]
        return f

    def p_wait(*cs):
        def f():
            for c_ in cs:
                c_()
            return None
        return f

    def layer_norm_tile(seg, t):
        xf = x_v[4 * seg + t].astype(f32)
        xn[0:288, 128 * t:128 * (t + 1)] = _pack(_layernorm_t(xf).astype(bf16))

    wk_cp.start()
    xn[288:320, :] = jnp.zeros((32, L), u32)
    for ref in (qt, phq, phk, vt):
        ref[NG - 1, 40:64] = jnp.zeros((24, L), u32)
    for u in range(4):
        x_cp[u].wait()
    wv_cp.start()
    layer_norm_tile(0, 0)
    wq_cp.wait()
    wo_cp.start()
    for c in range(NG):
        p_tr(wq_v, c)()
    p_perm(0)()
    for t in range(1, 4):
        layer_norm_tile(0, t)

    diag = _iota((128, 128), 0) <= _iota((128, 128), 1)

    def qk_logits(h, i):
        g, j = h // 7, h % 7
        n = 128 * (i + 1)
        qw = qt[g, :, 128 * i:128 * (i + 1)] & msk[j]
        s = jnp.dot(_unpack(kp[g, 0:n // 2, :]), _unpack(qw), preferred_element_type=f32)
        sl = jnp.where(diag, s[n - 128:], -1e30)
        return sl if i == 0 else jnp.concatenate([s[:n - 128], sl], axis=0)

    def pv(h, i, pb):
        g, j = h // 7, h % 7
        n = 128 * (i + 1)
        a8 = pl.multiple_of(((9 * j) // 8) * 8, 8)
        vw = vt[g, pl.ds(a8, 16), 0:n]
        mk = msk[j, pl.ds(a8, 16), :]
        mk = jnp.concatenate([mk] * (i + 1), axis=1)
        vw = (vw & mk) | (jnp.full((16, n), 0x3F803F80, u32) & ~mk)
        o = jnp.dot(_unpack(vw), pb, preferred_element_type=f32)
        og = omg[h]
        r32_ = _iota((32, 128), 0)
        off = 18 * j - 2 * a8
        is_head = (r32_ >= off) & (r32_ < off + 18)
        lsum = jnp.sum(jnp.where(is_head, 0.0, o), axis=0, keepdims=True)
        r = pl.reciprocal(lsum, approx=True) * 14.0
        w16 = pl.multiple_of(a8 * 2, 16)
        ot[g, pl.ds(w16, 32), 128 * i:128 * (i + 1)] += o * (r * og)

    pbs = (pb0, pb1)
    sbs = (sb0, sb1)
    mbs = (mb0, mb1)
    IORD = (3, 2, 1, 0)

    def fast_qk(h, i, pbuf):
        g, j = h // 7, h % 7
        a = (9 * j) // 8
        n = 128 * (i + 1)
        qw = qt[g, 8 * a:8 * a + 16, 128 * i:128 * (i + 1)] & msk[j, 8 * a:8 * a + 16, :]
        parts = [jnp.zeros((8 * a, 128), u32)] if a > 0 else []
        parts.append(qw)
        if 48 - 8 * a > 0:
            parts.append(jnp.zeros((48 - 8 * a, 128), u32))
        qm = _unpack(jnp.concatenate(parts, axis=0))
        s = jnp.dot(_unpack(kp[g, 0:n // 2, :]), qm, preferred_element_type=f32)
        sl = jnp.where(diag, s[n - 128:], -1e30)
        s = sl if i == 0 else jnp.concatenate([s[:n - 128], sl], axis=0)
        pbuf[OFF[i] // 2:(OFF[i] + n) // 2, :] = _pack(jnp.exp2(s).astype(bf16))

    def fast_pv(h, i, pbuf):
        g, j = h // 7, h % 7
        a = (9 * j) // 8
        n = 128 * (i + 1)
        pb = _unpack(pbuf[OFF[i] // 2:(OFF[i] + n) // 2, :])
        mk = msk[j, 8 * a:8 * a + 16, :]
        mk = jnp.concatenate([mk] * (i + 1), axis=1)
        vw = (vt[g, 8 * a:8 * a + 16, 0:n] & mk) | (jnp.full((16, n), 0x3F803F80, u32) & ~mk)
        o = jnp.dot(_unpack(vw), pb, preferred_element_type=f32)
        off = 18 * j - 16 * a
        l8 = o[24:32] if off <= 6 else o[0:8]
        r = pl.reciprocal(l8, approx=True)
        for t in range(4):
            if 8 * t + 8 <= off or 8 * t >= off + 18:
                continue
            rs_ = slice(16 * a + 8 * t, 16 * a + 8 * t + 8)
            cs = slice(128 * i, 128 * (i + 1))
            ot[g, rs_, cs] += o[8 * t:8 * t + 8] * (r * omg[h, 8 * t:8 * t + 8, :])

    def slow_qk(h, i, sbuf, mbuf):
        n = 128 * (i + 1)
        s = qk_logits(h, i)
        sbuf[OFF[i]:OFF[i] + n, :] = s
        mbuf[8 * i:8 * i + 8, :] = jnp.broadcast_to(jnp.max(s, axis=0, keepdims=True), (8, 128))

    def slow_pv(h, i, sbuf, mbuf):
        n = 128 * (i + 1)
        s = sbuf[OFF[i]:OFF[i] + n, :]
        p = jnp.exp2(s - mbuf[8 * i:8 * i + 1, :]).astype(bf16)
        pv(h, i, p)

    def attention_fast():
        for i in IORD:
            fast_qk(0, i, pbs[0])
        for h in range(H):
            if h + 1 < H:
                for i in IORD:
                    fast_qk(h + 1, i, pbs[(h + 1) % 2])
            for i in IORD:
                fast_pv(h, i, pbs[h % 2])

    def attention_slow():
        for i in IORD:
            slow_qk(0, i, sbs[0], mbs[0])

        def body(it, c):
            for u in range(UN_SLOW):
                h = it * UN_SLOW + u
                hn_ = jnp.minimum(h + 1, H - 1)
                for i in IORD:
                    slow_qk(hn_, i, sbs[1 - u % 2], mbs[1 - u % 2])
                for i in IORD:
                    slow_pv(h, i, sbs[u % 2], mbs[u % 2])
            return c
        lax.fori_loop(0, H // UN_SLOW, body, 0)

    def wait_x(seg):
        for t in range(NSEG):
            @pl.when(seg == t)
            def _():
                for u in range(4):
                    x_cp[4 * t + u].wait()

    NPC = D // PCH

    def post_piece(seg, t, ch, valid):
        m = st[t, 0:1, :]
        rs = st[t, 1:2, :]
        rsl = slice(PCH * ch, PCH * (ch + 1))
        hf = hbuf[t, rsl].astype(f32)
        hnb = ((hf - m) * rs).astype(bf16)
        hnf = hnb.astype(f32)
        hn_v[4 * seg + t, rsl] = hnb
        ob_ = (hf + hnf).astype(bf16)
        out_v[4 * seg + t, rsl] = ob_
        r_ = jnp.sum((hnf * wcol[rsl]).reshape(PCH // 8, 8, 128), axis=0)
        if ch > 0:
            r_ = r_ + racc[...]
        if ch < NPC - 1:
            racc[...] = r_
        else:
            bv = best[0]
            bi = best[1]
            lane = _iota((8, 128), 1).astype(f32)
            rr = jnp.sum(r_, axis=0, keepdims=True).astype(bf16).astype(f32)
            rt = jnp.broadcast_to(rr, (8, 128))
            upd_ = rt > bv
            if valid is not None:
                upd_ = jnp.logical_and(upd_, valid)
            best[0] = jnp.where(upd_, rt, bv)
            best[1] = jnp.where(upd_, lane + jnp.asarray(seg * L + 128 * t, i32).astype(f32), bi)
        return _pack(ob_[0:16]) | pltpu.bitcast(r_, u32)

    def start_out(seg):
        for t in range(NSEG):
            @pl.when(seg == t)
            def _():
                for u in range(4):
                    o_cp[4 * t + u].start()

    def post_p(seg, t, ch, valid):
        return lambda: post_piece(seg, t, ch, valid)

    def qkv_block(pieces, opaque):
        pieces = list(pieces)
        zero = jnp.full((8, 128), lax.shift_right_logical(opaque, 8), i32).astype(u32)
        tok = None
        for w in range(3):
            m_ = None
            for t in range(4):
                cs = slice(128 * t, 128 * (t + 1))
                xt_ = _unpack(xn[:, cs])
                for g in range(NG):
                    nr = 128 if g < NG - 1 else 80
                    while pieces and pieces[0][0] is not None and pieces[0][0] <= (w * 4 + t) * NG + g - 1e-9:
                        tk = pieces.pop(0)[1]()
                        if tk is not None:
                            tok = tk if tok is None else tok | tk
                    r0_ = DC * w + 128 * g
                    lhs = wall[r0_ // 2:(r0_ + nr) // 2, :]
                    if tok is not None:
                        head = lhs[0:8, 0:128] | (tok & zero)
                        lhs = jnp.concatenate([
                            jnp.concatenate([head, lhs[0:8, 128:]], axis=1), lhs[8:]], axis=0)
                        tok = None
                    a = jnp.dot(_unpack(lhs), xt_, preferred_element_type=f32)
                    if w == 0:
                        phq[g, 0:nr // 2, cs] = _pack(_phi(a).astype(bf16))
                        a = a * QSCALE
                        qt[g, 0:nr // 2, cs] = _pack(a.astype(bf16))
                    elif w == 1:
                        phk[g, 0:nr // 2, cs] = _pack(_phi(a).astype(bf16))
                        ab = a.astype(bf16)
                        if nr < 128:
                            ab = jnp.concatenate([ab, jnp.zeros((128 - nr, 128), bf16)], axis=0)
                        kp[g, 64 * t:64 * (t + 1), :] = _pack(ab.T)
                    else:
                        vt[g, 0:nr // 2, cs] = _pack(a.astype(bf16))
                    am = jnp.max(jnp.abs(a).reshape(nr // 8, 8, 128), axis=0)
                    m_ = am if m_ is None else jnp.maximum(m_, am)
            mxs[w] = m_
        assert not pieces

    p0 = []
    p0.append((0.5, p_wait(wk_cp.wait, *[x_cp[t].start for t in range(4, NTILE)])))
    for c in range(NG):
        p0.append((1 + c, p_tr(wk_v, c)))
    p0.append((7, p_perm(1)))
    p0.append((8.5, p_wait(wv_cp.wait)))
    for c in range(NG):
        p0.append((9 + c, p_tr(wv_v, c)))
    p0.append((15, p_perm(2)))
    p0.append((16.5, p_wait(wo_cp.wait, wg_cp.start, wu_cp.start, wd_cp.start, beta_cp.wait, wr_cp.wait)))
    p0.append((17, p_wo_perm))
    for c in range(NG):
        p0.append((19 + c, p_wo_tr(c)))
    p0.append((25, p_masks))
    p0.append((26, p_zero_mt))
    for part in range(NG + 4):
        p0.append((28 + 2 * part, p_gate(part)))
    p0.append((47, p_wcol))
    qkv_block(p0, jnp.int32(0) if False else pl.program_id(0))

    def segment(s, c):
        sp = jnp.maximum(s - 1, 0)
        @pl.when(s > 0)
        def _():
            qkv_block([(0.5 + PSP * (t * NPC + ch), post_p(sp, t, ch, None)) for t in range(4) for ch in range(NPC)], s)

        @pl.when(s > 0)
        def _():
            start_out(s - 1)

        @pl.when(s == 0)
        def _():
            ot[...] = jnp.zeros((NG, 128, L), f32)

        @pl.when(s > 0)
        def _():
            for g in range(NG):
                nd = jnp.dot(_unpack(mlhs[g]), _unpack(phq[g]), preferred_element_type=f32)
                num = nd[0:128]
                den = nd[128:256] + 1e-06
                gr = grow[g]
                ot[g] = num * (pl.reciprocal(den, approx=True) * jnp.concatenate([gr] * 4, axis=1))

        mxv = [_absmax(mxs[w]) for w in range(3)]
        bound = mxv[0] * mxv[1] * (DH * 1.02)
        ok = jnp.where((bound <= BOUND) & (mxv[2] <= VBOUND), 1, 0).astype(i32)
        safe = jnp.max(ok) > 0

        @pl.when(safe)
        def _():
            attention_fast()

        @pl.when(jnp.logical_not(safe))
        def _():
            attention_slow()

        @pl.when(s < NSEG - 1)
        def _():
            r64_ = _iota((64, L), 0)
            ones = jnp.full((64, L), 0x3F803F80, u32)
            for g in range(NG):
                lhs = jnp.where(r64_ == 63, ones, vt[g])
                upd = lax.dot_general(_unpack(lhs), _unpack(phk[g]), NT,
                                      preferred_element_type=f32)
                cur = mt[g] + upd
                mt[g] = cur
                m_bd = jnp.where(bd_mask, cur, 0.0)
                z_bd = jnp.where(bd_mask, jnp.broadcast_to(cur[126:127, :], (128, 128)), 0.0)
                mlhs[g] = _pack(jnp.concatenate([m_bd, z_bd], axis=0).astype(bf16))
            wait_x(s + 1)

        sn = jnp.minimum(s + 1, NSEG - 1)
        for t in range(4):
            cs = slice(128 * t, 128 * (t + 1))
            ob = jnp.concatenate([ot[g, :, cs] for g in range(NG)], axis=0).astype(bf16)
            ao = jnp.dot(_unpack(wot[...]), ob, preferred_element_type=f32)
            piv = s1 = s2 = None
            for ch in range(D // PCH):
                rsl = slice(PCH * ch, PCH * (ch + 1))
                hb = (x_v[4 * s + t, rsl].astype(f32) + ao[rsl]).astype(bf16)
                hbuf[t, rsl] = hb
                h_v[4 * s + t, rsl] = hb
                hf = hb.astype(f32)
                if piv is None:
                    piv = hf[0:1, :]
                dd = hf - piv
                a1 = jnp.sum(dd.reshape(PCH // 8, 8, 128), axis=0)
                a2 = jnp.sum((dd * dd).reshape(PCH // 8, 8, 128), axis=0)
                s1 = a1 if s1 is None else s1 + a1
                s2 = a2 if s2 is None else s2 + a2
            e1 = jnp.sum(s1, axis=0, keepdims=True) * (1.0 / D)
            e2 = jnp.sum(s2, axis=0, keepdims=True) * (1.0 / D)
            var = jnp.maximum(e2 - e1 * e1, 0.0)
            st[t, 0:1, :] = piv + e1
            st[t, 1:2, :] = lax.rsqrt(var + EPS)
            layer_norm_tile(sn, t)
        return c

    lax.fori_loop(0, NSEG, segment, 0)
    for t in range(4):
        for ch in range(NPC):
            post_piece(NSEG - 1, t, ch, None)
    for u in range(4):
        o_cp[4 * (NSEG - 1) + u].start()

    bv = best[0]
    bi = best[1]
    vmax = jnp.max(bv, axis=1, keepdims=True)
    cand = jnp.where(bv == vmax, bi, float(S))
    imin = jnp.min(cand, axis=1, keepdims=True)
    idx = jnp.minimum(jnp.max(imin).astype(i32), S - 1)
    tile = idx // 128
    col = idx - tile * 128
    col16 = pl.multiple_of((col // 16) * 16, 16)
    hn_t = hn_v[tile]
    lane_sel = _iota((D, 128), 1) == col
    xs_t = jnp.where(lane_sel, hn_t, jnp.zeros_like(hn_t))
    xs_t = jnp.concatenate([xs_t, jnp.zeros((DP - D, 128), bf16)], axis=0)
    pb0[0:64, :] = jnp.zeros((64, 128), u32)
    xall = xs_t.T
    xn[0:64, 0:L] = _pack(xall[:, 0:L])
    pb0[0:64, :] = _pack(xall[:, L:DP])
    c8 = pl.multiple_of(col16 // 2, 8)
    xs = _unpack(jnp.concatenate([xn[pl.ds(c8, 8), 0:L], pb0[pl.ds(c8, 8), 0:64]], axis=1))
    wg_cp.wait()
    wu_cp.wait()
    gt = jnp.dot(xs, wg_v[...], preferred_element_type=f32)
    up = jnp.dot(xs, wu_v[...], preferred_element_type=f32)
    act = (gt * _sigmoid(gt) * up).astype(bf16)
    wd_cp.wait()
    y = lax.dot_general(act, wd_v[...], NT, preferred_element_type=f32)
    rsel = _sigmoid(vmax[0:1, 0:1])
    yb = (y * rsel).astype(bf16)
    y128 = jnp.concatenate([_pad_lanes(yb), jnp.zeros((112, DP), bf16)], axis=0)
    yt = y128.T[0:D].astype(f32)
    ycol = jnp.sum(jnp.where(_iota((D, 128), 1) == (col - col16), yt, 0.0), axis=1, keepdims=True)
    fin = (h_v[tile].astype(f32)
           + (hn_t.astype(f32) + jnp.where(lane_sel, ycol, 0.0))).astype(bf16)
    for t in range(NTILE):
        o_cp[t].wait()
    out_v[tile] = fin
    pc = cp(out_v.at[tile], out_hbm.at[:, pl.ds(pl.multiple_of(tile * 128, 128), 128)], 15)
    pc.start()
    pc.wait()


@jax.jit
def pallas_sequential_preLN__memory_aug_infini_attn__moe_arch_mod__prompt_kernel(
    A_x: jax.Array,
    A_wq: jax.Array,
    A_wk: jax.Array,
    A_wv: jax.Array,
    A_wo: jax.Array,
    A_beta: jax.Array,
    B_x: jax.Array,
    B_w_r: jax.Array,
    B_w_gate: jax.Array,
    B_w_up: jax.Array,
    B_w_down: jax.Array,
):
    del B_x
    xt = A_x.reshape(S, D).T
    wdt = B_w_down.T
    beta = A_beta.reshape(1, H)
    wr = B_w_r
    hbm = pl.BlockSpec(memory_space=pltpu.HBM)
    vm = pl.BlockSpec(memory_space=pltpu.VMEM)
    V = pltpu.VMEM
    scratch = [
        V((NTILE, D, 128), bf16),
        V((D, D), bf16), V((D, D), bf16), V((D, D), bf16), V((D, D), bf16),
        V((D, F), bf16), V((D, F), bf16), V((D, F), bf16),
        V((3 * DC // 2, DP), u32),
        V((D // 2, DP), u32),
        V((D // 2, D), u32),
        V((DP // 2, D), u32),
        V((DP // 2, L), u32),
        V((NG, L // 2, 128), u32),
        V((NG, 64, L), u32),
        V((NG, 64, L), u32),
        V((NG, 64, L), u32),
        V((NG, 64, L), u32),
        V((NG, 128, L), f32),
        V((640, 128), u32), V((640, 128), u32),
        V((1280, 128), f32), V((1280, 128), f32),
        V((32, 128), f32), V((32, 128), f32),
        V((NG, 128, 128), f32),
        V((NG, 128, 128), u32),
        V((4, D, 128), bf16),
        V((4, 8, 128), f32),
        V((3, 8, 128), f32),
        V((8, 128), f32),
        V((NTILE, D, 128), bf16), V((NTILE, D, 128), bf16), V((NTILE, D, 128), bf16),
        V((7, 64, 128), u32),
        V((H, 32, 128), f32),
        V((NG, 128, 128), f32),
        V((D, 128), f32),
        V((2, 8, 128), f32),
        V((1, H), bf16), V((D,), bf16),
        pltpu.SemaphoreType.DMA((18,)),
    ]
    out_t = pl.pallas_call(
        _kernel,
        out_shape=jax.ShapeDtypeStruct((D, S), bf16),
        grid=(1,),
        in_specs=[hbm] * 10,
        out_specs=hbm,
        scratch_shapes=scratch,
        compiler_params=pltpu.CompilerParams(vmem_limit_bytes=100 * 1024 * 1024),
    )(xt, A_wq, A_wk, A_wv, A_wo, beta, wr, B_w_gate, B_w_up, wdt)
    return out_t.T.reshape(1, S, D)
```

```python
import jax
import jax.numpy as jnp
from jax import lax
import jax.experimental.pallas as pl
import jax.experimental.pallas.tpu as pltpu

u32 = jnp.uint32
f32 = jnp.float32
bf16 = jnp.bfloat16
i32 = jnp.int32

S = 2048
D = 576
DP = 640
DC = 592
F = 4608
NSEG = 4
L = 512
NTILE = S // 128
H = 32
DH = 18
NG = 5
OFF = (0, 128, 384, 768)
LOG2E = 1.4426950408889634
QSCALE = float(DH ** (-0.5)) * LOG2E
EPS = 1e-05
BOUND = 30.0
VBOUND = 1e20
NT = (((1,), (1,)), ((), ()))
UN_FAST = 8
UN_SLOW = 2
POST_AT = 0
GCH = 1
DEP = True
PSTART = 0
PPS = 1
PSP = 1.0
PCH = 64


def _unpack(x):
    return pltpu.bitcast(x, bf16)


def _pack(x):
    return pltpu.bitcast(x, u32)


def _iota(shape, dim):
    return lax.broadcasted_iota(i32, shape, dim)


def _perm_rows(w, tail):
    c = w.shape[1]
    parts = []
    for g in range(NG):
        if g < NG - 1:
            parts += [w[63 * g:63 * g + 63], jnp.zeros((1, c), u32)]
        else:
            parts += [w[252:288], jnp.zeros((tail - 36, c), u32)]
    return jnp.concatenate(parts, axis=0)


def _pad_lanes(x):
    return jnp.concatenate([x, jnp.zeros((x.shape[0], DP - D), x.dtype)], axis=1)


def _layernorm_t(xf):
    m = jnp.sum(xf, axis=0, keepdims=True) * (1.0 / D)
    xc = xf - m
    v = jnp.sum(xc * xc, axis=0, keepdims=True) * (1.0 / D)
    return xc * lax.rsqrt(v + EPS)


def _phi(t):
    return jnp.where(t > 0, t + 1.0, jnp.exp2(t * LOG2E))


def _sigmoid(t):
    return 1.0 / (1.0 + jnp.exp(-t))


def _absmax(x):
    return jnp.max(jnp.max(jnp.abs(x), axis=0, keepdims=True), axis=1, keepdims=True)


def _kernel(x_hbm, wq_hbm, wk_hbm, wv_hbm, wo_hbm, beta_hbm, wr_hbm, wg_hbm, wu_hbm, wd_hbm,
            out_hbm,
            x_v, wq_v, wk_v, wv_v, wo_v, wg_v, wu_v, wd_v,
            wall, wot, wtmp, wtmp2, xn, kp, phk, qt, phq, vt, ot, pb0, pb1, sb0, sb1, mb0, mb1,
            mt, mlhs, hbuf, st, mxs, racc, h_v, hn_v, out_v, msk, omg, grow, wcol, best, beta_ref, wr_ref, sems):

    def cp(src, dst, i):
        return pltpu.make_async_copy(src, dst, sems.at[i])

    x_cp = [cp(x_hbm.at[:, pl.ds(128 * t, 128)], x_v.at[t], t // 4) for t in range(NTILE)]
    wq_cp, wk_cp, wv_cp, wo_cp = (cp(wq_hbm, wq_v, 4), cp(wk_hbm, wk_v, 5),
                                  cp(wv_hbm, wv_v, 6), cp(wo_hbm, wo_v, 7))
    wg_cp, wu_cp, wd_cp = cp(wg_hbm, wg_v, 8), cp(wu_hbm, wu_v, 9), cp(wd_hbm, wd_v, 10)
    o_cp = [cp(out_v.at[t], out_hbm.at[:, pl.ds(128 * t, 128)], 11 + t // 4) for t in range(NTILE)]

    beta_cp = cp(beta_hbm, beta_ref, 16)
    wr_cp = cp(wr_hbm, wr_ref, 17)
    beta_cp.start()
    wr_cp.start()
    for t in range(4):
        x_cp[t].start()
    wq_cp.start()

    lane128 = _iota((128, 128), 1)
    row128 = _iota((128, 128), 0)
    head_in_group = lax.shift_right_logical(row128 * 57, 10)
    head_col = lax.shift_right_logical(lane128 * 57, 10)
    bd_mask = (head_in_group == head_col) & (head_in_group < 7)

    def tok_of(v):
        return pltpu.bitcast(v[0:8, 0:128], u32)

    def p_masks():
        r64 = _iota((64, 128), 0)
        for j in range(7):
            msk[j] = jnp.where((r64 >= 9 * j) & (r64 < 9 * j + 9), u32(0xFFFFFFFF), u32(0))
        best[0] = jnp.full((8, 128), -jnp.inf, f32)
        best[1] = jnp.zeros((8, 128), f32)
        return None

    def p_zero_mt():
        mt[...] = jnp.zeros((NG, 128, 128), f32)
        return None

    def p_zero_h(t):
        def f():
            hbuf[t] = jnp.zeros((D, 128), bf16)
            return None
        return f

    def p_gate(part):
        def f():
            g_lane = _sigmoid(beta_ref[...].astype(f32))
            g_lane = jnp.concatenate([g_lane, jnp.zeros((1, 128 - H), f32)], axis=1)
            if part < NG:
                g = part
                hid = jnp.where(head_in_group < 7, head_in_group + 7 * g, 999)
                sel = jnp.where(lane128 == hid, jnp.broadcast_to(g_lane, (128, 128)), 0.0)
                v = jnp.broadcast_to(jnp.sum(sel, axis=1, keepdims=True), (128, 128))
                grow[g] = v
                return tok_of(v)
            r32 = _iota((32, 128), 0)
            tk = None
            for h in range(8 * (part - NG), 8 * (part - NG) + 8):
                j = h % 7
                off = 18 * j - 16 * ((9 * j) // 8)
                gh = jnp.broadcast_to(g_lane[:, h:h + 1], (32, 128))
                v = jnp.where((r32 >= off) & (r32 < off + 18), 1.0 - gh, 0.0)
                omg[h] = v
                tk = tok_of(v) if tk is None else tk | tok_of(v)
            return tk
        return f

    def p_wcol():
        wr = _pad_lanes(wr_ref[...].astype(f32).reshape(1, D))
        v = jnp.broadcast_to(wr, (128, DP)).T[0:D]
        wcol[...] = v
        return tok_of(v)

    def p_tr(w_ref, c):
        def f():
            wd_ = min(128, D - 128 * c)
            v = _pack(w_ref[:, 128 * c:128 * c + wd_].T)
            wtmp[64 * c:64 * c + wd_ // 2, :] = v
            return v[0:8, 0:128]
        return f

    def p_perm(w):
        def f():
            v = _pad_lanes(_perm_rows(wtmp[...], 40))
            wall[296 * w:296 * (w + 1), :] = v
            return v[0:8, 0:128] | v[288:296, 0:128]
        return f

    def p_wo_perm():
        v = _perm_rows(_pack(wo_v[...]), 64)
        wtmp2[...] = v
        return v[0:8, 0:128]

    def p_wo_tr(c):
        def f():
            wd_ = min(128, D - 128 * c)
            v = _pack(_unpack(wtmp2[:, 128 * c:128 * c + wd_]).T)
            wot[64 * c:64 * c + wd_ // 2, :] = v
            return v[0:8, 0:128]
        return f

    def p_wait(*cs):
        def f():
            for c_ in cs:
                c_()
            return None
        return f

    def layer_norm_tile(seg, t):
        xf = x_v[4 * seg + t].astype(f32)
        xn[0:288, 128 * t:128 * (t + 1)] = _pack(_layernorm_t(xf).astype(bf16))

    wk_cp.start()
    xn[288:320, :] = jnp.zeros((32, L), u32)
    for ref in (qt, phq, phk, vt):
        ref[NG - 1, 40:64] = jnp.zeros((24, L), u32)
    for u in range(4):
        x_cp[u].wait()
    wv_cp.start()
    layer_norm_tile(0, 0)
    wq_cp.wait()
    wo_cp.start()
    for c in range(NG):
        p_tr(wq_v, c)()
    p_perm(0)()
    for t in range(1, 4):
        layer_norm_tile(0, t)

    diag = _iota((128, 128), 0) <= _iota((128, 128), 1)

    def qk_logits(h, i):
        g, j = h // 7, h % 7
        n = 128 * (i + 1)
        qw = qt[g, :, 128 * i:128 * (i + 1)] & msk[j]
        s = jnp.dot(_unpack(kp[g, 0:n // 2, :]), _unpack(qw), preferred_element_type=f32)
        sl = jnp.where(diag, s[n - 128:], -1e30)
        return sl if i == 0 else jnp.concatenate([s[:n - 128], sl], axis=0)

    def pv(h, i, pb):
        g, j = h // 7, h % 7
        n = 128 * (i + 1)
        a8 = pl.multiple_of(((9 * j) // 8) * 8, 8)
        vw = vt[g, pl.ds(a8, 16), 0:n]
        mk = msk[j, pl.ds(a8, 16), :]
        mk = jnp.concatenate([mk] * (i + 1), axis=1)
        vw = (vw & mk) | (jnp.full((16, n), 0x3F803F80, u32) & ~mk)
        o = jnp.dot(_unpack(vw), pb, preferred_element_type=f32)
        og = omg[h]
        r32_ = _iota((32, 128), 0)
        off = 18 * j - 2 * a8
        is_head = (r32_ >= off) & (r32_ < off + 18)
        lsum = jnp.sum(jnp.where(is_head, 0.0, o), axis=0, keepdims=True)
        r = pl.reciprocal(lsum, approx=True) * 14.0
        w16 = pl.multiple_of(a8 * 2, 16)
        ot[g, pl.ds(w16, 32), 128 * i:128 * (i + 1)] += o * (r * og)

    pbs = (pb0, pb1)
    sbs = (sb0, sb1)
    mbs = (mb0, mb1)
    IORD = (3, 2, 1, 0)

    def fast_qk(h, i, pbuf):
        g, j = h // 7, h % 7
        a = (9 * j) // 8
        n = 128 * (i + 1)
        qw = qt[g, 8 * a:8 * a + 16, 128 * i:128 * (i + 1)] & msk[j, 8 * a:8 * a + 16, :]
        parts = [jnp.zeros((8 * a, 128), u32)] if a > 0 else []
        parts.append(qw)
        if 48 - 8 * a > 0:
            parts.append(jnp.zeros((48 - 8 * a, 128), u32))
        qm = _unpack(jnp.concatenate(parts, axis=0))
        s = jnp.dot(_unpack(kp[g, 0:n // 2, :]), qm, preferred_element_type=f32)
        sl = jnp.where(diag, s[n - 128:], -1e30)
        s = sl if i == 0 else jnp.concatenate([s[:n - 128], sl], axis=0)
        pbuf[OFF[i] // 2:(OFF[i] + n) // 2, :] = _pack(jnp.exp2(s).astype(bf16))

    def fast_pv(h, i, pbuf):
        g, j = h // 7, h % 7
        a = (9 * j) // 8
        n = 128 * (i + 1)
        pb = _unpack(pbuf[OFF[i] // 2:(OFF[i] + n) // 2, :])
        mk = msk[j, 8 * a:8 * a + 16, :]
        mk = jnp.concatenate([mk] * (i + 1), axis=1)
        vw = (vt[g, 8 * a:8 * a + 16, 0:n] & mk) | (jnp.full((16, n), 0x3F803F80, u32) & ~mk)
        o = jnp.dot(_unpack(vw), pb, preferred_element_type=f32)
        off = 18 * j - 16 * a
        l8 = o[24:32] if off <= 6 else o[0:8]
        r = pl.reciprocal(l8, approx=True)
        for t in range(4):
            if 8 * t + 8 <= off or 8 * t >= off + 18:
                continue
            rs_ = slice(16 * a + 8 * t, 16 * a + 8 * t + 8)
            cs = slice(128 * i, 128 * (i + 1))
            ot[g, rs_, cs] += o[8 * t:8 * t + 8] * (r * omg[h, 8 * t:8 * t + 8, :])

    def slow_qk(h, i, sbuf, mbuf):
        n = 128 * (i + 1)
        s = qk_logits(h, i)
        sbuf[OFF[i]:OFF[i] + n, :] = s
        mbuf[8 * i:8 * i + 8, :] = jnp.broadcast_to(jnp.max(s, axis=0, keepdims=True), (8, 128))

    def slow_pv(h, i, sbuf, mbuf):
        n = 128 * (i + 1)
        s = sbuf[OFF[i]:OFF[i] + n, :]
        p = jnp.exp2(s - mbuf[8 * i:8 * i + 1, :]).astype(bf16)
        pv(h, i, p)

    def attention_fast():
        for i in IORD:
            fast_qk(0, i, pbs[0])
        for h in range(H):
            if h + 1 < H:
                for i in IORD:
                    fast_qk(h + 1, i, pbs[(h + 1) % 2])
            for i in IORD:
                fast_pv(h, i, pbs[h % 2])

    def attention_slow():
        for i in IORD:
            slow_qk(0, i, sbs[0], mbs[0])

        def body(it, c):
            for u in range(UN_SLOW):
                h = it * UN_SLOW + u
                hn_ = jnp.minimum(h + 1, H - 1)
                for i in IORD:
                    slow_qk(hn_, i, sbs[1 - u % 2], mbs[1 - u % 2])
                for i in IORD:
                    slow_pv(h, i, sbs[u % 2], mbs[u % 2])
            return c
        lax.fori_loop(0, H // UN_SLOW, body, 0)

    def wait_x(seg):
        for t in range(NSEG):
            @pl.when(seg == t)
            def _():
                for u in range(4):
                    x_cp[4 * t + u].wait()

    NPC = D // PCH

    def post_piece(seg, t, ch, valid):
        m = st[t, 0:1, :]
        rs = st[t, 1:2, :]
        rsl = slice(PCH * ch, PCH * (ch + 1))
        hf = hbuf[t, rsl].astype(f32)
        hnb = ((hf - m) * rs).astype(bf16)
        hnf = hnb.astype(f32)
        hn_v[4 * seg + t, rsl] = hnb
        ob_ = (hf + hnf).astype(bf16)
        out_v[4 * seg + t, rsl] = ob_
        r_ = jnp.sum((hnf * wcol[rsl]).reshape(PCH // 8, 8, 128), axis=0)
        if ch > 0:
            r_ = r_ + racc[...]
        if ch < NPC - 1:
            racc[...] = r_
        else:
            bv = best[0]
            bi = best[1]
            lane = _iota((8, 128), 1).astype(f32)
            rr = jnp.sum(r_, axis=0, keepdims=True).astype(bf16).astype(f32)
            rt = jnp.broadcast_to(rr, (8, 128))
            upd_ = rt > bv
            if valid is not None:
                upd_ = jnp.logical_and(upd_, valid)
            best[0] = jnp.where(upd_, rt, bv)
            best[1] = jnp.where(upd_, lane + jnp.asarray(seg * L + 128 * t, i32).astype(f32), bi)
        return _pack(ob_[0:16]) | pltpu.bitcast(r_, u32)

    def start_out(seg):
        for t in range(NSEG):
            @pl.when(seg == t)
            def _():
                for u in range(4):
                    o_cp[4 * t + u].start()

    def post_p(seg, t, ch, valid):
        return lambda: post_piece(seg, t, ch, valid)

    def qkv_block(pieces, opaque):
        pieces = list(pieces)
        zero = jnp.full((8, 128), lax.shift_right_logical(opaque, 8), i32).astype(u32)
        tok = None
        for w in range(3):
            m_ = None
            for t in range(4):
                cs = slice(128 * t, 128 * (t + 1))
                xt_ = _unpack(xn[:, cs])
                for g in range(NG):
                    nr = 128 if g < NG - 1 else 80
                    while pieces and pieces[0][0] is not None and pieces[0][0] <= (w * 4 + t) * NG + g - 1e-9:
                        tk = pieces.pop(0)[1]()
                        if tk is not None:
                            tok = tk if tok is None else tok | tk
                    r0_ = DC * w + 128 * g
                    lhs = wall[r0_ // 2:(r0_ + nr) // 2, :]
                    if tok is not None:
                        head = lhs[0:8, 0:128] | (tok & zero)
                        lhs = jnp.concatenate([
                            jnp.concatenate([head, lhs[0:8, 128:]], axis=1), lhs[8:]], axis=0)
                        tok = None
                    a = jnp.dot(_unpack(lhs), xt_, preferred_element_type=f32)
                    if w == 0:
                        phq[g, 0:nr // 2, cs] = _pack(_phi(a).astype(bf16))
                        a = a * QSCALE
                        qt[g, 0:nr // 2, cs] = _pack(a.astype(bf16))
                    elif w == 1:
                        phk[g, 0:nr // 2, cs] = _pack(_phi(a).astype(bf16))
                        ab = a.astype(bf16)
                        if nr < 128:
                            ab = jnp.concatenate([ab, jnp.zeros((128 - nr, 128), bf16)], axis=0)
                        kp[g, 64 * t:64 * (t + 1), :] = _pack(ab.T)
                    else:
                        vt[g, 0:nr // 2, cs] = _pack(a.astype(bf16))
                    am = jnp.max(jnp.abs(a).reshape(nr // 8, 8, 128), axis=0)
                    m_ = am if m_ is None else jnp.maximum(m_, am)
            mxs[w] = m_
        assert not pieces

    p0 = []
    p0.append((0.5, p_wait(wk_cp.wait, *[x_cp[t].start for t in range(4, NTILE)])))
    for c in range(NG):
        p0.append((1 + c, p_tr(wk_v, c)))
    p0.append((7, p_perm(1)))
    p0.append((8.5, p_wait(wv_cp.wait)))
    for c in range(NG):
        p0.append((9 + c, p_tr(wv_v, c)))
    p0.append((15, p_perm(2)))
    p0.append((16.5, p_wait(wo_cp.wait, wg_cp.start, wu_cp.start, wd_cp.start, beta_cp.wait, wr_cp.wait)))
    p0.append((17, p_wo_perm))
    for c in range(NG):
        p0.append((19 + c, p_wo_tr(c)))
    p0.append((25, p_masks))
    p0.append((26, p_zero_mt))
    for part in range(NG + 4):
        p0.append((28 + 2 * part, p_gate(part)))
    p0.append((47, p_wcol))
    qkv_block(p0, jnp.int32(0) if False else pl.program_id(0))

    def segment(s, c):
        @pl.when(s == 0)
        def _():
            ot[...] = jnp.zeros((NG, 128, L), f32)

        @pl.when(s > 0)
        def _():
            sp = s - 1
            r64_ = _iota((64, L), 0)
            ones = jnp.full((64, L), 0x3F803F80, u32)
            for g in range(NG):
                lhs = jnp.where(r64_ == 63, ones, vt[g])
                upd = lax.dot_general(_unpack(lhs), _unpack(phk[g]), NT,
                                      preferred_element_type=f32)
                cur = mt[g] + upd
                mt[g] = cur
                m_bd = jnp.where(bd_mask, cur, 0.0)
                z_bd = jnp.where(bd_mask, jnp.broadcast_to(cur[126:127, :], (128, 128)), 0.0)
                mlhs[g] = _pack(jnp.concatenate([m_bd, z_bd], axis=0).astype(bf16))
            qkv_block([(0.5 + PSP * (t * NPC + ch), post_p(sp, t, ch, None))
                       for t in range(4) for ch in range(NPC)], s)
            for g in range(NG):
                nr = 128 if g < NG - 1 else 80
                lhs = jnp.concatenate([mlhs[g, 0:nr // 2], mlhs[g, 64:64 + nr // 2]], axis=0)
                nd = jnp.dot(_unpack(lhs), _unpack(phq[g]), preferred_element_type=f32)
                num = nd[0:nr]
                den = nd[nr:2 * nr] + 1e-06
                gr = grow[g, 0:nr]
                ot[g, 0:nr] = num * (pl.reciprocal(den, approx=True) * jnp.concatenate([gr] * 4, axis=1))
            start_out(sp)

        mxv = [_absmax(mxs[w]) for w in range(3)]
        bound = mxv[0] * mxv[1] * (DH * 1.02)
        ok = jnp.where((bound <= BOUND) & (mxv[2] <= VBOUND), 1, 0).astype(i32)
        safe = jnp.max(ok) > 0

        @pl.when(safe)
        def _():
            attention_fast()

        @pl.when(jnp.logical_not(safe))
        def _():
            attention_slow()

        @pl.when(s < NSEG - 1)
        def _():
            wait_x(s + 1)

        sn = jnp.minimum(s + 1, NSEG - 1)
        for t in range(4):
            cs = slice(128 * t, 128 * (t + 1))
            ob = jnp.concatenate([ot[g, :, cs] for g in range(NG)], axis=0).astype(bf16)
            ao = jnp.dot(_unpack(wot[...]), ob, preferred_element_type=f32)
            piv = s1 = s2 = None
            for ch in range(D // PCH):
                rsl = slice(PCH * ch, PCH * (ch + 1))
                hb = (x_v[4 * s + t, rsl].astype(f32) + ao[rsl]).astype(bf16)
                hbuf[t, rsl] = hb
                h_v[4 * s + t, rsl] = hb
                hf = hb.astype(f32)
                if piv is None:
                    piv = hf[0:1, :]
                dd = hf - piv
                a1 = jnp.sum(dd.reshape(PCH // 8, 8, 128), axis=0)
                a2 = jnp.sum((dd * dd).reshape(PCH // 8, 8, 128), axis=0)
                s1 = a1 if s1 is None else s1 + a1
                s2 = a2 if s2 is None else s2 + a2
            e1 = jnp.sum(s1, axis=0, keepdims=True) * (1.0 / D)
            e2 = jnp.sum(s2, axis=0, keepdims=True) * (1.0 / D)
            var = jnp.maximum(e2 - e1 * e1, 0.0)
            st[t, 0:1, :] = piv + e1
            st[t, 1:2, :] = lax.rsqrt(var + EPS)
            layer_norm_tile(sn, t)
        return c

    lax.fori_loop(0, NSEG, segment, 0)
    for t in range(4):
        for ch in range(NPC):
            post_piece(NSEG - 1, t, ch, None)
    for u in range(4):
        o_cp[4 * (NSEG - 1) + u].start()

    bv = best[0]
    bi = best[1]
    vmax = jnp.max(bv, axis=1, keepdims=True)
    cand = jnp.where(bv == vmax, bi, float(S))
    imin = jnp.min(cand, axis=1, keepdims=True)
    idx = jnp.minimum(jnp.max(imin).astype(i32), S - 1)
    tile = idx // 128
    col = idx - tile * 128
    col16 = pl.multiple_of((col // 16) * 16, 16)
    hn_t = hn_v[tile]
    lane_sel = _iota((D, 128), 1) == col
    xs_t = jnp.where(lane_sel, hn_t, jnp.zeros_like(hn_t))
    xs_t = jnp.concatenate([xs_t, jnp.zeros((DP - D, 128), bf16)], axis=0)
    pb0[0:64, :] = jnp.zeros((64, 128), u32)
    xall = xs_t.T
    xn[0:64, 0:L] = _pack(xall[:, 0:L])
    pb0[0:64, :] = _pack(xall[:, L:DP])
    c8 = pl.multiple_of(col16 // 2, 8)
    xs = _unpack(jnp.concatenate([xn[pl.ds(c8, 8), 0:L], pb0[pl.ds(c8, 8), 0:64]], axis=1))
    wg_cp.wait()
    wu_cp.wait()
    gt = jnp.dot(xs, wg_v[...], preferred_element_type=f32)
    up = jnp.dot(xs, wu_v[...], preferred_element_type=f32)
    act = (gt * _sigmoid(gt) * up).astype(bf16)
    wd_cp.wait()
    y = lax.dot_general(act, wd_v[...], NT, preferred_element_type=f32)
    rsel = _sigmoid(vmax[0:1, 0:1])
    yb = (y * rsel).astype(bf16)
    y128 = jnp.concatenate([_pad_lanes(yb), jnp.zeros((112, DP), bf16)], axis=0)
    yt = y128.T[0:D].astype(f32)
    ycol = jnp.sum(jnp.where(_iota((D, 128), 1) == (col - col16), yt, 0.0), axis=1, keepdims=True)
    fin = (h_v[tile].astype(f32)
           + (hn_t.astype(f32) + jnp.where(lane_sel, ycol, 0.0))).astype(bf16)
    for t in range(NTILE):
        o_cp[t].wait()
    out_v[tile] = fin
    pc = cp(out_v.at[tile], out_hbm.at[:, pl.ds(pl.multiple_of(tile * 128, 128), 128)], 15)
    pc.start()
    pc.wait()


@jax.jit
def pallas_sequential_preLN__memory_aug_infini_attn__moe_arch_mod__prompt_kernel(
    A_x: jax.Array,
    A_wq: jax.Array,
    A_wk: jax.Array,
    A_wv: jax.Array,
    A_wo: jax.Array,
    A_beta: jax.Array,
    B_x: jax.Array,
    B_w_r: jax.Array,
    B_w_gate: jax.Array,
    B_w_up: jax.Array,
    B_w_down: jax.Array,
):
    del B_x
    xt = A_x.reshape(S, D).T
    wdt = B_w_down.T
    beta = A_beta.reshape(1, H)
    wr = B_w_r
    hbm = pl.BlockSpec(memory_space=pltpu.HBM)
    vm = pl.BlockSpec(memory_space=pltpu.VMEM)
    V = pltpu.VMEM
    scratch = [
        V((NTILE, D, 128), bf16),
        V((D, D), bf16), V((D, D), bf16), V((D, D), bf16), V((D, D), bf16),
        V((D, F), bf16), V((D, F), bf16), V((D, F), bf16),
        V((3 * DC // 2, DP), u32),
        V((D // 2, DP), u32),
        V((D // 2, D), u32),
        V((DP // 2, D), u32),
        V((DP // 2, L), u32),
        V((NG, L // 2, 128), u32),
        V((NG, 64, L), u32),
        V((NG, 64, L), u32),
        V((NG, 64, L), u32),
        V((NG, 64, L), u32),
        V((NG, 128, L), f32),
        V((640, 128), u32), V((640, 128), u32),
        V((1280, 128), f32), V((1280, 128), f32),
        V((32, 128), f32), V((32, 128), f32),
        V((NG, 128, 128), f32),
        V((NG, 128, 128), u32),
        V((4, D, 128), bf16),
        V((4, 8, 128), f32),
        V((3, 8, 128), f32),
        V((8, 128), f32),
        V((NTILE, D, 128), bf16), V((NTILE, D, 128), bf16), V((NTILE, D, 128), bf16),
        V((7, 64, 128), u32),
        V((H, 32, 128), f32),
        V((NG, 128, 128), f32),
        V((D, 128), f32),
        V((2, 8, 128), f32),
        V((1, H), bf16), V((D,), bf16),
        pltpu.SemaphoreType.DMA((18,)),
    ]
    out_t = pl.pallas_call(
        _kernel,
        out_shape=jax.ShapeDtypeStruct((D, S), bf16),
        grid=(1,),
        in_specs=[hbm] * 10,
        out_specs=hbm,
        scratch_shapes=scratch,
        compiler_params=pltpu.CompilerParams(vmem_limit_bytes=100 * 1024 * 1024),
    )(xt, A_wq, A_wk, A_wv, A_wo, beta, wr, B_w_gate, B_w_up, wdt)
    return out_t.T.reshape(1, S, D)
```

```python
import jax
import jax.numpy as jnp
from jax import lax
import jax.experimental.pallas as pl
import jax.experimental.pallas.tpu as pltpu

u32 = jnp.uint32
f32 = jnp.float32
bf16 = jnp.bfloat16
i32 = jnp.int32

S = 2048
D = 576
DP = 640
DC = 592
F = 4608
NSEG = 4
L = 512
NTILE = S // 128
H = 32
DH = 18
NG = 5
OFF = (0, 128, 384, 768)
LOG2E = 1.4426950408889634
QSCALE = float(DH ** (-0.5)) * LOG2E
EPS = 1e-05
BOUND = 30.0
VBOUND = 1e20
NT = (((1,), (1,)), ((), ()))
UN_FAST = 8
UN_SLOW = 2
POST_AT = 0
GCH = 1
DEP = True
PSTART = 0
PPS = 1
PSP = 1.0
PCH = 64


def _unpack(x):
    return pltpu.bitcast(x, bf16)


def _pack(x):
    return pltpu.bitcast(x, u32)


def _iota(shape, dim):
    return lax.broadcasted_iota(i32, shape, dim)


def _perm_rows(w, tail):
    c = w.shape[1]
    parts = []
    for g in range(NG):
        if g < NG - 1:
            parts += [w[63 * g:63 * g + 63], jnp.zeros((1, c), u32)]
        else:
            parts += [w[252:288], jnp.zeros((tail - 36, c), u32)]
    return jnp.concatenate(parts, axis=0)


def _pad_lanes(x):
    return jnp.concatenate([x, jnp.zeros((x.shape[0], DP - D), x.dtype)], axis=1)


def _layernorm_t(xf):
    m = jnp.sum(xf, axis=0, keepdims=True) * (1.0 / D)
    xc = xf - m
    v = jnp.sum(xc * xc, axis=0, keepdims=True) * (1.0 / D)
    return xc * lax.rsqrt(v + EPS)


def _phi(t):
    return jnp.where(t > 0, t + 1.0, jnp.exp2(t * LOG2E))


def _sigmoid(t):
    return 1.0 / (1.0 + jnp.exp(-t))


def _absmax(x):
    return jnp.max(jnp.max(jnp.abs(x), axis=0, keepdims=True), axis=1, keepdims=True)


def _kernel(x_hbm, wq_hbm, wk_hbm, wv_hbm, wo_hbm, beta_hbm, wr_hbm, wg_hbm, wu_hbm, wd_hbm,
            out_hbm,
            x_v, wq_v, wk_v, wv_v, wo_v, wg_v, wu_v, wd_v,
            wall, wot, wtmp, wtmp2, xn, kp, phk, qt, phq, vt, ot, pb0, pb1, sb0, sb1, mb0, mb1,
            mt, mlhs, hbuf, st, mxs, racc, h_v, hn_v, out_v, msk, omg, grow, wcol, best, beta_ref, wr_ref, sems):

    def cp(src, dst, i):
        return pltpu.make_async_copy(src, dst, sems.at[i])

    x_cp = [cp(x_hbm.at[:, pl.ds(128 * t, 128)], x_v.at[t], t // 4) for t in range(NTILE)]
    wq_cp, wk_cp, wv_cp, wo_cp = (cp(wq_hbm, wq_v, 4), cp(wk_hbm, wk_v, 5),
                                  cp(wv_hbm, wv_v, 6), cp(wo_hbm, wo_v, 7))
    wg_cp, wu_cp, wd_cp = cp(wg_hbm, wg_v, 8), cp(wu_hbm, wu_v, 9), cp(wd_hbm, wd_v, 10)
    o_cp = [cp(out_v.at[t], out_hbm.at[:, pl.ds(128 * t, 128)], 11 + t // 4) for t in range(NTILE)]

    beta_cp = cp(beta_hbm, beta_ref, 16)
    wr_cp = cp(wr_hbm, wr_ref, 17)
    beta_cp.start()
    wr_cp.start()
    for t in range(4):
        x_cp[t].start()
    wq_cp.start()

    lane128 = _iota((128, 128), 1)
    row128 = _iota((128, 128), 0)
    head_in_group = lax.shift_right_logical(row128 * 57, 10)
    head_col = lax.shift_right_logical(lane128 * 57, 10)
    bd_mask = (head_in_group == head_col) & (head_in_group < 7)

    def tok_of(v):
        return pltpu.bitcast(v[0:8, 0:128], u32)

    def p_masks():
        r64 = _iota((64, 128), 0)
        for j in range(7):
            msk[j] = jnp.where((r64 >= 9 * j) & (r64 < 9 * j + 9), u32(0xFFFFFFFF), u32(0))
        best[0] = jnp.full((8, 128), -jnp.inf, f32)
        best[1] = jnp.zeros((8, 128), f32)
        return None

    def p_zero_mt():
        mt[...] = jnp.zeros((NG, 128, 128), f32)
        return None

    def p_zero_h(t):
        def f():
            hbuf[t] = jnp.zeros((D, 128), bf16)
            return None
        return f

    def p_gate(part):
        def f():
            g_lane = _sigmoid(beta_ref[...].astype(f32))
            g_lane = jnp.concatenate([g_lane, jnp.zeros((1, 128 - H), f32)], axis=1)
            if part < NG:
                g = part
                hid = jnp.where(head_in_group < 7, head_in_group + 7 * g, 999)
                sel = jnp.where(lane128 == hid, jnp.broadcast_to(g_lane, (128, 128)), 0.0)
                v = jnp.broadcast_to(jnp.sum(sel, axis=1, keepdims=True), (128, 128))
                grow[g] = v
                return tok_of(v)
            r32 = _iota((32, 128), 0)
            tk = None
            for h in range(8 * (part - NG), 8 * (part - NG) + 8):
                j = h % 7
                off = 18 * j - 16 * ((9 * j) // 8)
                gh = jnp.broadcast_to(g_lane[:, h:h + 1], (32, 128))
                v = jnp.where((r32 >= off) & (r32 < off + 18), 1.0 - gh, 0.0)
                omg[h] = v
                tk = tok_of(v) if tk is None else tk | tok_of(v)
            return tk
        return f

    def p_wcol():
        wr = _pad_lanes(wr_ref[...].astype(f32).reshape(1, D))
        v = jnp.broadcast_to(wr, (128, DP)).T[0:D]
        wcol[...] = v
        return tok_of(v)

    def p_tr(w_ref, c):
        def f():
            wd_ = min(128, D - 128 * c)
            v = _pack(w_ref[:, 128 * c:128 * c + wd_].T)
            wtmp[64 * c:64 * c + wd_ // 2, :] = v
            return v[0:8, 0:128]
        return f

    def p_perm(w):
        def f():
            v = _pad_lanes(_perm_rows(wtmp[...], 40))
            wall[296 * w:296 * (w + 1), :] = v
            return v[0:8, 0:128] | v[288:296, 0:128]
        return f

    def p_wo_perm():
        v = _perm_rows(_pack(wo_v[...]), 64)
        wtmp2[...] = v
        return v[0:8, 0:128]

    def p_wo_tr(c):
        def f():
            wd_ = min(128, D - 128 * c)
            v = _pack(_unpack(wtmp2[:, 128 * c:128 * c + wd_]).T)
            wot[64 * c:64 * c + wd_ // 2, :] = v
            return v[0:8, 0:128]
        return f

    def p_wait(*cs):
        def f():
            for c_ in cs:
                c_()
            return None
        return f

    def layer_norm_tile(seg, t):
        xf = x_v[4 * seg + t].astype(f32)
        xn[0:288, 128 * t:128 * (t + 1)] = _pack(_layernorm_t(xf).astype(bf16))

    wk_cp.start()
    xn[288:320, :] = jnp.zeros((32, L), u32)
    for ref in (qt, phq, phk, vt):
        ref[NG - 1, 40:64] = jnp.zeros((24, L), u32)
    for u in range(4):
        x_cp[u].wait()
    wv_cp.start()
    layer_norm_tile(0, 0)
    wq_cp.wait()
    wo_cp.start()
    for c in range(NG):
        p_tr(wq_v, c)()
    p_perm(0)()
    for t in range(1, 4):
        layer_norm_tile(0, t)

    diag = _iota((128, 128), 0) <= _iota((128, 128), 1)

    def qk_logits(h, i):
        g, j = h // 7, h % 7
        n = 128 * (i + 1)
        qw = qt[g, :, 128 * i:128 * (i + 1)] & msk[j]
        s = jnp.dot(_unpack(kp[g, 0:n // 2, :]), _unpack(qw), preferred_element_type=f32)
        sl = jnp.where(diag, s[n - 128:], -1e30)
        return sl if i == 0 else jnp.concatenate([s[:n - 128], sl], axis=0)

    def pv(h, i, pb):
        g, j = h // 7, h % 7
        n = 128 * (i + 1)
        a8 = pl.multiple_of(((9 * j) // 8) * 8, 8)
        vw = vt[g, pl.ds(a8, 16), 0:n]
        mk = msk[j, pl.ds(a8, 16), :]
        mk = jnp.concatenate([mk] * (i + 1), axis=1)
        vw = (vw & mk) | (jnp.full((16, n), 0x3F803F80, u32) & ~mk)
        o = jnp.dot(_unpack(vw), pb, preferred_element_type=f32)
        og = omg[h]
        r32_ = _iota((32, 128), 0)
        off = 18 * j - 2 * a8
        is_head = (r32_ >= off) & (r32_ < off + 18)
        lsum = jnp.sum(jnp.where(is_head, 0.0, o), axis=0, keepdims=True)
        r = pl.reciprocal(lsum, approx=True) * 14.0
        w16 = pl.multiple_of(a8 * 2, 16)
        ot[g, pl.ds(w16, 32), 128 * i:128 * (i + 1)] += o * (r * og)

    pbs = (pb0, pb1)
    sbs = (sb0, sb1)
    mbs = (mb0, mb1)
    IORD = (3, 2, 1, 0)

    def fast_qk(h, i, pbuf):
        g, j = h // 7, h % 7
        a = (9 * j) // 8
        n = 128 * (i + 1)
        qw = qt[g, 8 * a:8 * a + 16, 128 * i:128 * (i + 1)] & msk[j, 8 * a:8 * a + 16, :]
        parts = [jnp.zeros((8 * a, 128), u32)] if a > 0 else []
        parts.append(qw)
        if 48 - 8 * a > 0:
            parts.append(jnp.zeros((48 - 8 * a, 128), u32))
        qm = _unpack(jnp.concatenate(parts, axis=0))
        s = jnp.dot(_unpack(kp[g, 0:n // 2, :]), qm, preferred_element_type=f32)
        sl = jnp.where(diag, s[n - 128:], -1e30)
        s = sl if i == 0 else jnp.concatenate([s[:n - 128], sl], axis=0)
        pbuf[OFF[i] // 2:(OFF[i] + n) // 2, :] = _pack(jnp.exp2(s).astype(bf16))

    def fast_pv(h, i, pbuf):
        g, j = h // 7, h % 7
        a = (9 * j) // 8
        n = 128 * (i + 1)
        pb = _unpack(pbuf[OFF[i] // 2:(OFF[i] + n) // 2, :])
        mk = msk[j, 8 * a:8 * a + 16, :]
        mk = jnp.concatenate([mk] * (i + 1), axis=1)
        vw = (vt[g, 8 * a:8 * a + 16, 0:n] & mk) | (jnp.full((16, n), 0x3F803F80, u32) & ~mk)
        o = jnp.dot(_unpack(vw), pb, preferred_element_type=f32)
        off = 18 * j - 16 * a
        l8 = o[24:32] if off <= 6 else o[0:8]
        r = pl.reciprocal(l8, approx=True)
        for t in range(4):
            if 8 * t + 8 <= off or 8 * t >= off + 18:
                continue
            rs_ = slice(16 * a + 8 * t, 16 * a + 8 * t + 8)
            cs = slice(128 * i, 128 * (i + 1))
            ot[g, rs_, cs] += o[8 * t:8 * t + 8] * (r * omg[h, 8 * t:8 * t + 8, :])

    def slow_qk(h, i, sbuf, mbuf):
        n = 128 * (i + 1)
        s = qk_logits(h, i)
        sbuf[OFF[i]:OFF[i] + n, :] = s
        mbuf[8 * i:8 * i + 8, :] = jnp.broadcast_to(jnp.max(s, axis=0, keepdims=True), (8, 128))

    def slow_pv(h, i, sbuf, mbuf):
        n = 128 * (i + 1)
        s = sbuf[OFF[i]:OFF[i] + n, :]
        p = jnp.exp2(s - mbuf[8 * i:8 * i + 1, :]).astype(bf16)
        pv(h, i, p)

    def attention_fast():
        for i in IORD:
            fast_qk(0, i, pbs[0])
        for h in range(H):
            if h + 1 < H:
                for i in IORD:
                    fast_qk(h + 1, i, pbs[(h + 1) % 2])
            for i in IORD:
                fast_pv(h, i, pbs[h % 2])

    def attention_slow():
        for i in IORD:
            slow_qk(0, i, sbs[0], mbs[0])

        def body(it, c):
            for u in range(UN_SLOW):
                h = it * UN_SLOW + u
                hn_ = jnp.minimum(h + 1, H - 1)
                for i in IORD:
                    slow_qk(hn_, i, sbs[1 - u % 2], mbs[1 - u % 2])
                for i in IORD:
                    slow_pv(h, i, sbs[u % 2], mbs[u % 2])
            return c
        lax.fori_loop(0, H // UN_SLOW, body, 0)

    def wait_x(seg):
        for t in range(NSEG):
            @pl.when(seg == t)
            def _():
                for u in range(4):
                    x_cp[4 * t + u].wait()

    NPC = D // PCH

    def post_piece(seg, t, ch, valid):
        m = st[t, 0:1, :]
        rs = st[t, 1:2, :]
        rsl = slice(PCH * ch, PCH * (ch + 1))
        hf = hbuf[t, rsl].astype(f32)
        hnb = ((hf - m) * rs).astype(bf16)
        hnf = hnb.astype(f32)
        hn_v[4 * seg + t, rsl] = hnb
        ob_ = (hf + hnf).astype(bf16)
        out_v[4 * seg + t, rsl] = ob_
        r_ = jnp.sum((hnf * wcol[rsl]).reshape(PCH // 8, 8, 128), axis=0)
        if ch > 0:
            r_ = r_ + racc[...]
        if ch < NPC - 1:
            racc[...] = r_
        else:
            bv = best[0]
            bi = best[1]
            lane = _iota((8, 128), 1).astype(f32)
            rr = jnp.sum(r_, axis=0, keepdims=True).astype(bf16).astype(f32)
            rt = jnp.broadcast_to(rr, (8, 128))
            upd_ = rt > bv
            if valid is not None:
                upd_ = jnp.logical_and(upd_, valid)
            best[0] = jnp.where(upd_, rt, bv)
            best[1] = jnp.where(upd_, lane + jnp.asarray(seg * L + 128 * t, i32).astype(f32), bi)
        return _pack(ob_[0:16]) | pltpu.bitcast(r_, u32)

    def start_out(seg):
        for t in range(NSEG):
            @pl.when(seg == t)
            def _():
                for u in range(4):
                    o_cp[4 * t + u].start()

    def post_p(seg, t, ch, valid):
        return lambda: post_piece(seg, t, ch, valid)

    def qkv_block(pieces, opaque):
        pieces = list(pieces)
        zero = jnp.full((8, 128), lax.shift_right_logical(opaque, 8), i32).astype(u32)
        tok = None
        for w in range(3):
            m_ = None
            for t in range(4):
                cs = slice(128 * t, 128 * (t + 1))
                xt_ = _unpack(xn[:, cs])
                for g in range(NG):
                    nr = 128 if g < NG - 1 else 80
                    while pieces and pieces[0][0] is not None and pieces[0][0] <= (w * 4 + t) * NG + g - 1e-9:
                        tk = pieces.pop(0)[1]()
                        if tk is not None:
                            tok = tk if tok is None else tok | tk
                    r0_ = DC * w + 128 * g
                    lhs = wall[r0_ // 2:(r0_ + nr) // 2, :]
                    if tok is not None:
                        head = lhs[0:8, 0:128] | (tok & zero)
                        lhs = jnp.concatenate([
                            jnp.concatenate([head, lhs[0:8, 128:]], axis=1), lhs[8:]], axis=0)
                        tok = None
                    a = jnp.dot(_unpack(lhs), xt_, preferred_element_type=f32)
                    if w == 0:
                        phq[g, 0:nr // 2, cs] = _pack(_phi(a).astype(bf16))
                        a = a * QSCALE
                        qt[g, 0:nr // 2, cs] = _pack(a.astype(bf16))
                    elif w == 1:
                        phk[g, 0:nr // 2, cs] = _pack(_phi(a).astype(bf16))
                        ab = a.astype(bf16)
                        if nr < 128:
                            ab = jnp.concatenate([ab, jnp.zeros((128 - nr, 128), bf16)], axis=0)
                        kp[g, 64 * t:64 * (t + 1), :] = _pack(ab.T)
                    else:
                        vt[g, 0:nr // 2, cs] = _pack(a.astype(bf16))
                    am = jnp.max(jnp.abs(a).reshape(nr // 8, 8, 128), axis=0)
                    m_ = am if m_ is None else jnp.maximum(m_, am)
            mxs[w] = m_
        assert not pieces

    p0 = []
    p0.append((0.5, p_wait(wk_cp.wait, *[x_cp[t].start for t in range(4, NTILE)])))
    for c in range(NG):
        p0.append((1 + c, p_tr(wk_v, c)))
    p0.append((7, p_perm(1)))
    p0.append((8.5, p_wait(wv_cp.wait)))
    for c in range(NG):
        p0.append((9 + c, p_tr(wv_v, c)))
    p0.append((15, p_perm(2)))
    p0.append((16.5, p_wait(wo_cp.wait, wg_cp.start, wu_cp.start, wd_cp.start, beta_cp.wait, wr_cp.wait)))
    p0.append((17, p_wo_perm))
    for c in range(NG):
        p0.append((19 + c, p_wo_tr(c)))
    p0.append((25, p_masks))
    p0.append((26, p_zero_mt))
    for part in range(NG + 4):
        p0.append((28 + 2 * part, p_gate(part)))
    p0.append((47, p_wcol))
    def p_zero_ot(g):
        def f():
            ot[g] = jnp.zeros((128, L), f32)
            return None
        return f
    for g in range(NG):
        p0.append((49 + 2 * g, p_zero_ot(g)))
    qkv_block(p0, jnp.int32(0) if False else pl.program_id(0))

    def segment(s, c):
        @pl.when(s > 0)
        def _():
            sp = s - 1
            r64_ = _iota((64, L), 0)
            ones = jnp.full((64, L), 0x3F803F80, u32)
            for g in range(NG):
                lhs = jnp.where(r64_ == 63, ones, vt[g])
                upd = lax.dot_general(_unpack(lhs), _unpack(phk[g]), NT,
                                      preferred_element_type=f32)
                cur = mt[g] + upd
                mt[g] = cur
                m_bd = jnp.where(bd_mask, cur, 0.0)
                z_bd = jnp.where(bd_mask, jnp.broadcast_to(cur[126:127, :], (128, 128)), 0.0)
                mlhs[g] = _pack(jnp.concatenate([m_bd, z_bd], axis=0).astype(bf16))
            qkv_block([(0.5 + PSP * (t * NPC + ch), post_p(sp, t, ch, None))
                       for t in range(4) for ch in range(NPC)], s)
            for g in range(NG):
                nr = 128 if g < NG - 1 else 80
                lhs = jnp.concatenate([mlhs[g, 0:nr // 2], mlhs[g, 64:64 + nr // 2]], axis=0)
                nd = jnp.dot(_unpack(lhs), _unpack(phq[g]), preferred_element_type=f32)
                num = nd[0:nr]
                den = nd[nr:2 * nr] + 1e-06
                gr = grow[g, 0:nr]
                ot[g, 0:nr] = num * (pl.reciprocal(den, approx=True) * jnp.concatenate([gr] * 4, axis=1))
            start_out(sp)

        mxv = [_absmax(mxs[w]) for w in range(3)]
        bound = mxv[0] * mxv[1] * (DH * 1.02)
        ok = jnp.where((bound <= BOUND) & (mxv[2] <= VBOUND), 1, 0).astype(i32)
        safe = jnp.max(ok) > 0

        @pl.when(safe)
        def _():
            attention_fast()

        @pl.when(jnp.logical_not(safe))
        def _():
            attention_slow()

        @pl.when(s < NSEG - 1)
        def _():
            wait_x(s + 1)

        sn = jnp.minimum(s + 1, NSEG - 1)
        for t in range(4):
            cs = slice(128 * t, 128 * (t + 1))
            ob = jnp.concatenate([ot[g, :, cs] for g in range(NG)], axis=0).astype(bf16)
            ao = jnp.dot(_unpack(wot[...]), ob, preferred_element_type=f32)
            piv = s1 = s2 = None
            for ch in range(D // PCH):
                rsl = slice(PCH * ch, PCH * (ch + 1))
                hb = (x_v[4 * s + t, rsl].astype(f32) + ao[rsl]).astype(bf16)
                hbuf[t, rsl] = hb
                h_v[4 * s + t, rsl] = hb
                hf = hb.astype(f32)
                if piv is None:
                    piv = hf[0:1, :]
                dd = hf - piv
                a1 = jnp.sum(dd.reshape(PCH // 8, 8, 128), axis=0)
                a2 = jnp.sum((dd * dd).reshape(PCH // 8, 8, 128), axis=0)
                s1 = a1 if s1 is None else s1 + a1
                s2 = a2 if s2 is None else s2 + a2
            e1 = jnp.sum(s1, axis=0, keepdims=True) * (1.0 / D)
            e2 = jnp.sum(s2, axis=0, keepdims=True) * (1.0 / D)
            var = jnp.maximum(e2 - e1 * e1, 0.0)
            st[t, 0:1, :] = piv + e1
            st[t, 1:2, :] = lax.rsqrt(var + EPS)
            layer_norm_tile(sn, t)
        return c

    lax.fori_loop(0, NSEG, segment, 0)
    for t in range(4):
        for ch in range(NPC):
            post_piece(NSEG - 1, t, ch, None)
    for u in range(4):
        o_cp[4 * (NSEG - 1) + u].start()

    bv = best[0]
    bi = best[1]
    vmax = jnp.max(bv, axis=1, keepdims=True)
    cand = jnp.where(bv == vmax, bi, float(S))
    imin = jnp.min(cand, axis=1, keepdims=True)
    idx = jnp.minimum(jnp.max(imin).astype(i32), S - 1)
    tile = idx // 128
    col = idx - tile * 128
    col16 = pl.multiple_of((col // 16) * 16, 16)
    hn_t = hn_v[tile]
    lane_sel = _iota((D, 128), 1) == col
    xs_t = jnp.where(lane_sel, hn_t, jnp.zeros_like(hn_t))
    xs_t = jnp.concatenate([xs_t, jnp.zeros((DP - D, 128), bf16)], axis=0)
    pb0[0:64, :] = jnp.zeros((64, 128), u32)
    xall = xs_t.T
    xn[0:64, 0:L] = _pack(xall[:, 0:L])
    pb0[0:64, :] = _pack(xall[:, L:DP])
    c8 = pl.multiple_of(col16 // 2, 8)
    xs = _unpack(jnp.concatenate([xn[pl.ds(c8, 8), 0:L], pb0[pl.ds(c8, 8), 0:64]], axis=1))
    wg_cp.wait()
    wu_cp.wait()
    gt = jnp.dot(xs, wg_v[...], preferred_element_type=f32)
    up = jnp.dot(xs, wu_v[...], preferred_element_type=f32)
    act = (gt * _sigmoid(gt) * up).astype(bf16).astype(f32)
    act = jnp.broadcast_to(jnp.sum(act, axis=0, keepdims=True), (8, F))
    wd_cp.wait()
    cols = []
    RB = 64
    for rb in range(D // RB):
        acc = None
        for c in range(F // 128):
            wv_ = wd_v[RB * rb:RB * (rb + 1), 128 * c:128 * (c + 1)].astype(f32)
            pr = wv_.reshape(RB // 8, 8, 128) * act[None, :, 128 * c:128 * (c + 1)]
            acc = pr if acc is None else acc + pr
        cols.append(jnp.sum(acc.reshape(RB, 128), axis=1, keepdims=True))
    ycol = jnp.concatenate(cols, axis=0)
    rsel = _sigmoid(vmax[0:1, 0:1])
    ycol = (ycol.astype(bf16).astype(f32) * rsel).astype(bf16).astype(f32)
    fin = (h_v[tile].astype(f32)
           + (hn_t.astype(f32) + jnp.where(lane_sel, ycol, 0.0))).astype(bf16)
    for t in range(NTILE):
        o_cp[t].wait()
    out_v[tile] = fin
    pc = cp(out_v.at[tile], out_hbm.at[:, pl.ds(pl.multiple_of(tile * 128, 128), 128)], 15)
    pc.start()
    pc.wait()


@jax.jit
def pallas_sequential_preLN__memory_aug_infini_attn__moe_arch_mod__prompt_kernel(
    A_x: jax.Array,
    A_wq: jax.Array,
    A_wk: jax.Array,
    A_wv: jax.Array,
    A_wo: jax.Array,
    A_beta: jax.Array,
    B_x: jax.Array,
    B_w_r: jax.Array,
    B_w_gate: jax.Array,
    B_w_up: jax.Array,
    B_w_down: jax.Array,
):
    del B_x
    xt = A_x.reshape(S, D).T
    wdt = B_w_down.T
    beta = A_beta.reshape(1, H)
    wr = B_w_r
    hbm = pl.BlockSpec(memory_space=pltpu.HBM)
    vm = pl.BlockSpec(memory_space=pltpu.VMEM)
    V = pltpu.VMEM
    scratch = [
        V((NTILE, D, 128), bf16),
        V((D, D), bf16), V((D, D), bf16), V((D, D), bf16), V((D, D), bf16),
        V((D, F), bf16), V((D, F), bf16), V((D, F), bf16),
        V((3 * DC // 2, DP), u32),
        V((D // 2, DP), u32),
        V((D // 2, D), u32),
        V((DP // 2, D), u32),
        V((DP // 2, L), u32),
        V((NG, L // 2, 128), u32),
        V((NG, 64, L), u32),
        V((NG, 64, L), u32),
        V((NG, 64, L), u32),
        V((NG, 64, L), u32),
        V((NG, 128, L), f32),
        V((640, 128), u32), V((640, 128), u32),
        V((1280, 128), f32), V((1280, 128), f32),
        V((32, 128), f32), V((32, 128), f32),
        V((NG, 128, 128), f32),
        V((NG, 128, 128), u32),
        V((4, D, 128), bf16),
        V((4, 8, 128), f32),
        V((3, 8, 128), f32),
        V((8, 128), f32),
        V((NTILE, D, 128), bf16), V((NTILE, D, 128), bf16), V((NTILE, D, 128), bf16),
        V((7, 64, 128), u32),
        V((H, 32, 128), f32),
        V((NG, 128, 128), f32),
        V((D, 128), f32),
        V((2, 8, 128), f32),
        V((1, H), bf16), V((D,), bf16),
        pltpu.SemaphoreType.DMA((18,)),
    ]
    out_t = pl.pallas_call(
        _kernel,
        out_shape=jax.ShapeDtypeStruct((D, S), bf16),
        grid=(1,),
        in_specs=[hbm] * 10,
        out_specs=hbm,
        scratch_shapes=scratch,
        compiler_params=pltpu.CompilerParams(vmem_limit_bytes=100 * 1024 * 1024),
    )(xt, A_wq, A_wk, A_wv, A_wo, beta, wr, B_w_gate, B_w_up, wdt)
    return out_t.T.reshape(1, S, D)
```

```python
import jax
import jax.numpy as jnp
from jax import lax
import jax.experimental.pallas as pl
import jax.experimental.pallas.tpu as pltpu

u32 = jnp.uint32
f32 = jnp.float32
bf16 = jnp.bfloat16
i32 = jnp.int32

S = 2048
D = 576
DP = 640
DC = 592
F = 4608
NSEG = 4
L = 512
NTILE = S // 128
H = 32
DH = 18
NG = 5
OFF = (0, 128, 384, 768)
LOG2E = 1.4426950408889634
QSCALE = float(DH ** (-0.5)) * LOG2E
EPS = 1e-05
BOUND = 30.0
VBOUND = 1e20
NT = (((1,), (1,)), ((), ()))
UN_FAST = 8
UN_SLOW = 2
POST_AT = 0
GCH = 1
DEP = True
PSTART = 0
PPS = 1
PSP = 1.0
PCH = 64


def _unpack(x):
    return pltpu.bitcast(x, bf16)


def _pack(x):
    return pltpu.bitcast(x, u32)


def _iota(shape, dim):
    return lax.broadcasted_iota(i32, shape, dim)


def _perm_rows(w, tail):
    c = w.shape[1]
    parts = []
    for g in range(NG):
        if g < NG - 1:
            parts += [w[63 * g:63 * g + 63], jnp.zeros((1, c), u32)]
        else:
            parts += [w[252:288], jnp.zeros((tail - 36, c), u32)]
    return jnp.concatenate(parts, axis=0)


def _pad_lanes(x):
    return jnp.concatenate([x, jnp.zeros((x.shape[0], DP - D), x.dtype)], axis=1)


def _layernorm_t(xf):
    m = jnp.sum(xf, axis=0, keepdims=True) * (1.0 / D)
    xc = xf - m
    v = jnp.sum(xc * xc, axis=0, keepdims=True) * (1.0 / D)
    return xc * lax.rsqrt(v + EPS)


def _phi(t):
    return jnp.where(t > 0, t + 1.0, jnp.exp2(t * LOG2E))


def _sigmoid(t):
    return 1.0 / (1.0 + jnp.exp(-t))


def _absmax(x):
    return jnp.max(jnp.max(jnp.abs(x), axis=0, keepdims=True), axis=1, keepdims=True)


def _kernel(x_hbm, wq_hbm, wk_hbm, wv_hbm, wo_hbm, beta_hbm, wr_hbm, wg_hbm, wu_hbm, wd_hbm,
            out_hbm,
            x_v, wq_v, wk_v, wv_v, wo_v, wg_v, wu_v, wd_v,
            wall, wot, wtmp, wtmp2, xn, kp, phk, qt, phq, vt, ot, pb0, pb1, sb0, sb1, mb0, mb1,
            mt, mlhs, hbuf, st, mxs, racc, h_v, hn_v, out_v, msk, omg, grow, wcol, best, beta_ref, wr_ref, sems):

    def cp(src, dst, i):
        return pltpu.make_async_copy(src, dst, sems.at[i])

    x_cp = [cp(x_hbm.at[:, pl.ds(128 * t, 128)], x_v.at[t], t // 4) for t in range(NTILE)]
    wq_cp, wk_cp, wv_cp, wo_cp = (cp(wq_hbm, wq_v, 4), cp(wk_hbm, wk_v, 5),
                                  cp(wv_hbm, wv_v, 6), cp(wo_hbm, wo_v, 7))
    wg_cp, wu_cp, wd_cp = cp(wg_hbm, wg_v, 8), cp(wu_hbm, wu_v, 9), cp(wd_hbm, wd_v, 10)
    o_cp = [cp(out_v.at[t], out_hbm.at[:, pl.ds(128 * t, 128)], 11 + t // 4) for t in range(NTILE)]

    beta_cp = cp(beta_hbm, beta_ref, 16)
    wr_cp = cp(wr_hbm, wr_ref, 17)
    beta_cp.start()
    wr_cp.start()
    for t in range(4):
        x_cp[t].start()
    wq_cp.start()

    lane128 = _iota((128, 128), 1)
    row128 = _iota((128, 128), 0)
    head_in_group = lax.shift_right_logical(row128 * 57, 10)
    head_col = lax.shift_right_logical(lane128 * 57, 10)
    bd_mask = (head_in_group == head_col) & (head_in_group < 7)

    def tok_of(v):
        return pltpu.bitcast(v[0:8, 0:128], u32)

    def p_masks():
        r64 = _iota((64, 128), 0)
        for j in range(7):
            msk[j] = jnp.where((r64 >= 9 * j) & (r64 < 9 * j + 9), u32(0xFFFFFFFF), u32(0))
        best[0] = jnp.full((8, 128), -jnp.inf, f32)
        best[1] = jnp.zeros((8, 128), f32)
        return None

    def p_zero_mt():
        mt[...] = jnp.zeros((NG, 128, 128), f32)
        return None

    def p_zero_h(t):
        def f():
            hbuf[t] = jnp.zeros((D, 128), bf16)
            return None
        return f

    def p_gate(part):
        def f():
            g_lane = _sigmoid(beta_ref[...].astype(f32))
            g_lane = jnp.concatenate([g_lane, jnp.zeros((1, 128 - H), f32)], axis=1)
            if part < NG:
                g = part
                hid = jnp.where(head_in_group < 7, head_in_group + 7 * g, 999)
                sel = jnp.where(lane128 == hid, jnp.broadcast_to(g_lane, (128, 128)), 0.0)
                v = jnp.broadcast_to(jnp.sum(sel, axis=1, keepdims=True), (128, 128))
                grow[g] = v
                return tok_of(v)
            r32 = _iota((32, 128), 0)
            tk = None
            for h in range(8 * (part - NG), 8 * (part - NG) + 8):
                j = h % 7
                off = 18 * j - 16 * ((9 * j) // 8)
                gh = jnp.broadcast_to(g_lane[:, h:h + 1], (32, 128))
                v = jnp.where((r32 >= off) & (r32 < off + 18), 1.0 - gh, 0.0)
                omg[h] = v
                tk = tok_of(v) if tk is None else tk | tok_of(v)
            return tk
        return f

    def p_wcol():
        wr = _pad_lanes(wr_ref[...].astype(f32).reshape(1, D))
        v = jnp.broadcast_to(wr, (128, DP)).T[0:D]
        wcol[...] = v
        return tok_of(v)

    def p_tr(w_ref, c):
        def f():
            wd_ = min(128, D - 128 * c)
            v = _pack(w_ref[:, 128 * c:128 * c + wd_].T)
            wtmp[64 * c:64 * c + wd_ // 2, :] = v
            return v[0:8, 0:128]
        return f

    def p_perm(w):
        def f():
            v = _pad_lanes(_perm_rows(wtmp[...], 40))
            wall[296 * w:296 * (w + 1), :] = v
            return v[0:8, 0:128] | v[288:296, 0:128]
        return f

    def p_wo_perm():
        v = _perm_rows(_pack(wo_v[...]), 64)
        wtmp2[...] = v
        return v[0:8, 0:128]

    def p_wo_tr(c):
        def f():
            wd_ = min(128, D - 128 * c)
            v = _pack(_unpack(wtmp2[:, 128 * c:128 * c + wd_]).T)
            wot[64 * c:64 * c + wd_ // 2, :] = v
            return v[0:8, 0:128]
        return f

    def p_wait(*cs):
        def f():
            for c_ in cs:
                c_()
            return None
        return f

    def layer_norm_tile(seg, t):
        xf = x_v[4 * seg + t].astype(f32)
        v = _pack(_layernorm_t(xf).astype(bf16))
        xn[0:288, 128 * t:128 * (t + 1)] = v
        return v[0:8] | v[280:288]

    wk_cp.start()
    xn[288:320, :] = jnp.zeros((32, L), u32)
    for ref in (qt, phq, phk, vt):
        ref[NG - 1, 40:64] = jnp.zeros((24, L), u32)
    for u in range(4):
        x_cp[u].wait()
    wv_cp.start()
    layer_norm_tile(0, 0)
    wq_cp.wait()
    wo_cp.start()
    for c in range(NG):
        p_tr(wq_v, c)()
    p_perm(0)()
    for t in range(1, 4):
        layer_norm_tile(0, t)

    diag = _iota((128, 128), 0) <= _iota((128, 128), 1)

    def qk_logits(h, i):
        g, j = h // 7, h % 7
        n = 128 * (i + 1)
        qw = qt[g, :, 128 * i:128 * (i + 1)] & msk[j]
        s = jnp.dot(_unpack(kp[g, 0:n // 2, :]), _unpack(qw), preferred_element_type=f32)
        sl = jnp.where(diag, s[n - 128:], -1e30)
        return sl if i == 0 else jnp.concatenate([s[:n - 128], sl], axis=0)

    def pv(h, i, pb):
        g, j = h // 7, h % 7
        n = 128 * (i + 1)
        a8 = pl.multiple_of(((9 * j) // 8) * 8, 8)
        vw = vt[g, pl.ds(a8, 16), 0:n]
        mk = msk[j, pl.ds(a8, 16), :]
        mk = jnp.concatenate([mk] * (i + 1), axis=1)
        vw = (vw & mk) | (jnp.full((16, n), 0x3F803F80, u32) & ~mk)
        o = jnp.dot(_unpack(vw), pb, preferred_element_type=f32)
        og = omg[h]
        r32_ = _iota((32, 128), 0)
        off = 18 * j - 2 * a8
        is_head = (r32_ >= off) & (r32_ < off + 18)
        lsum = jnp.sum(jnp.where(is_head, 0.0, o), axis=0, keepdims=True)
        r = pl.reciprocal(lsum, approx=True) * 14.0
        w16 = pl.multiple_of(a8 * 2, 16)
        ot[g, pl.ds(w16, 32), 128 * i:128 * (i + 1)] += o * (r * og)

    pbs = (pb0, pb1)
    sbs = (sb0, sb1)
    mbs = (mb0, mb1)
    IORD = (3, 2, 1, 0)

    def fast_qk(h, i, pbuf):
        g, j = h // 7, h % 7
        a = (9 * j) // 8
        n = 128 * (i + 1)
        qw = qt[g, 8 * a:8 * a + 16, 128 * i:128 * (i + 1)] & msk[j, 8 * a:8 * a + 16, :]
        parts = [jnp.zeros((8 * a, 128), u32)] if a > 0 else []
        parts.append(qw)
        if 48 - 8 * a > 0:
            parts.append(jnp.zeros((48 - 8 * a, 128), u32))
        qm = _unpack(jnp.concatenate(parts, axis=0))
        s = jnp.dot(_unpack(kp[g, 0:n // 2, :]), qm, preferred_element_type=f32)
        sl = jnp.where(diag, s[n - 128:], -1e30)
        s = sl if i == 0 else jnp.concatenate([s[:n - 128], sl], axis=0)
        pbuf[OFF[i] // 2:(OFF[i] + n) // 2, :] = _pack(jnp.exp2(s).astype(bf16))

    def fast_pv(h, i, pbuf):
        g, j = h // 7, h % 7
        a = (9 * j) // 8
        n = 128 * (i + 1)
        pb = _unpack(pbuf[OFF[i] // 2:(OFF[i] + n) // 2, :])
        mk = msk[j, 8 * a:8 * a + 16, :]
        mk = jnp.concatenate([mk] * (i + 1), axis=1)
        vw = (vt[g, 8 * a:8 * a + 16, 0:n] & mk) | (jnp.full((16, n), 0x3F803F80, u32) & ~mk)
        o = jnp.dot(_unpack(vw), pb, preferred_element_type=f32)
        off = 18 * j - 16 * a
        l8 = o[24:32] if off <= 6 else o[0:8]
        r = pl.reciprocal(l8, approx=True)
        for t in range(4):
            if 8 * t + 8 <= off or 8 * t >= off + 18:
                continue
            rs_ = slice(16 * a + 8 * t, 16 * a + 8 * t + 8)
            cs = slice(128 * i, 128 * (i + 1))
            ot[g, rs_, cs] += o[8 * t:8 * t + 8] * (r * omg[h, 8 * t:8 * t + 8, :])

    def slow_qk(h, i, sbuf, mbuf):
        n = 128 * (i + 1)
        s = qk_logits(h, i)
        sbuf[OFF[i]:OFF[i] + n, :] = s
        mbuf[8 * i:8 * i + 8, :] = jnp.broadcast_to(jnp.max(s, axis=0, keepdims=True), (8, 128))

    def slow_pv(h, i, sbuf, mbuf):
        n = 128 * (i + 1)
        s = sbuf[OFF[i]:OFF[i] + n, :]
        p = jnp.exp2(s - mbuf[8 * i:8 * i + 1, :]).astype(bf16)
        pv(h, i, p)

    def attention_fast():
        for i in IORD:
            fast_qk(0, i, pbs[0])
        for h in range(H):
            if h + 1 < H:
                for i in IORD:
                    fast_qk(h + 1, i, pbs[(h + 1) % 2])
            for i in IORD:
                fast_pv(h, i, pbs[h % 2])

    def attention_slow():
        for i in IORD:
            slow_qk(0, i, sbs[0], mbs[0])

        def body(it, c):
            for u in range(UN_SLOW):
                h = it * UN_SLOW + u
                hn_ = jnp.minimum(h + 1, H - 1)
                for i in IORD:
                    slow_qk(hn_, i, sbs[1 - u % 2], mbs[1 - u % 2])
                for i in IORD:
                    slow_pv(h, i, sbs[u % 2], mbs[u % 2])
            return c
        lax.fori_loop(0, H // UN_SLOW, body, 0)

    def wait_x(seg):
        for t in range(NSEG):
            @pl.when(seg == t)
            def _():
                for u in range(4):
                    x_cp[4 * t + u].wait()

    NPC = D // PCH

    def post_piece(seg, t, ch, valid):
        m = st[t, 0:1, :]
        rs = st[t, 1:2, :]
        rsl = slice(PCH * ch, PCH * (ch + 1))
        hf = hbuf[t, rsl].astype(f32)
        hnb = ((hf - m) * rs).astype(bf16)
        hnf = hnb.astype(f32)
        hn_v[4 * seg + t, rsl] = hnb
        ob_ = (hf + hnf).astype(bf16)
        out_v[4 * seg + t, rsl] = ob_
        r_ = jnp.sum((hnf * wcol[rsl]).reshape(PCH // 8, 8, 128), axis=0)
        if ch > 0:
            r_ = r_ + racc[...]
        if ch < NPC - 1:
            racc[...] = r_
        else:
            bv = best[0]
            bi = best[1]
            lane = _iota((8, 128), 1).astype(f32)
            rr = jnp.sum(r_, axis=0, keepdims=True).astype(bf16).astype(f32)
            rt = jnp.broadcast_to(rr, (8, 128))
            upd_ = rt > bv
            if valid is not None:
                upd_ = jnp.logical_and(upd_, valid)
            best[0] = jnp.where(upd_, rt, bv)
            best[1] = jnp.where(upd_, lane + jnp.asarray(seg * L + 128 * t, i32).astype(f32), bi)
        return _pack(ob_[0:16]) | pltpu.bitcast(r_, u32)

    def start_out(seg):
        for t in range(NSEG):
            @pl.when(seg == t)
            def _():
                for u in range(4):
                    o_cp[4 * t + u].start()

    def post_p(seg, t, ch, valid):
        return lambda: post_piece(seg, t, ch, valid)

    def qkv_block(pieces, opaque):
        pieces = list(pieces)
        zero = jnp.full((8, 128), lax.shift_right_logical(opaque, 8), i32).astype(u32)
        tok = None
        for w in range(3):
            m_ = None
            for t in range(4):
                cs = slice(128 * t, 128 * (t + 1))
                xt_ = _unpack(xn[:, cs])
                for g in range(NG):
                    nr = 128 if g < NG - 1 else 80
                    while pieces and pieces[0][0] is not None and pieces[0][0] <= (w * 4 + t) * NG + g - 1e-9:
                        tk = pieces.pop(0)[1]()
                        if tk is not None:
                            tok = tk if tok is None else tok | tk
                    r0_ = DC * w + 128 * g
                    lhs = wall[r0_ // 2:(r0_ + nr) // 2, :]
                    if tok is not None:
                        head = lhs[0:8, 0:128] | (tok & zero)
                        lhs = jnp.concatenate([
                            jnp.concatenate([head, lhs[0:8, 128:]], axis=1), lhs[8:]], axis=0)
                        tok = None
                    a = jnp.dot(_unpack(lhs), xt_, preferred_element_type=f32)
                    if w == 0:
                        phq[g, 0:nr // 2, cs] = _pack(_phi(a).astype(bf16))
                        a = a * QSCALE
                        qt[g, 0:nr // 2, cs] = _pack(a.astype(bf16))
                    elif w == 1:
                        phk[g, 0:nr // 2, cs] = _pack(_phi(a).astype(bf16))
                        ab = a.astype(bf16)
                        if nr < 128:
                            ab = jnp.concatenate([ab, jnp.zeros((128 - nr, 128), bf16)], axis=0)
                        kp[g, 64 * t:64 * (t + 1), :] = _pack(ab.T)
                    else:
                        vt[g, 0:nr // 2, cs] = _pack(a.astype(bf16))
                    am = jnp.max(jnp.abs(a).reshape(nr // 8, 8, 128), axis=0)
                    m_ = am if m_ is None else jnp.maximum(m_, am)
            mxs[w] = m_
        assert not pieces

    p0 = []
    p0.append((0.5, p_wait(wk_cp.wait, *[x_cp[t].start for t in range(4, NTILE)])))
    for c in range(NG):
        p0.append((1 + c, p_tr(wk_v, c)))
    p0.append((7, p_perm(1)))
    p0.append((8.5, p_wait(wv_cp.wait)))
    for c in range(NG):
        p0.append((9 + c, p_tr(wv_v, c)))
    p0.append((15, p_perm(2)))
    p0.append((16.5, p_wait(wo_cp.wait, wg_cp.start, wu_cp.start, wd_cp.start, beta_cp.wait, wr_cp.wait)))
    p0.append((17, p_wo_perm))
    for c in range(NG):
        p0.append((19 + c, p_wo_tr(c)))
    p0.append((25, p_masks))
    p0.append((26, p_zero_mt))
    for part in range(NG + 4):
        p0.append((28 + 2 * part, p_gate(part)))
    p0.append((47, p_wcol))
    def p_zero_ot(g):
        def f():
            ot[g] = jnp.zeros((128, L), f32)
            return None
        return f
    for g in range(NG):
        p0.append((49 + 2 * g, p_zero_ot(g)))
    qkv_block(p0, jnp.int32(0) if False else pl.program_id(0))

    def segment(s, c):
        mxv = [_absmax(mxs[w]) for w in range(3)]
        bound = mxv[0] * mxv[1] * (DH * 1.02)
        ok = jnp.where((bound <= BOUND) & (mxv[2] <= VBOUND), 1, 0).astype(i32)
        safe = jnp.max(ok) > 0

        @pl.when(safe)
        def _():
            attention_fast()

        @pl.when(jnp.logical_not(safe))
        def _():
            attention_slow()

        def wo_tile(t, dep):
            cs = slice(128 * t, 128 * (t + 1))
            ob = jnp.concatenate([ot[g, :, cs] for g in range(NG)], axis=0).astype(bf16)
            lhs = wot[...]
            if dep is not None:
                lhs = jnp.concatenate([
                    jnp.concatenate([lhs[0:8, 0:128] | dep, lhs[0:8, 128:]], axis=1), lhs[8:]], axis=0)
            ao = jnp.dot(_unpack(lhs), ob, preferred_element_type=f32)
            piv = s1 = s2 = None
            for ch in range(D // PCH):
                rsl = slice(PCH * ch, PCH * (ch + 1))
                hb = (x_v[4 * s + t, rsl].astype(f32) + ao[rsl]).astype(bf16)
                hbuf[t, rsl] = hb
                h_v[4 * s + t, rsl] = hb
                hf = hb.astype(f32)
                if piv is None:
                    piv = hf[0:1, :]
                dd = hf - piv
                a1 = jnp.sum(dd.reshape(PCH // 8, 8, 128), axis=0)
                a2 = jnp.sum((dd * dd).reshape(PCH // 8, 8, 128), axis=0)
                s1 = a1 if s1 is None else s1 + a1
                s2 = a2 if s2 is None else s2 + a2
            e1 = jnp.sum(s1, axis=0, keepdims=True) * (1.0 / D)
            e2 = jnp.sum(s2, axis=0, keepdims=True) * (1.0 / D)
            var = jnp.maximum(e2 - e1 * e1, 0.0)
            st[t, 0:1, :] = piv + e1
            st[t, 1:2, :] = lax.rsqrt(var + EPS)

        zero = jnp.full((8, 128), lax.shift_right_logical(s, 8), i32).astype(u32)

        @pl.when(s < NSEG - 1)
        def _():
            wait_x(s + 1)
            r64_ = _iota((64, L), 0)
            ones = jnp.full((64, L), 0x3F803F80, u32)
            for g in range(NG):
                lhs = jnp.where(r64_ == 63, ones, vt[g])
                upd = lax.dot_general(_unpack(lhs), _unpack(phk[g]), NT,
                                      preferred_element_type=f32)
                cur = mt[g] + upd
                mt[g] = cur
                m_bd = jnp.where(bd_mask, cur, 0.0)
                z_bd = jnp.where(bd_mask, jnp.broadcast_to(cur[126:127, :], (128, 128)), 0.0)
                mlhs[g] = _pack(jnp.concatenate([m_bd, z_bd], axis=0).astype(bf16))
            dep = None
            for t in range(4):
                tk = layer_norm_tile(s + 1, t)
                wo_tile(t, dep)
                dep = tk & zero
            qkv_block([(0.5 + PSP * (t * NPC + ch), post_p(s, t, ch, None))
                       for t in range(4) for ch in range(NPC)], s)
            for g in range(NG):
                nr = 128 if g < NG - 1 else 80
                lhs = jnp.concatenate([mlhs[g, 0:nr // 2], mlhs[g, 64:64 + nr // 2]], axis=0)
                nd = jnp.dot(_unpack(lhs), _unpack(phq[g]), preferred_element_type=f32)
                num = nd[0:nr]
                den = nd[nr:2 * nr] + 1e-06
                gr = grow[g, 0:nr]
                ot[g, 0:nr] = num * (pl.reciprocal(den, approx=True) * jnp.concatenate([gr] * 4, axis=1))
            start_out(s)

        @pl.when(s == NSEG - 1)
        def _():
            dep = None
            for t in range(4):
                wo_tile(t, dep)
                dep = None
                if t > 0:
                    for ch in range(NPC):
                        tk = post_piece(s, t - 1, ch, None)
                        dep = tk if dep is None else dep | tk
                    dep = dep & zero
            for ch in range(NPC):
                post_piece(s, 3, ch, None)
        return c

    lax.fori_loop(0, NSEG, segment, 0)
    for u in range(4):
        o_cp[4 * (NSEG - 1) + u].start()

    bv = best[0]
    bi = best[1]
    vmax = jnp.max(bv, axis=1, keepdims=True)
    cand = jnp.where(bv == vmax, bi, float(S))
    imin = jnp.min(cand, axis=1, keepdims=True)
    idx = jnp.minimum(jnp.max(imin).astype(i32), S - 1)
    tile = idx // 128
    col = idx - tile * 128
    col16 = pl.multiple_of((col // 16) * 16, 16)
    hn_t = hn_v[tile]
    lane_sel = _iota((D, 128), 1) == col
    xs_t = jnp.where(lane_sel, hn_t, jnp.zeros_like(hn_t))
    xs_t = jnp.concatenate([xs_t, jnp.zeros((DP - D, 128), bf16)], axis=0)
    pb0[0:64, :] = jnp.zeros((64, 128), u32)
    xall = xs_t.T
    xn[0:64, 0:L] = _pack(xall[:, 0:L])
    pb0[0:64, :] = _pack(xall[:, L:DP])
    c8 = pl.multiple_of(col16 // 2, 8)
    xs = _unpack(jnp.concatenate([xn[pl.ds(c8, 8), 0:L], pb0[pl.ds(c8, 8), 0:64]], axis=1))
    wg_cp.wait()
    wu_cp.wait()
    gt = jnp.dot(xs, wg_v[...], preferred_element_type=f32)
    up = jnp.dot(xs, wu_v[...], preferred_element_type=f32)
    act = (gt * _sigmoid(gt) * up).astype(bf16).astype(f32)
    act = jnp.broadcast_to(jnp.sum(act, axis=0, keepdims=True), (8, F))
    wd_cp.wait()
    cols = []
    RB = 64
    for rb in range(D // RB):
        acc = None
        for c in range(F // 128):
            wv_ = wd_v[RB * rb:RB * (rb + 1), 128 * c:128 * (c + 1)].astype(f32)
            pr = wv_.reshape(RB // 8, 8, 128) * act[None, :, 128 * c:128 * (c + 1)]
            acc = pr if acc is None else acc + pr
        cols.append(jnp.sum(acc.reshape(RB, 128), axis=1, keepdims=True))
    ycol = jnp.concatenate(cols, axis=0)
    rsel = _sigmoid(vmax[0:1, 0:1])
    ycol = (ycol.astype(bf16).astype(f32) * rsel).astype(bf16).astype(f32)
    fin = (h_v[tile].astype(f32)
           + (hn_t.astype(f32) + jnp.where(lane_sel, ycol, 0.0))).astype(bf16)
    for t in range(NTILE):
        o_cp[t].wait()
    out_v[tile] = fin
    pc = cp(out_v.at[tile], out_hbm.at[:, pl.ds(pl.multiple_of(tile * 128, 128), 128)], 15)
    pc.start()
    pc.wait()


@jax.jit
def pallas_sequential_preLN__memory_aug_infini_attn__moe_arch_mod__prompt_kernel(
    A_x: jax.Array,
    A_wq: jax.Array,
    A_wk: jax.Array,
    A_wv: jax.Array,
    A_wo: jax.Array,
    A_beta: jax.Array,
    B_x: jax.Array,
    B_w_r: jax.Array,
    B_w_gate: jax.Array,
    B_w_up: jax.Array,
    B_w_down: jax.Array,
):
    del B_x
    xt = A_x.reshape(S, D).T
    wdt = B_w_down.T
    beta = A_beta.reshape(1, H)
    wr = B_w_r
    hbm = pl.BlockSpec(memory_space=pltpu.HBM)
    vm = pl.BlockSpec(memory_space=pltpu.VMEM)
    V = pltpu.VMEM
    scratch = [
        V((NTILE, D, 128), bf16),
        V((D, D), bf16), V((D, D), bf16), V((D, D), bf16), V((D, D), bf16),
        V((D, F), bf16), V((D, F), bf16), V((D, F), bf16),
        V((3 * DC // 2, DP), u32),
        V((D // 2, DP), u32),
        V((D // 2, D), u32),
        V((DP // 2, D), u32),
        V((DP // 2, L), u32),
        V((NG, L // 2, 128), u32),
        V((NG, 64, L), u32),
        V((NG, 64, L), u32),
        V((NG, 64, L), u32),
        V((NG, 64, L), u32),
        V((NG, 128, L), f32),
        V((640, 128), u32), V((640, 128), u32),
        V((1280, 128), f32), V((1280, 128), f32),
        V((32, 128), f32), V((32, 128), f32),
        V((NG, 128, 128), f32),
        V((NG, 128, 128), u32),
        V((4, D, 128), bf16),
        V((4, 8, 128), f32),
        V((3, 8, 128), f32),
        V((8, 128), f32),
        V((NTILE, D, 128), bf16), V((NTILE, D, 128), bf16), V((NTILE, D, 128), bf16),
        V((7, 64, 128), u32),
        V((H, 32, 128), f32),
        V((NG, 128, 128), f32),
        V((D, 128), f32),
        V((2, 8, 128), f32),
        V((1, H), bf16), V((D,), bf16),
        pltpu.SemaphoreType.DMA((18,)),
    ]
    out_t = pl.pallas_call(
        _kernel,
        out_shape=jax.ShapeDtypeStruct((D, S), bf16),
        grid=(1,),
        in_specs=[hbm] * 10,
        out_specs=hbm,
        scratch_shapes=scratch,
        compiler_params=pltpu.CompilerParams(vmem_limit_bytes=100 * 1024 * 1024),
    )(xt, A_wq, A_wk, A_wv, A_wo, beta, wr, B_w_gate, B_w_up, wdt)
    return out_t.T.reshape(1, S, D)
```

```python
import jax
import jax.numpy as jnp
from jax import lax
import jax.experimental.pallas as pl
import jax.experimental.pallas.tpu as pltpu

u32 = jnp.uint32
f32 = jnp.float32
bf16 = jnp.bfloat16
i32 = jnp.int32

S = 2048
D = 576
DP = 640
DC = 592
F = 4608
NSEG = 4
L = 512
NTILE = S // 128
H = 32
DH = 18
NG = 5
OFF = (0, 128, 384, 768)
LOG2E = 1.4426950408889634
QSCALE = float(DH ** (-0.5)) * LOG2E
EPS = 1e-05
BOUND = 30.0
VBOUND = 1e20
NT = (((1,), (1,)), ((), ()))
UN_SLOW = 2
PSP = 1.0
PST = 20.5
PCH = 64


def _unpack(x):
    return pltpu.bitcast(x, bf16)


def _pack(x):
    return pltpu.bitcast(x, u32)


def _iota(shape, dim):
    return lax.broadcasted_iota(i32, shape, dim)


def _perm_rows(w, tail):
    c = w.shape[1]
    parts = []
    for g in range(NG):
        if g < NG - 1:
            parts += [w[63 * g:63 * g + 63], jnp.zeros((1, c), u32)]
        else:
            parts += [w[252:288], jnp.zeros((tail - 36, c), u32)]
    return jnp.concatenate(parts, axis=0)


def _pad_lanes(x):
    return jnp.concatenate([x, jnp.zeros((x.shape[0], DP - D), x.dtype)], axis=1)


def _layernorm_t(xf):
    m = jnp.sum(xf, axis=0, keepdims=True) * (1.0 / D)
    xc = xf - m
    v = jnp.sum(xc * xc, axis=0, keepdims=True) * (1.0 / D)
    return xc * lax.rsqrt(v + EPS)


def _phi(t):
    return jnp.where(t > 0, t + 1.0, jnp.exp2(t * LOG2E))


def _sigmoid(t):
    return 1.0 / (1.0 + jnp.exp(-t))


def _absmax(x):
    return jnp.max(jnp.max(jnp.abs(x), axis=0, keepdims=True), axis=1, keepdims=True)


def _kernel(x_hbm, wq_hbm, wk_hbm, wv_hbm, wo_hbm, beta_hbm, wr_hbm, wg_hbm, wu_hbm, wd_hbm,
            out_hbm,
            x_v, wq_v, wk_v, wv_v, wo_v, wg_v, wu_v, wd_v,
            wall, wot, wtmp, wtmp2, xn, kp, phk, qt, phq, vt, ot, pb0, pb1, sb0, sb1, mb0, mb1,
            mt, mlhs, hbuf, st, mxs, racc, h_v, hn_v, out_v, msk, omg, grow, wcol, best, beta_ref, wr_ref, sems):

    def cp(src, dst, i):
        return pltpu.make_async_copy(src, dst, sems.at[i])

    x_cp = [cp(x_hbm.at[:, pl.ds(128 * t, 128)], x_v.at[t], t // 4) for t in range(NTILE)]
    wq_cp, wk_cp, wv_cp, wo_cp = (cp(wq_hbm, wq_v, 4), cp(wk_hbm, wk_v, 5),
                                  cp(wv_hbm, wv_v, 6), cp(wo_hbm, wo_v, 7))
    wg_cp, wu_cp, wd_cp = cp(wg_hbm, wg_v, 8), cp(wu_hbm, wu_v, 9), cp(wd_hbm, wd_v, 10)
    o_cp = [cp(out_v.at[t], out_hbm.at[:, pl.ds(128 * t, 128)], 11 + t // 4) for t in range(NTILE)]

    beta_cp = cp(beta_hbm, beta_ref, 16)
    wr_cp = cp(wr_hbm, wr_ref, 17)
    beta_cp.start()
    wr_cp.start()
    for t in range(4):
        x_cp[t].start()
    wq_cp.start()

    lane128 = _iota((128, 128), 1)
    row128 = _iota((128, 128), 0)
    head_in_group = lax.shift_right_logical(row128 * 57, 10)
    head_col = lax.shift_right_logical(lane128 * 57, 10)
    bd_mask = (head_in_group == head_col) & (head_in_group < 7)

    def tok_of(v):
        return pltpu.bitcast(v[0:8, 0:128], u32)

    def p_masks():
        r64 = _iota((64, 128), 0)
        for j in range(7):
            msk[j] = jnp.where((r64 >= 9 * j) & (r64 < 9 * j + 9), u32(0xFFFFFFFF), u32(0))
        best[0] = jnp.full((8, 128), -jnp.inf, f32)
        best[1] = jnp.zeros((8, 128), f32)
        return None

    def p_zero_mt():
        mt[...] = jnp.zeros((NG, 128, 128), f32)
        return None

    def p_gate(part):
        def f():
            g_lane = _sigmoid(beta_ref[...].astype(f32))
            g_lane = jnp.concatenate([g_lane, jnp.zeros((1, 128 - H), f32)], axis=1)
            if part < NG:
                g = part
                hid = jnp.where(head_in_group < 7, head_in_group + 7 * g, 999)
                sel = jnp.where(lane128 == hid, jnp.broadcast_to(g_lane, (128, 128)), 0.0)
                v = jnp.broadcast_to(jnp.sum(sel, axis=1, keepdims=True), (128, 128))
                grow[g] = v
                return tok_of(v)
            r32 = _iota((32, 128), 0)
            tk = None
            for h in range(8 * (part - NG), 8 * (part - NG) + 8):
                j = h % 7
                off = 18 * j - 16 * ((9 * j) // 8)
                gh = jnp.broadcast_to(g_lane[:, h:h + 1], (32, 128))
                v = jnp.where((r32 >= off) & (r32 < off + 18), 1.0 - gh, 0.0)
                omg[h] = v
                tk = tok_of(v) if tk is None else tk | tok_of(v)
            return tk
        return f

    def p_wcol():
        wr = _pad_lanes(wr_ref[...].astype(f32).reshape(1, D))
        v = jnp.broadcast_to(wr, (128, DP)).T[0:D]
        wcol[...] = v
        return tok_of(v)

    def p_tr(w_ref, c):
        def f():
            wd_ = min(128, D - 128 * c)
            v = _pack(w_ref[:, 128 * c:128 * c + wd_].T)
            wtmp[64 * c:64 * c + wd_ // 2, :] = v
            return v[0:8, 0:128]
        return f

    def p_perm(w):
        def f():
            v = _pad_lanes(_perm_rows(wtmp[...], 40))
            wall[296 * w:296 * (w + 1), :] = v
            return v[0:8, 0:128] | v[288:296, 0:128]
        return f

    def p_wo_perm():
        v = _perm_rows(_pack(wo_v[...]), 64)
        wtmp2[...] = v
        return v[0:8, 0:128]

    def p_wo_tr(c):
        def f():
            wd_ = min(128, D - 128 * c)
            v = _pack(_unpack(wtmp2[:, 128 * c:128 * c + wd_]).T)
            wot[64 * c:64 * c + wd_ // 2, :] = v
            return v[0:8, 0:128]
        return f

    def p_wait(*cs):
        def f():
            for c_ in cs:
                c_()
            return None
        return f

    def layer_norm_tile(seg, t):
        xf = x_v[4 * seg + t].astype(f32)
        v = _pack(_layernorm_t(xf).astype(bf16))
        xn[0:288, 128 * t:128 * (t + 1)] = v
        return v[0:8] | v[280:288]

    wk_cp.start()
    xn[288:320, :] = jnp.zeros((32, L), u32)
    for ref in (qt, phq, phk, vt):
        ref[NG - 1, 40:64] = jnp.zeros((24, L), u32)
    for u in range(4):
        x_cp[u].wait()
    wv_cp.start()
    layer_norm_tile(0, 0)
    wq_cp.wait()
    wo_cp.start()
    for c in range(NG):
        p_tr(wq_v, c)()
    p_perm(0)()
    for t in range(1, 4):
        layer_norm_tile(0, t)

    diag = _iota((128, 128), 0) <= _iota((128, 128), 1)

    def qk_logits(h, i):
        g, j = h // 7, h % 7
        n = 128 * (i + 1)
        qw = qt[g, :, 128 * i:128 * (i + 1)] & msk[j]
        s = jnp.dot(_unpack(kp[g, 0:n // 2, :]), _unpack(qw), preferred_element_type=f32)
        sl = jnp.where(diag, s[n - 128:], -1e30)
        return sl if i == 0 else jnp.concatenate([s[:n - 128], sl], axis=0)

    def pv(h, i, pb):
        g, j = h // 7, h % 7
        n = 128 * (i + 1)
        a8 = pl.multiple_of(((9 * j) // 8) * 8, 8)
        vw = vt[g, pl.ds(a8, 16), 0:n]
        mk = msk[j, pl.ds(a8, 16), :]
        mk = jnp.concatenate([mk] * (i + 1), axis=1)
        vw = (vw & mk) | (jnp.full((16, n), 0x3F803F80, u32) & ~mk)
        o = jnp.dot(_unpack(vw), pb, preferred_element_type=f32)
        og = omg[h]
        r32_ = _iota((32, 128), 0)
        off = 18 * j - 2 * a8
        is_head = (r32_ >= off) & (r32_ < off + 18)
        lsum = jnp.sum(jnp.where(is_head, 0.0, o), axis=0, keepdims=True)
        r = pl.reciprocal(lsum, approx=True) * 14.0
        w16 = pl.multiple_of(a8 * 2, 16)
        ot[g, pl.ds(w16, 32), 128 * i:128 * (i + 1)] += o * (r * og)

    pbs = (pb0, pb1)
    sbs = (sb0, sb1)
    mbs = (mb0, mb1)
    IORD = (3, 2, 1, 0)

    def fast_qk(h, i, pbuf):
        g, j = h // 7, h % 7
        a = (9 * j) // 8
        n = 128 * (i + 1)
        qw = qt[g, 8 * a:8 * a + 16, 128 * i:128 * (i + 1)] & msk[j, 8 * a:8 * a + 16, :]
        parts = [jnp.zeros((8 * a, 128), u32)] if a > 0 else []
        parts.append(qw)
        if 48 - 8 * a > 0:
            parts.append(jnp.zeros((48 - 8 * a, 128), u32))
        qm = _unpack(jnp.concatenate(parts, axis=0))
        s = jnp.dot(_unpack(kp[g, 0:n // 2, :]), qm, preferred_element_type=f32)
        sl = jnp.where(diag, s[n - 128:], -1e30)
        s = sl if i == 0 else jnp.concatenate([s[:n - 128], sl], axis=0)
        pbuf[OFF[i] // 2:(OFF[i] + n) // 2, :] = _pack(jnp.exp2(s).astype(bf16))

    def fast_pv(h, i, pbuf):
        g, j = h // 7, h % 7
        a = (9 * j) // 8
        n = 128 * (i + 1)
        pb = _unpack(pbuf[OFF[i] // 2:(OFF[i] + n) // 2, :])
        mk = msk[j, 8 * a:8 * a + 16, :]
        mk = jnp.concatenate([mk] * (i + 1), axis=1)
        vw = (vt[g, 8 * a:8 * a + 16, 0:n] & mk) | (jnp.full((16, n), 0x3F803F80, u32) & ~mk)
        o = jnp.dot(_unpack(vw), pb, preferred_element_type=f32)
        off = 18 * j - 16 * a
        l8 = o[24:32] if off <= 6 else o[0:8]
        r = pl.reciprocal(l8, approx=True)
        for t in range(4):
            if 8 * t + 8 <= off or 8 * t >= off + 18:
                continue
            rs_ = slice(16 * a + 8 * t, 16 * a + 8 * t + 8)
            cs = slice(128 * i, 128 * (i + 1))
            ot[g, rs_, cs] += o[8 * t:8 * t + 8] * (r * omg[h, 8 * t:8 * t + 8, :])

    def slow_qk(h, i, sbuf, mbuf):
        n = 128 * (i + 1)
        s = qk_logits(h, i)
        sbuf[OFF[i]:OFF[i] + n, :] = s
        mbuf[8 * i:8 * i + 8, :] = jnp.broadcast_to(jnp.max(s, axis=0, keepdims=True), (8, 128))

    def slow_pv(h, i, sbuf, mbuf):
        n = 128 * (i + 1)
        s = sbuf[OFF[i]:OFF[i] + n, :]
        p = jnp.exp2(s - mbuf[8 * i:8 * i + 1, :]).astype(bf16)
        pv(h, i, p)

    def attention_fast():
        for i in IORD:
            fast_qk(0, i, pbs[0])
        for h in range(H):
            if h + 1 < H:
                for i in IORD:
                    fast_qk(h + 1, i, pbs[(h + 1) % 2])
            for i in IORD:
                fast_pv(h, i, pbs[h % 2])

    def attention_slow():
        for i in IORD:
            slow_qk(0, i, sbs[0], mbs[0])

        def body(it, c):
            for u in range(UN_SLOW):
                h = it * UN_SLOW + u
                hn_ = jnp.minimum(h + 1, H - 1)
                for i in IORD:
                    slow_qk(hn_, i, sbs[1 - u % 2], mbs[1 - u % 2])
                for i in IORD:
                    slow_pv(h, i, sbs[u % 2], mbs[u % 2])
            return c
        lax.fori_loop(0, H // UN_SLOW, body, 0)

    def wait_x(seg):
        for t in range(NSEG):
            @pl.when(seg == t)
            def _():
                for u in range(4):
                    x_cp[4 * t + u].wait()

    NPC = D // PCH

    def post_piece(seg, t, ch, valid):
        m = st[t, 0:1, :]
        rs = st[t, 1:2, :]
        rsl = slice(PCH * ch, PCH * (ch + 1))
        hf = hbuf[t, rsl].astype(f32)
        hnb = ((hf - m) * rs).astype(bf16)
        hnf = hnb.astype(f32)
        hn_v[4 * seg + t, rsl] = hnb
        ob_ = (hf + hnf).astype(bf16)
        out_v[4 * seg + t, rsl] = ob_
        r_ = jnp.sum((hnf * wcol[rsl]).reshape(PCH // 8, 8, 128), axis=0)
        if ch > 0:
            r_ = r_ + racc[...]
        if ch < NPC - 1:
            racc[...] = r_
        else:
            bv = best[0]
            bi = best[1]
            lane = _iota((8, 128), 1).astype(f32)
            rr = jnp.sum(r_, axis=0, keepdims=True).astype(bf16).astype(f32)
            rt = jnp.broadcast_to(rr, (8, 128))
            upd_ = rt > bv
            if valid is not None:
                upd_ = jnp.logical_and(upd_, valid)
            best[0] = jnp.where(upd_, rt, bv)
            best[1] = jnp.where(upd_, lane + jnp.asarray(seg * L + 128 * t, i32).astype(f32), bi)
        return _pack(ob_[0:16]) | pltpu.bitcast(r_, u32)

    def start_out(seg):
        for t in range(NSEG):
            @pl.when(seg == t)
            def _():
                for u in range(4):
                    o_cp[4 * t + u].start()

    def post_p(seg, t, ch, valid):
        return lambda: post_piece(seg, t, ch, valid)

    def qkv_block(pieces, opaque):
        pieces = list(pieces)
        zero = jnp.full((8, 128), lax.shift_right_logical(opaque, 8), i32).astype(u32)
        tok = None
        for w in range(3):
            m_ = None
            for t in range(4):
                cs = slice(128 * t, 128 * (t + 1))
                xt_ = _unpack(xn[:, cs])
                for g in range(NG):
                    nr = 128 if g < NG - 1 else 80
                    while pieces and pieces[0][0] is not None and pieces[0][0] <= (w * 4 + t) * NG + g - 1e-9:
                        tk = pieces.pop(0)[1]()
                        if tk is not None:
                            tok = tk if tok is None else tok | tk
                    r0_ = DC * w + 128 * g
                    lhs = wall[r0_ // 2:(r0_ + nr) // 2, :]
                    if tok is not None:
                        head = lhs[0:8, 0:128] | (tok & zero)
                        lhs = jnp.concatenate([
                            jnp.concatenate([head, lhs[0:8, 128:]], axis=1), lhs[8:]], axis=0)
                        tok = None
                    a = jnp.dot(_unpack(lhs), xt_, preferred_element_type=f32)
                    if w == 0:
                        phq[g, 0:nr // 2, cs] = _pack(_phi(a).astype(bf16))
                        a = a * QSCALE
                        qt[g, 0:nr // 2, cs] = _pack(a.astype(bf16))
                    elif w == 1:
                        phk[g, 0:nr // 2, cs] = _pack(_phi(a).astype(bf16))
                        ab = a.astype(bf16)
                        if nr < 128:
                            ab = jnp.concatenate([ab, jnp.zeros((128 - nr, 128), bf16)], axis=0)
                        kp[g, 64 * t:64 * (t + 1), :] = _pack(ab.T)
                    else:
                        vt[g, 0:nr // 2, cs] = _pack(a.astype(bf16))
                    am = jnp.max(jnp.abs(a).reshape(nr // 8, 8, 128), axis=0)
                    m_ = am if m_ is None else jnp.maximum(m_, am)
            mxs[w] = m_
        assert not pieces

    p0 = []
    p0.append((0.5, p_wait(wk_cp.wait, *[x_cp[t].start for t in range(4, NTILE)])))
    for c in range(NG):
        p0.append((1 + c, p_tr(wk_v, c)))
    p0.append((7, p_perm(1)))
    p0.append((8.5, p_wait(wv_cp.wait)))
    for c in range(NG):
        p0.append((9 + c, p_tr(wv_v, c)))
    p0.append((15, p_perm(2)))
    p0.append((16.5, p_wait(wo_cp.wait, wg_cp.start, wu_cp.start, wd_cp.start, beta_cp.wait, wr_cp.wait)))
    p0.append((17, p_wo_perm))
    for c in range(NG):
        p0.append((19 + c, p_wo_tr(c)))
    p0.append((25, p_masks))
    p0.append((26, p_zero_mt))
    for part in range(NG + 4):
        p0.append((28 + 2 * part, p_gate(part)))
    p0.append((47, p_wcol))
    def p_zero_ot(g):
        def f():
            ot[g] = jnp.zeros((128, L), f32)
            return None
        return f
    for g in range(NG):
        p0.append((49 + 2 * g, p_zero_ot(g)))
    qkv_block(p0, pl.program_id(0))

    def segment(s, c):
        mxv = [_absmax(mxs[w]) for w in range(3)]
        bound = mxv[0] * mxv[1] * (DH * 1.02)
        ok = jnp.where((bound <= BOUND) & (mxv[2] <= VBOUND), 1, 0).astype(i32)
        safe = jnp.max(ok) > 0

        @pl.when(safe)
        def _():
            attention_fast()

        @pl.when(jnp.logical_not(safe))
        def _():
            attention_slow()

        def wo_tile(t, dep):
            cs = slice(128 * t, 128 * (t + 1))
            ob = jnp.concatenate([ot[g, :, cs] for g in range(NG)], axis=0).astype(bf16)
            lhs = wot[...]
            if dep is not None:
                lhs = jnp.concatenate([
                    jnp.concatenate([lhs[0:8, 0:128] | dep, lhs[0:8, 128:]], axis=1), lhs[8:]], axis=0)
            ao = jnp.dot(_unpack(lhs), ob, preferred_element_type=f32)
            piv = s1 = s2 = None
            for ch in range(D // PCH):
                rsl = slice(PCH * ch, PCH * (ch + 1))
                hb = (x_v[4 * s + t, rsl].astype(f32) + ao[rsl]).astype(bf16)
                hbuf[t, rsl] = hb
                h_v[4 * s + t, rsl] = hb
                hf = hb.astype(f32)
                if piv is None:
                    piv = hf[0:1, :]
                dd = hf - piv
                a1 = jnp.sum(dd.reshape(PCH // 8, 8, 128), axis=0)
                a2 = jnp.sum((dd * dd).reshape(PCH // 8, 8, 128), axis=0)
                s1 = a1 if s1 is None else s1 + a1
                s2 = a2 if s2 is None else s2 + a2
            e1 = jnp.sum(s1, axis=0, keepdims=True) * (1.0 / D)
            e2 = jnp.sum(s2, axis=0, keepdims=True) * (1.0 / D)
            var = jnp.maximum(e2 - e1 * e1, 0.0)
            st[t, 0:1, :] = piv + e1
            st[t, 1:2, :] = lax.rsqrt(var + EPS)

        zero = jnp.full((8, 128), lax.shift_right_logical(s, 8), i32).astype(u32)

        @pl.when(s < NSEG - 1)
        def _():
            wait_x(s + 1)
            r64_ = _iota((64, L), 0)
            ones = jnp.full((64, L), 0x3F803F80, u32)
            for g in range(NG):
                lhs = jnp.where(r64_ == 63, ones, vt[g])
                upd = lax.dot_general(_unpack(lhs), _unpack(phk[g]), NT,
                                      preferred_element_type=f32)
                cur = mt[g] + upd
                mt[g] = cur
                m_bd = jnp.where(bd_mask, cur, 0.0)
                z_bd = jnp.where(bd_mask, jnp.broadcast_to(cur[126:127, :], (128, 128)), 0.0)
                mlhs[g] = _pack(jnp.concatenate([m_bd, z_bd], axis=0).astype(bf16))
            dep = None
            for t in range(4):
                tk = layer_norm_tile(s + 1, t)
                wo_tile(t, dep)
                dep = tk & zero
            qkv_block([(PST + PSP * (t * NPC + ch), post_p(s, t, ch, None))
                       for t in range(4) for ch in range(NPC)], s)
            for g in range(NG):
                nr = 128 if g < NG - 1 else 80
                lhs = jnp.concatenate([mlhs[g, 0:nr // 2], mlhs[g, 64:64 + nr // 2]], axis=0)
                nd = jnp.dot(_unpack(lhs), _unpack(phq[g]), preferred_element_type=f32)
                num = nd[0:nr]
                den = nd[nr:2 * nr] + 1e-06
                gr = grow[g, 0:nr]
                ot[g, 0:nr] = num * (pl.reciprocal(den, approx=True) * jnp.concatenate([gr] * 4, axis=1))
            start_out(s)

        @pl.when(s == NSEG - 1)
        def _():
            dep = None
            for t in range(4):
                wo_tile(t, dep)
                dep = None
                if t > 0:
                    for ch in range(NPC):
                        tk = post_piece(s, t - 1, ch, None)
                        dep = tk if dep is None else dep | tk
                    dep = dep & zero
            for ch in range(NPC):
                post_piece(s, 3, ch, None)
        return c

    lax.fori_loop(0, NSEG, segment, 0)
    for u in range(4):
        o_cp[4 * (NSEG - 1) + u].start()

    bv = best[0]
    bi = best[1]
    vmax = jnp.max(bv, axis=1, keepdims=True)
    cand = jnp.where(bv == vmax, bi, float(S))
    imin = jnp.min(cand, axis=1, keepdims=True)
    idx = jnp.minimum(jnp.max(imin).astype(i32), S - 1)
    tile = idx // 128
    col = idx - tile * 128
    col16 = pl.multiple_of((col // 16) * 16, 16)
    hn_t = hn_v[tile]
    lane_sel = _iota((D, 128), 1) == col
    xs_t = jnp.where(lane_sel, hn_t, jnp.zeros_like(hn_t))
    xs_t = jnp.concatenate([xs_t, jnp.zeros((DP - D, 128), bf16)], axis=0)
    pb0[0:64, :] = jnp.zeros((64, 128), u32)
    xall = xs_t.T
    xn[0:64, 0:L] = _pack(xall[:, 0:L])
    pb0[0:64, :] = _pack(xall[:, L:DP])
    c8 = pl.multiple_of(col16 // 2, 8)
    xs = _unpack(jnp.concatenate([xn[pl.ds(c8, 8), 0:L], pb0[pl.ds(c8, 8), 0:64]], axis=1))
    wg_cp.wait()
    wu_cp.wait()
    gt = jnp.dot(xs, wg_v[...], preferred_element_type=f32)
    up = jnp.dot(xs, wu_v[...], preferred_element_type=f32)
    act = (gt * _sigmoid(gt) * up).astype(bf16).astype(f32)
    act = jnp.broadcast_to(jnp.sum(act, axis=0, keepdims=True), (8, F))
    wd_cp.wait()
    cols = []
    RB = 64
    for rb in range(D // RB):
        acc = None
        for c in range(F // 128):
            wv_ = wd_v[RB * rb:RB * (rb + 1), 128 * c:128 * (c + 1)].astype(f32)
            pr = wv_.reshape(RB // 8, 8, 128) * act[None, :, 128 * c:128 * (c + 1)]
            acc = pr if acc is None else acc + pr
        cols.append(jnp.sum(acc.reshape(RB, 128), axis=1, keepdims=True))
    ycol = jnp.concatenate(cols, axis=0)
    rsel = _sigmoid(vmax[0:1, 0:1])
    ycol = (ycol.astype(bf16).astype(f32) * rsel).astype(bf16).astype(f32)
    fin = (h_v[tile].astype(f32)
           + (hn_t.astype(f32) + jnp.where(lane_sel, ycol, 0.0))).astype(bf16)
    for t in range(NTILE):
        o_cp[t].wait()
    out_v[tile] = fin
    pc = cp(out_v.at[tile], out_hbm.at[:, pl.ds(pl.multiple_of(tile * 128, 128), 128)], 15)
    pc.start()
    pc.wait()


@jax.jit
def pallas_sequential_preLN__memory_aug_infini_attn__moe_arch_mod__prompt_kernel(
    A_x: jax.Array,
    A_wq: jax.Array,
    A_wk: jax.Array,
    A_wv: jax.Array,
    A_wo: jax.Array,
    A_beta: jax.Array,
    B_x: jax.Array,
    B_w_r: jax.Array,
    B_w_gate: jax.Array,
    B_w_up: jax.Array,
    B_w_down: jax.Array,
):
    del B_x
    xt = A_x.reshape(S, D).T
    wdt = B_w_down.T
    beta = A_beta.reshape(1, H)
    wr = B_w_r
    hbm = pl.BlockSpec(memory_space=pltpu.HBM)
    V = pltpu.VMEM
    scratch = [
        V((NTILE, D, 128), bf16),
        V((D, D), bf16), V((D, D), bf16), V((D, D), bf16), V((D, D), bf16),
        V((D, F), bf16), V((D, F), bf16), V((D, F), bf16),
        V((3 * DC // 2, DP), u32),
        V((D // 2, DP), u32),
        V((D // 2, D), u32),
        V((DP // 2, D), u32),
        V((DP // 2, L), u32),
        V((NG, L // 2, 128), u32),
        V((NG, 64, L), u32),
        V((NG, 64, L), u32),
        V((NG, 64, L), u32),
        V((NG, 64, L), u32),
        V((NG, 128, L), f32),
        V((640, 128), u32), V((640, 128), u32),
        V((1280, 128), f32), V((1280, 128), f32),
        V((32, 128), f32), V((32, 128), f32),
        V((NG, 128, 128), f32),
        V((NG, 128, 128), u32),
        V((4, D, 128), bf16),
        V((4, 8, 128), f32),
        V((3, 8, 128), f32),
        V((8, 128), f32),
        V((NTILE, D, 128), bf16), V((NTILE, D, 128), bf16), V((NTILE, D, 128), bf16),
        V((7, 64, 128), u32),
        V((H, 32, 128), f32),
        V((NG, 128, 128), f32),
        V((D, 128), f32),
        V((2, 8, 128), f32),
        V((1, H), bf16), V((D,), bf16),
        pltpu.SemaphoreType.DMA((18,)),
    ]
    out_t = pl.pallas_call(
        _kernel,
        out_shape=jax.ShapeDtypeStruct((D, S), bf16),
        grid=(1,),
        in_specs=[hbm] * 10,
        out_specs=hbm,
        scratch_shapes=scratch,
        compiler_params=pltpu.CompilerParams(vmem_limit_bytes=100 * 1024 * 1024),
    )(xt, A_wq, A_wk, A_wv, A_wo, beta, wr, B_w_gate, B_w_up, wdt)
    return out_t.T.reshape(1, S, D)
```
